```python
import jax
import jax.numpy as jnp

def _softmax(x, axis=-1):
    return jax.nn.softmax(x, axis=axis)

def _gelu(x):
    return jax.nn.gelu(x, approximate=True)

def _silu(x):
    return jax.nn.silu(x)

def _sigmoid(x):
    return jax.nn.sigmoid(x)

def _layernorm(x, axis=-1, eps=1e-05):
    m = jnp.mean(x, axis=axis, keepdims=True)
    v = jnp.var(x, axis=axis, keepdims=True)
    return (x - m) / jnp.sqrt(v + eps)

def _scatter_add(tgt, idx, src, axis=0):
    return tgt.at[idx].add(src)

def _segment_sum(src, seg, n):
    return jax.ops.segment_sum(src, seg, n)

class _Rng:

    def __init__(self, key):
        self._k = key

    def _next(self):
        self._k, sub = jax.random.split(self._k)
        return sub

    def normal(self, shape):
        return jax.random.normal(self._next(), shape, dtype=jnp.bfloat16)

    def randint(self, lo, hi, shape):
        return jax.random.randint(self._next(), shape, lo, hi, dtype=jnp.int32)

    def uniform(self, shape, lo=0.0, hi=1.0):
        return jax.random.uniform(self._next(), shape, jnp.bfloat16, lo, hi)

    def permutation(self, n):
        return jax.random.permutation(self._next(), n)
kernel_name = 'interleave_layers__linear_kernel_hedgehog__memory_aug_recurrent_mem_tr__prompt'

def setup_inputs():
    _rng = _Rng(jax.random.key(int.from_bytes(__import__("os").urandom(4), "little")))
    _w = lambda a: (lambda t: t.astype(jnp.bfloat16) if jnp.issubdtype(t.dtype, jnp.floating) else t)(jnp.asarray(a))

    def _A_setup():
        B, S, D, H = (1, 2048, 640, 32)
        Dh = D // H
        return {'x': _w((lambda *s: _rng.normal(s) * 0.05)(B, S, D)), 'wqkv': _w((lambda *s: _rng.normal(s) * 0.05)(D, 3 * D)), 'w_phi': _w((lambda *s: _rng.normal(s) * 0.05)(H, Dh, Dh) * Dh ** (-0.5)), 'wo': _w((lambda *s: _rng.normal(s) * 0.05)(D, D))}
    _A_in = _A_setup()

    def _B_setup():
        B, S, Dm = (1, 2048, 640)
        H, Dh = (32, 192)
        M, seg = (8, 32)
        seg = min(seg, S)
        S = S // seg * seg
        return {'x': _w((lambda *s: _rng.normal(s) * 0.05)(B, S, Dm)), 'mem0': _w((lambda *s: _rng.normal(s) * 0.05)(B, M, Dm)), 'Wq': _w((lambda *s: _rng.normal(s) * 0.05)(Dm, H, Dh) * Dm ** (-0.5)), 'Wk': _w((lambda *s: _rng.normal(s) * 0.05)(Dm, H, Dh) * Dm ** (-0.5)), 'Wv': _w((lambda *s: _rng.normal(s) * 0.05)(Dm, H, Dh) * Dm ** (-0.5)), 'Wo': _w((lambda *s: _rng.normal(s) * 0.05)(H, Dh, Dm) * (H * Dh) ** (-0.5)), 'seg_len': seg}
    _B_in = _B_setup()
    return {'A_x': _A_in['x'], 'A_wqkv': _A_in['wqkv'], 'A_w_phi': _A_in['w_phi'], 'A_wo': _A_in['wo'], 'B_x': _B_in['x'], 'B_mem0': _B_in['mem0'], 'B_Wq': _B_in['Wq'], 'B_Wk': _B_in['Wk'], 'B_Wv': _B_in['Wv'], 'B_Wo': _B_in['Wo'], 'B_seg_len': _B_in['seg_len']}

def reference(A_x, A_wqkv, A_w_phi, A_wo, B_x, B_mem0, B_Wq, B_Wk, B_Wv, B_Wo, B_seg_len):

    def _A_ref(x, wqkv, w_phi, wo):
        B, S, D = x.shape
        H = 32
        Dh = D // H
        qkv = (lambda x, *d: x.transpose(*d))((x @ wqkv).reshape(B, S, 3, H, Dh), 2, 0, 3, 1, 4)
        q, k, v = (qkv[0], qkv[1], qkv[2])
        pq = jnp.einsum('bhsd,hdf->bhsf', q, w_phi)
        pk = jnp.einsum('bhsd,hdf->bhsf', k, w_phi)
        phi_q = jnp.concatenate([_softmax(pq, axis=-1), _softmax(-pq, axis=-1)], axis=-1)
        phi_k = jnp.concatenate([_softmax(pk, axis=-1), _softmax(-pk, axis=-1)], axis=-1)
        kv = jnp.einsum('bhsf,bhsd->bhfd', phi_k, v)
        z = jnp.einsum('bhsf->bhf', phi_k)
        num = jnp.einsum('bhqf,bhfd->bhqd', phi_q, kv)
        den = jnp.einsum('bhqf,bhf->bhq', phi_q, z)[..., None] + 1e-06
        o = num / den
        return (lambda x, *d: x.transpose(*d))(o, 0, 2, 1, 3).reshape(B, S, D) @ wo

    def _B_ref(x, mem0, Wq, Wk, Wv, Wo, seg_len):
        B, S, Dm = x.shape
        H, Dh = (Wq.shape[1], Wq.shape[2])
        M = mem0.shape[1]
        scale = Dh ** (-0.5)
        n_seg = S // seg_len
        L = M + seg_len
        idx = jnp.arange(L)
        mask = (idx[:, None] < M) | (idx[:, None] >= idx[None, :])
        mem = mem0
        outs = []
        for s in range(n_seg):
            xs = x[:, s * seg_len:(s + 1) * seg_len, :].copy()
            h = jnp.concatenate([mem, xs], axis=1)
            q = jnp.einsum('btd,dhe->bhte', h, Wq)
            k = jnp.einsum('btd,dhe->bhte', h, Wk)
            v = jnp.einsum('btd,dhe->bhte', h, Wv)
            scores = jnp.einsum('bhqe,bhke->bhqk', q, k) * scale
            scores = jnp.where(mask[None, None], scores, -1000000000.0)
            p = _softmax(scores, axis=-1)
            o = jnp.einsum('bhqk,bhke->bhqe', p, v)
            o = jnp.einsum('bhte,hed->btd', o, Wo)
            mem = o[:, :M, :].copy()
            outs.append(o[:, M:, :])
        return jnp.concatenate(outs, axis=1)
    x = A_x
    x = x + _A_ref(_layernorm(x, axis=-1), A_wqkv, A_w_phi, A_wo)
    x = x + _B_ref(_layernorm(x, axis=-1), B_mem0, B_Wq, B_Wk, B_Wv, B_Wo, B_seg_len)
    x = x + _A_ref(_layernorm(x, axis=-1), A_wqkv, A_w_phi, A_wo)
    x = x + _B_ref(_layernorm(x, axis=-1), B_mem0, B_Wq, B_Wk, B_Wv, B_Wo, B_seg_len)
    return x
```

```python
import functools

import jax
import jax.numpy as jnp
from jax import lax
import jax.experimental.pallas as pl
import jax.experimental.pallas.tpu as pltpu

f32, bf16, u32 = jnp.float32, jnp.bfloat16, jnp.uint32

S, D = 2048, 640
HA, FA = 32, 20
HB, DHB = 32, 192
MEM, SEG = 8, 32
L = MEM + SEG
NP = HB // 2
PW = 2 * DHB
TB = 128
NG = 4
NT = (((1,), (1,)), ((), ()))


def _dot(a, b):
    return jnp.dot(a, b, preferred_element_type=f32)


def _dot_nt(a, b):
    return lax.dot_general(a, b, NT, preferred_element_type=f32)


def _pack(x):
    return pltpu.bitcast(x.astype(bf16), u32)


def _unpack(x):
    return pltpu.bitcast(x, bf16)


def _recip(x):
    r = pl.reciprocal(x, approx=True)
    return r * (2.0 - x * r)


def _layernorm(x):
    m = jnp.mean(x, axis=-1, keepdims=True)
    xc = x - m
    v = jnp.mean(xc * xc, axis=-1, keepdims=True)
    return xc * lax.rsqrt(v + 1e-5)


def _iota(shape, dim):
    return lax.broadcasted_iota(jnp.int32, shape, dim)


def _kernel(x_ref, wqkv_ref, wphi_ref, woa_ref, mem0_ref, wqt_hbm, wkt_hbm, wvt_hbm, wob_hbm,
            out_ref,
            stage_ref, wb_ref, wob_ref, xres_ref, xna_ref, xnb_ref,
            wpq_ref, wpkt_ref, wv_ref, acc_ref, kvw_ref, z_ref,
            mem_ref, svq_ref, svo_ref, sems):
    big = [pltpu.make_async_copy(src, stage_ref.at[i], sems.at[i])
           for i, src in enumerate((wqt_hbm, wkt_hbm, wvt_hbm, wob_hbm))]
    for c in big:
        c.start()

    wphi = wphi_ref[...].astype(f32)
    tmat = jnp.concatenate([wphi[:, f, :] for f in range(FA)], axis=1)
    tmat = jnp.concatenate([tmat, jnp.zeros((32 - FA, D), f32)], axis=0).astype(bf16)
    r_row, r_col = _iota((D, 32), 0), _iota((D, 32), 1)
    r_head = (r_row * 3277) >> 16
    rep = (r_row - FA * r_head == r_col).astype(f32).astype(bf16)
    p_row, p_col = _iota((D, D), 0), _iota((D, D), 1)
    phi = jnp.where(((p_row * 3277) >> 16) == (p_col & 31), _dot(rep, tmat), 0.0).astype(bf16)
    wpq_ref[...] = _pack(_dot(wqkv_ref[:, 0:D], phi))
    wpkt = _dot(wqkv_ref[:, D:2 * D], phi).T.reshape(FA, HA, D)
    for g in range(NG):
        wpkt_ref[g] = _pack(wpkt[:, 8 * g:8 * g + 8, :].reshape(8 * FA, D))
    wv_ref[...] = pltpu.bitcast(wqkv_ref[:, 2 * D:3 * D], u32)

    def kside_mm(x):
        xn = _layernorm(x).astype(bf16)
        v = _dot(xn, _unpack(wv_ref[...])).astype(bf16)
        pk = [_dot_nt(_unpack(wpkt_ref[g]), xn) for g in range(NG)]
        return xn, v, pk

    def kside_kv(v, pk):
        lane = _iota((TB, 128), 1)
        out = []
        for g in range(NG):
            p = pk[g].reshape(FA, 8, TB)
            ep = jnp.exp(p - jnp.max(p, axis=0, keepdims=True))
            en = jnp.exp(jnp.min(p, axis=0, keepdims=True) - p)
            ep = ep * _recip(jnp.sum(ep, axis=0, keepdims=True))
            en = en * _recip(jnp.sum(en, axis=0, keepdims=True))
            lhs = jnp.concatenate([ep, en], axis=0).reshape(16 * FA, TB).astype(bf16)
            w0, w1 = v[:, 128 * g:128 * g + 128], v[:, 128 * g + 128:128 * g + 256]
            one = jnp.ones((TB, 128), bf16)
            if g < NG - 1:
                w1 = jnp.where(lane == 127, one, w1)
            else:
                w0 = jnp.where(lane == 0, one, w0)
            out.append(_dot(lhs, jnp.concatenate([w0, w1], axis=1)))
        return out

    def kside_pass(load_x, nsub):
        acc_ref[...] = jnp.zeros(acc_ref.shape, f32)

        def body(i, c):
            st = {}

            def mm(j):
                r0 = pl.multiple_of((i * nsub + j) * TB, TB)
                xn, v, pk = kside_mm(load_x(r0))
                xna_ref[pl.ds(pl.multiple_of(r0 // 2, TB // 2), TB // 2), :] = pltpu.bitcast(xn, u32)
                st[j] = (v, pk)

            def kv(j):
                o = kside_kv(*st[j])
                for g in range(NG):
                    acc_ref[g] += o[g]

            for j in range(nsub):
                mm(j)
                if j >= 1:
                    kv(j - 1)
            kv(nsub - 1)
            return c
        lax.fori_loop(0, S // (TB * nsub), body, 0)

    def build_kvw():
        row, col = _iota((16 * FA, 256), 0), _iota((16 * FA, 256), 1)
        lane = _iota((16 * FA, 128), 1)
        kws, zs = [], []
        for g in range(NG):
            a = acc_ref[g]
            lo = 32 * g + FA * (row & 7)
            kv = jnp.where((col >= lo) & (col < lo + FA), a, 0.0).astype(bf16)
            kws.append(_dot(kv, woa_ref[128 * g:128 * g + 256, :]).reshape(2 * FA, 8, D))
            zt = jnp.where(lane == 127, a[:, 128:], 0.0) if g < NG - 1 else jnp.where(lane == 0, a[:, :128], 0.0)
            zc = jnp.sum(zt, axis=1, keepdims=True)
            zs.append(jnp.broadcast_to(zc, (16 * FA, 128)).reshape(2 * FA, 8, 128))
        kvw_ref[...] = _pack(jnp.concatenate(kws, axis=1).reshape(2 * D, D))
        z_ref[...] = jnp.concatenate(zs, axis=1).reshape(2 * D, 128).T[0:8, :]

    def fold5(x, op):
        r = op(op(op(x[:, 0:128], x[:, 128:256]), op(x[:, 256:384], x[:, 384:512])), x[:, 512:640])
        r = op(r, pltpu.roll(r, 32, 1))
        return op(r, pltpu.roll(r, 64, 1))

    def tile5(x):
        return jnp.concatenate([x] * 5, axis=1)

    def qside_phi(pq):
        ep = jnp.exp(pq - tile5(fold5(pq, jnp.maximum)))
        en = jnp.exp(tile5(fold5(pq, jnp.minimum)) - pq)
        rp = _recip(fold5(ep, jnp.add))
        rn = _recip(fold5(en, jnp.add))
        ep = ep * tile5(rp)
        en = en * tile5(rn)
        z = z_ref[0:1, :]
        den = fold5(ep * z[:, :D] + en * z[:, D:], jnp.add) + 1e-6
        rd = tile5(1.0 / den)
        return jnp.concatenate([ep * rd, en * rd], axis=1).astype(bf16)

    def qside_pass(load_x, nsub, extra):
        def body(i, c):
            st = {}

            def mm1(j):
                r0 = pl.multiple_of((i * nsub + j) * TB, TB)
                xn = _unpack(xna_ref[pl.ds(pl.multiple_of(r0 // 2, TB // 2), TB // 2), :])
                st[j] = _dot(xn, _unpack(wpq_ref[...]))

            def mm2(j):
                r0 = pl.multiple_of((i * nsub + j) * TB, TB)
                y = load_x(r0) + _dot(qside_phi(st[j]), _unpack(kvw_ref[...]))
                xres_ref[pl.ds(r0, TB), :] = y
                xnb_ref[pl.ds(r0, TB), :] = _layernorm(y)
                if extra is not None:
                    extra(i * nsub + j)

            mm1(0)
            for j in range(nsub):
                if j + 1 < nsub:
                    mm1(j + 1)
                mm2(j)
            return c
        lax.fori_loop(0, S // (TB * nsub), body, 0)

    def relayout_weights(j):
        r0 = pl.multiple_of(j * PW, PW)
        for m in range(3):
            wb_ref[j, :, m * PW:(m + 1) * PW] = pltpu.bitcast(stage_ref[m, pl.ds(r0, PW), :].T, u32)
        wob_ref[j] = pltpu.bitcast(stage_ref[3, pl.ds(r0, PW), :], u32)

    scale = DHB ** -0.5
    row, col = _iota((2 * L, 2 * L), 0), _iota((2 * L, 2 * L), 1)
    same = (row < L) == (col < L)
    rr = jnp.where(row < L, row, row - L)
    kk = jnp.where(col < L, col, col - L)
    keep = same & ((rr < MEM) | (rr >= kk))
    fill = jnp.where(same, -1e9, -jnp.inf).astype(f32)
    lo_half = _iota((L, 128), 1) < 64

    def halves(mid):
        return jnp.concatenate([jnp.where(lo_half, mid, 0.0), jnp.where(lo_half, 0.0, mid)], axis=0).astype(bf16)

    def outer(x):
        return jnp.concatenate([x[:, 0:128], x[:, 256:384]], axis=0).astype(bf16)

    def scores(q, k):
        s1 = _dot_nt(outer(q), outer(k))
        s2 = _dot_nt(q[:, 128:256].astype(bf16), halves(k[:, 128:256]))
        s = s1 + jnp.concatenate([s2, s2], axis=0)
        s = jnp.where(keep, s * scale, fill)
        e = jnp.exp(s - jnp.max(s, axis=1, keepdims=True))
        return e, _recip(jnp.sum(e, axis=1, keepdims=True))

    def values(e, r, v):
        o1 = _dot(e.astype(bf16), outer(v)) * r
        o2 = _dot((e[:L] + e[L:]).astype(bf16), halves(v[:, 128:256])) * jnp.where(lo_half, r[:L], r[L:])
        return jnp.concatenate([o1[:L], o2, o1[L:]], axis=1)

    def bstep(lhs, first):
        qkv, ps, os_ = {}, {}, {}
        acc = [None]
        nxt = [0]

        def QKV(t):
            r = _dot(lhs, _unpack(wb_ref[t]))
            if first:
                svq_ref[t] = r[L:L + 8]
                r = r[:L]
            else:
                r = jnp.concatenate([r[:MEM], svq_ref[t], r[MEM:]], axis=0)
            qkv[t] = r

        def SS(j):
            ps[j] = scores(qkv[j][:, :PW], qkv[j][:, PW:2 * PW])

        def PV(j):
            o = values(*ps[j], qkv[j][:, 2 * PW:])
            if first:
                svo_ref[j] = o[32:L]
                o = o[:32]
            else:
                o = jnp.concatenate([o, svo_ref[j]], axis=0)
            os_[j] = o.astype(bf16)

        def OO(n):
            for _ in range(n):
                j = nxt[0]
                c = _dot(os_[j], _unpack(wob_ref[j]))
                acc[0] = c if acc[0] is None else acc[0] + c
                nxt[0] += 1

        n1, n2, n3 = (2, 3, 2) if first else (2, 2, 1)
        nd = n1 + n2 + n3 + 1
        for t in range(NP):
            QKV(t)
            if t >= 1:
                SS(t - 1)
            if t >= 2:
                PV(t - 2)
            if 3 <= t < NP - 1 and nxt[0] < NP - nd:
                OO(1)
        OO(n1)
        SS(NP - 1)
        PV(NP - 2)
        OO(n2)
        PV(NP - 1)
        OO(n3 + 1)
        return acc[0]

    def bpass(store):
        mem_ref[...] = mem0_ref[...].astype(f32)

        def body(i, c):
            r0 = pl.multiple_of(i * 64, 64)
            xa = xnb_ref[pl.ds(r0, 64), :]
            ya = bstep(jnp.concatenate([mem_ref[...], xa[:L]], axis=0).astype(bf16), True)
            yb = bstep(jnp.concatenate([ya[:MEM], xa[L:]], axis=0).astype(bf16), False)
            mem_ref[...] = yb[:MEM]
            y = jnp.concatenate([ya[MEM:32], yb[L:L + 8], yb[MEM:L]], axis=0)
            store(r0, xres_ref[pl.ds(r0, 64), :] + y)
            return c
        lax.fori_loop(0, S // 64, body, 0)

    def store_res(r0, y):
        xres_ref[pl.ds(r0, 64), :] = y

    def store_out(r0, y):
        out_ref[pl.ds(r0, 64), :] = y.astype(bf16)

    load_in = lambda r0: x_ref[pl.ds(r0, TB), :].astype(f32)
    load_res = lambda r0: xres_ref[pl.ds(r0, TB), :]

    kside_pass(load_in, 4)
    build_kvw()
    for c in big:
        c.wait()
    qside_pass(load_in, 4, relayout_weights)
    bpass(store_res)
    kside_pass(load_res, 4)
    build_kvw()
    qside_pass(load_res, 4, None)
    bpass(store_out)


@functools.partial(jax.jit, static_argnames=("B_seg_len",))
def pallas_interleave_layers__linear_kernel_hedgehog__memory_aug_recurrent_mem_tr__prompt_kernel(
    A_x: jax.Array,
    A_wqkv: jax.Array,
    A_w_phi: jax.Array,
    A_wo: jax.Array,
    B_x: jax.Array,
    B_mem0: jax.Array,
    B_Wq: jax.Array,
    B_Wk: jax.Array,
    B_Wv: jax.Array,
    B_Wo: jax.Array,
    B_seg_len: int,
):
    del B_x
    assert B_seg_len == SEG
    assert A_x.shape == (1, S, D) and B_mem0.shape == (1, MEM, D)
    assert B_Wq.shape == (D, HB, DHB) and A_w_phi.shape == (HA, FA, FA)
    tr = lambda w: jnp.transpose(w, (1, 2, 0)).reshape(HB * DHB, D)
    vmem = pl.BlockSpec(memory_space=pltpu.VMEM)
    hbm = pl.BlockSpec(memory_space=pl.ANY)
    out = pl.pallas_call(
        _kernel,
        out_shape=jax.ShapeDtypeStruct((S, D), bf16),
        in_specs=[vmem] * 5 + [hbm] * 4,
        out_specs=vmem,
        scratch_shapes=[
            pltpu.VMEM((4, HB * DHB, D), bf16),
            pltpu.VMEM((NP, D // 2, 3 * PW), u32),
            pltpu.VMEM((NP, PW // 2, D), u32),
            pltpu.VMEM((S, D), f32),
            pltpu.VMEM((S // 2, D), u32),
            pltpu.VMEM((S, D), f32),
            pltpu.VMEM((D // 2, D), u32),
            pltpu.VMEM((NG, 4 * FA, D), u32),
            pltpu.VMEM((D // 2, D), u32),
            pltpu.VMEM((NG, 16 * FA, 256), f32),
            pltpu.VMEM((D, D), u32),
            pltpu.VMEM((8, 2 * D), f32),
            pltpu.VMEM((MEM, D), f32),
            pltpu.VMEM((NP, 8, 3 * PW), f32),
            pltpu.VMEM((NP, 8, PW), f32),
            pltpu.SemaphoreType.DMA((4,)),
        ],
        compiler_params=pltpu.CompilerParams(vmem_limit_bytes=120 * 1024 * 1024),
        name="hedgehog_rmt",
    )(A_x.reshape(S, D), A_wqkv, jnp.transpose(A_w_phi, (1, 2, 0)), A_wo, B_mem0.reshape(MEM, D),
      tr(B_Wq), tr(B_Wk), tr(B_Wv), B_Wo.reshape(HB * DHB, D))
    return out.reshape(1, S, D)
```

```python
import contextlib
import functools

import jax
import jax.numpy as jnp
from jax import lax
import jax.experimental.pallas as pl
import jax.experimental.pallas.tpu as pltpu

f32, bf16, u32 = jnp.float32, jnp.bfloat16, jnp.uint32

S, D = 2048, 640
HA, FA = 32, 20
HB, DHB = 32, 192
MEM, SEG = 8, 32
L = MEM + SEG
NP = HB // 2
PW = 2 * DHB
TB = 128
NG = 16
GR = 2 * FA
NCH = 4
NT = (((1,), (1,)), ((), ()))


_scope = lambda name: contextlib.nullcontext()


def _dot(a, b):
    return jnp.dot(a, b, preferred_element_type=f32)


def _dot_nt(a, b):
    return lax.dot_general(a, b, NT, preferred_element_type=f32)


def _pack(x):
    return pltpu.bitcast(x.astype(bf16), u32)


def _unpack(x):
    return pltpu.bitcast(x, bf16)


def _recip(x):
    r = pl.reciprocal(x, approx=True)
    return r * (2.0 - x * r)


def _layernorm(x):
    m = jnp.mean(x, axis=-1, keepdims=True)
    xc = x - m
    v = jnp.mean(xc * xc, axis=-1, keepdims=True)
    return xc * lax.rsqrt(v + 1e-5)


def _iota(shape, dim):
    return lax.broadcasted_iota(jnp.int32, shape, dim)


def _kernel(x_hbm, wqkv_hbm, wphi_hbm, woa_hbm, mem0_hbm, wqt_hbm, wkt_hbm, wvt_hbm, wob_hbm,
            out_hbm,
            x_ref, wqkv_ref, wphi_ref, woa_ref, mem0_ref, out_ref,
            stage_ref, wb_ref, wob_ref, xres_ref, xna_ref, xnb_ref,
            wpqt_ref, wpkt_ref, wv_ref, wo_ref, acc_ref, z_ref, kvt_ref, o_ref,
            mem_ref, prev_ref, svq_ref, svo_ref, sems):
    XC = S // NCH
    WC = HB * DHB // NCH

    def cp_wqkv(m):
        return pltpu.make_async_copy(wqkv_hbm.at[:, pl.ds(m * D, D)], wqkv_ref.at[m], sems.at[m])

    def cp_x(i):
        rows = pl.ds(pl.multiple_of(i * XC, XC), XC)
        return pltpu.make_async_copy(x_hbm.at[rows, :], x_ref.at[rows, :], sems.at[8 + i])

    def cp_w(m, i):
        rows = pl.ds(pl.multiple_of(i * WC, WC), WC)
        return pltpu.make_async_copy((wqt_hbm, wkt_hbm, wvt_hbm)[m].at[rows, :], stage_ref.at[m, rows, :],
                                     sems.at[8 + NCH * (m + 1) + i])

    cp_phi = pltpu.make_async_copy(wphi_hbm, wphi_ref, sems.at[3])
    cp_woa = pltpu.make_async_copy(woa_hbm, woa_ref, sems.at[4])
    cp_mem = pltpu.make_async_copy(mem0_hbm, mem0_ref, sems.at[5])
    cp_wob = pltpu.make_async_copy(wob_hbm, wob_ref, sems.at[6])
    cp_phi.start()
    cp_wqkv(1).start()
    cp_x(0).start()
    cp_wqkv(2).start()
    for i in range(1, NCH):
        cp_x(i).start()
    cp_wqkv(0).start()
    cp_woa.start()
    cp_mem.start()
    for i in range(NCH):
        for m in range(3):
            cp_w(m, i).start()
    cp_wob.start()

    def fold_phi(m, dst):
        wphi = wphi_ref[...].astype(f32)
        cat = jnp.concatenate([wphi[d] for d in range(FA)], axis=1)
        cat = jnp.concatenate([cat, jnp.zeros((32 - FA, D), f32)], axis=0).astype(bf16)
        p_row, p_col = _iota((D, D), 0), _iota((D, D), 1)
        spread = (FA * (p_row & 31) + (p_row >> 5) == p_col).astype(f32).astype(bf16)
        u = _dot(cat, spread).astype(bf16)
        dup = ((_iota((48, 32), 0) >> 1) == _iota((48, 32), 1)).astype(f32).astype(bf16)
        u2 = _dot(dup, u)[:GR]
        lane, par = _iota((GR, 128), 1), _iota((GR, 128), 0) & 1
        lhs = []
        for c in range(5):
            blocks = []
            for g in range(3 * c, 3 * c + 4):
                lo = GR * g - 128 * c + FA * par
                blocks.append(jnp.where((lane >= lo) & (lane < lo + FA), u2[:, 128 * c:128 * c + 128], 0.0))
            lhs.append(jnp.concatenate(blocks, axis=0).astype(bf16))
        cp_wqkv(m).wait()
        parts = [_dot_nt(lhs[c], wqkv_ref[m, :, 128 * c:128 * c + 128]) for c in range(5)]
        rows = []
        for c in range(5):
            first = parts[c][:GR] if c == 0 else parts[c][:GR] + parts[c - 1][3 * GR:]
            rows += [first, parts[c][GR:3 * GR]]
        rows.append(parts[4][3 * GR:])
        dst[...] = _pack(jnp.concatenate(rows, axis=0))

    def fold(x, op):
        r = op(op(op(x[:, 0], x[:, 1]), op(x[:, 2], x[:, 3])), x[:, 4])
        r = op(r, pltpu.roll(r, 2, 1))
        return op(r, pltpu.roll(r, 4, 1))

    def feature_map(pt):
        p = pt.reshape(-1, 5, 8, TB)
        ep = jnp.exp(p - fold(p, jnp.maximum)[:, None])
        en = jnp.exp(fold(p, jnp.minimum)[:, None] - p)
        ep = ep * _recip(fold(ep, jnp.add))[:, None]
        en = en * _recip(fold(en, jnp.add))[:, None]
        return jnp.concatenate([ep, en], axis=1)

    def half(r0):
        return pl.ds(pl.multiple_of(r0 // 2, TB // 2), TB // 2)

    CG = 4
    NC = NG // CG
    CR = CG * GR

    def kside_pass(load_x, nsub, pre=None):
        acc_ref[...] = jnp.zeros(acc_ref.shape, f32)
        z_ref[...] = jnp.zeros(z_ref.shape, f32)

        def body(i, c):
            xn, v, phi = {}, {}, {}
            if pre is not None:
                pre(i)

            def LN(j):
                r0 = pl.multiple_of((i * nsub + j) * TB, TB)
                if load_x is not None:
                    xn[j] = _layernorm(load_x(r0)).astype(bf16)
                    xna_ref[half(r0), :] = pltpu.bitcast(xn[j], u32)
                else:
                    xn[j] = _unpack(xna_ref[half(r0), :])

            def P(j, c):
                pk = _dot_nt(_unpack(wpkt_ref[c * CR // 2:(c + 1) * CR // 2, :]), xn[j])
                f = feature_map(pk).reshape(2 * CR, TB)
                z_ref[2 * CR * c:2 * CR * (c + 1), :] += f
                phi[j, c] = f

            def V(j, t):
                v[j, t] = _dot(xn[j], _unpack(wv_ref[:, 128 * t:128 * t + 128])).astype(bf16)

            def KV(j, t):
                f = jnp.concatenate([phi[j, c] for c in range(NC)], axis=0)
                acc_ref[t] += _dot(f[6 * GR * t:6 * GR * t + 8 * GR].astype(bf16), v[j, t])

            LN(0)
            for j in range(nsub):
                if j + 1 < nsub:
                    LN(j + 1)
                for c in range(NC):
                    P(j, c)
                for t in range(5):
                    V(j, t)
                for t in range(5):
                    KV(j, t)
            return c
        lax.fori_loop(0, S // (TB * nsub), body, 0)

    def finish_kv():
        z_ref[...] = jnp.broadcast_to(jnp.sum(z_ref[...], axis=1, keepdims=True), z_ref.shape)
        pad = jnp.zeros((128 - 2 * GR, 128), f32)
        tr = {}
        for t in range(5):
            for g in range(3 * t, 3 * t + 4):
                r = 2 * GR * (g - 3 * t)
                tr[t, g] = jnp.concatenate([acc_ref[t, r:r + 2 * GR, :], pad], axis=0).T
        same = (_iota((GR, 128), 0) >= FA) == ((_iota((GR, 128), 1) & 1) == 1)
        for g in range(NG):
            lo, hi = GR * g, GR * g + GR
            t0, t1 = lo // 128, (hi - 1) // 128
            if t0 == t1:
                blk = tr[t0, g][lo - 128 * t0:hi - 128 * t0]
            else:
                blk = jnp.concatenate([tr[t0, g][lo - 128 * t0:], tr[t1, g][:hi - 128 * t1]], axis=0)
            blk = jnp.where(same, blk, 0.0)
            kvt_ref[g] = _pack(jnp.concatenate([blk, jnp.zeros((8, 128), f32)], axis=0))

    def qside_pass(load_x, nsub, extra=None, pre=None):
        even = (_iota((CG, 8, TB), 1) & 1) == 0
        top = _iota((CG, 8, TB), 1) < 4

        def body(i, c):
            xn, phi, sc, ot, o, y = {}, {}, {}, {}, {}, {}
            if pre is not None:
                pre(i)

            def P(j, c):
                if c == 0:
                    xn[j] = _unpack(xna_ref[half(pl.multiple_of((i * nsub + j) * TB, TB)), :])
                pq = _dot_nt(_unpack(wpqt_ref[c * CR // 2:(c + 1) * CR // 2, :]), xn[j])
                f = feature_map(pq)
                pz = f * z_ref[2 * CR * c:2 * CR * (c + 1), :].reshape(CG, 10, 8, TB)
                rd = 1.0 / (fold(pz[:, :5] + pz[:, 5:], jnp.add) + 1e-6)
                rs = pltpu.roll(rd, 1, 1)
                r0_, r1_ = jnp.where(even, rd, rs), jnp.where(even, rs, rd)
                sc[j, c] = (r0_, jnp.where(top, r0_, r1_), r1_)
                phi[j, c] = f.reshape(2 * CR, TB)

            def N(j, c):
                r0_, rm, r1_ = sc[j, c]
                outs = []
                for g in range(CG):
                    num = _dot(_unpack(kvt_ref[CG * c + g])[:, :2 * GR], phi[j, c][2 * GR * g:2 * GR * (g + 1)].astype(bf16))[:GR]
                    outs.append(num * jnp.concatenate([r0_[g], r0_[g], rm[g], r1_[g], r1_[g]], axis=0))
                ot[j, c] = jnp.concatenate(outs, axis=0)

            def W(j, t):
                if t == 0:
                    o_ref[j] = pltpu.bitcast(jnp.concatenate([ot[j, c] for c in range(NC)], axis=0).astype(bf16).T, u32)
                    o[j] = _unpack(o_ref[j])
                y[j, t] = _dot(o[j], _unpack(wo_ref[:, 128 * t:128 * t + 128]))
                if t == 4:
                    r0 = pl.multiple_of((i * nsub + j) * TB, TB)
                    yy = load_x(r0) + jnp.concatenate([y[j, t] for t in range(5)], axis=1)
                    xres_ref[pl.ds(r0, TB), :] = yy
                    if extra is not None:
                        extra(i * nsub + j)

            for j in range(nsub + 1):
                if j < nsub:
                    for c in range(NC):
                        P(j, c)
                if j >= 1:
                    W(j - 1, 0), W(j - 1, 1)
                if j < nsub:
                    N(j, 0), N(j, 1)
                if j >= 1:
                    W(j - 1, 2), W(j - 1, 3), W(j - 1, 4)
                if j < nsub:
                    N(j, 2), N(j, 3)
            return c
        lax.fori_loop(0, S // (TB * nsub), body, 0)

    def relayout_weights(j):
        r0 = pl.multiple_of(j * PW, PW)
        for m in range(3):
            wb_ref[j, :, m * PW:(m + 1) * PW] = pltpu.bitcast(stage_ref[m, pl.ds(r0, PW), :].T, u32)

    scale = DHB ** -0.5
    row, col = _iota((2 * L, 2 * L), 0), _iota((2 * L, 2 * L), 1)
    same = (row < L) == (col < L)
    rr = jnp.where(row < L, row, row - L)
    kk = jnp.where(col < L, col, col - L)
    keep = same & ((rr < MEM) | (rr >= kk))
    fill = jnp.where(same, -1e9, -jnp.inf).astype(f32)
    lo_half = _iota((L, 128), 1) < 64

    def halves(mid):
        return jnp.concatenate([jnp.where(lo_half, mid, 0.0), jnp.where(lo_half, 0.0, mid)], axis=0).astype(bf16)

    def outer(x):
        return jnp.concatenate([x[:, 0:128], x[:, 256:384]], axis=0).astype(bf16)

    def scores(q, k):
        s1 = _dot_nt(outer(q), outer(k))
        s2 = _dot_nt(q[:, 128:256].astype(bf16), halves(k[:, 128:256]))
        s = s1 + jnp.concatenate([s2, s2], axis=0)
        s = jnp.where(keep, s * scale, fill)
        e = jnp.exp(s - jnp.max(s, axis=1, keepdims=True))
        return e, _recip(jnp.sum(e, axis=1, keepdims=True))

    def values(e, r, v):
        o1 = _dot(e.astype(bf16), outer(v)) * r
        o2 = _dot((e[:L] + e[L:]).astype(bf16), halves(v[:, 128:256])) * jnp.where(lo_half, r[:L], r[L:])
        return jnp.concatenate([o1[:L], o2, o1[L:]], axis=1)

    def bstep(lhs, first):
        qkv, ps, os_ = {}, {}, {}
        acc = [None]
        nxt = [0]

        def QKV(t):
            r = _dot(lhs, _unpack(wb_ref[t]))
            if first:
                svq_ref[t] = r[L:L + 8]
                r = r[:L]
            else:
                r = jnp.concatenate([r[:MEM], svq_ref[t], r[MEM:]], axis=0)
            qkv[t] = r

        def SS(j):
            ps[j] = scores(qkv[j][:, :PW], qkv[j][:, PW:2 * PW])

        def PV(j):
            o = values(*ps[j], qkv[j][:, 2 * PW:])
            if first:
                svo_ref[j] = o[32:L]
                o = o[:32]
            else:
                o = jnp.concatenate([o, svo_ref[j]], axis=0)
            os_[j] = o.astype(bf16)

        def OO(n):
            for _ in range(n):
                j = nxt[0]
                c = _dot(os_[j], wob_ref[j * PW:(j + 1) * PW, :])
                acc[0] = c if acc[0] is None else acc[0] + c
                nxt[0] += 1

        n1, n2, n3 = (2, 3, 2) if first else (2, 2, 1)
        nd = n1 + n2 + n3 + 1
        for t in range(NP):
            QKV(t)
            if t >= 1:
                SS(t - 1)
            if t >= 2:
                PV(t - 2)
            if 3 <= t < NP - 1 and nxt[0] < NP - nd:
                OO(1)
        OO(n1)
        SS(NP - 1)
        PV(NP - 2)
        OO(n2)
        PV(NP - 1)
        OO(n3 + 1)
        return acc[0]

    def bpass(last):
        mem_ref[...] = mem0_ref[...].astype(f32)
        xnb_ref[...] = _layernorm(xres_ref[0:64, :])

        def body(i, c):
            r0 = pl.multiple_of(i * 64, 64)
            xa = xnb_ref[...]
            rn = pl.multiple_of(jnp.minimum(r0 + 64, S - 64), 64)
            xnext = _layernorm(xres_ref[pl.ds(rn, 64), :])
            ya = bstep(jnp.concatenate([mem_ref[...], xa[:L]], axis=0).astype(bf16), True)
            yb = bstep(jnp.concatenate([ya[:MEM], xa[L:]], axis=0).astype(bf16), False)
            mem_ref[...] = yb[:MEM]
            xnb_ref[...] = xnext
            y = xres_ref[pl.ds(r0, 64), :] + jnp.concatenate([ya[MEM:32], yb[L:L + 8], yb[MEM:L]], axis=0)
            if last:
                out_ref[pl.ds(r0, 64), :] = y.astype(bf16)
                pltpu.make_async_copy(out_ref.at[pl.ds(r0, 64), :], out_hbm.at[pl.ds(r0, 64), :], sems.at[7]).start()
            else:
                xres_ref[pl.ds(r0, 64), :] = y
                rp = pl.multiple_of(jnp.maximum(r0 - 64, 0), 64)
                xna_ref[pl.ds(pl.multiple_of(rp // 2, 32), 32), :] = _pack(_layernorm(prev_ref[...]))
                prev_ref[...] = y
            return c
        if not last:
            prev_ref[...] = jnp.zeros(prev_ref.shape, f32)
        lax.fori_loop(0, S // 64, body, 0)
        if not last:
            xna_ref[(S - 64) // 2:, :] = _pack(_layernorm(prev_ref[...]))

    load_in = lambda r0: x_ref[pl.ds(r0, TB), :].astype(f32)
    load_res = lambda r0: xres_ref[pl.ds(r0, TB), :]

    def wait_w(i):
        for m in range(3):
            cp_w(m, i).wait()

    with _scope("pro"):
        cp_phi.wait()
        fold_phi(1, wpkt_ref)
        cp_wqkv(2).wait()
        wv_ref[...] = pltpu.bitcast(wqkv_ref[2], u32)
    with _scope("k1"):
        kside_pass(load_in, S // (TB * NCH), pre=lambda i: cp_x(i).wait())
    with _scope("f1"):
        cp_woa.wait()
        cp_mem.wait()
        fold_phi(0, wpqt_ref)
        wo_ref[...] = pltpu.bitcast(woa_ref[...], u32)
        finish_kv()
    with _scope("q1"):
        qside_pass(load_in, S // (TB * NCH), relayout_weights, wait_w)
    with _scope("wait"):
        cp_wob.wait()
    with _scope("b1"):
        bpass(False)
    with _scope("k2"):
        kside_pass(None, 8)
    with _scope("f2"):
        finish_kv()
    with _scope("q2"):
        qside_pass(load_res, 8)
    with _scope("b2"):
        bpass(True)
    pltpu.make_async_copy(out_ref, out_hbm, sems.at[7]).wait()


@functools.partial(jax.jit, static_argnames=("B_seg_len",))
def pallas_interleave_layers__linear_kernel_hedgehog__memory_aug_recurrent_mem_tr__prompt_kernel(
    A_x: jax.Array,
    A_wqkv: jax.Array,
    A_w_phi: jax.Array,
    A_wo: jax.Array,
    B_x: jax.Array,
    B_mem0: jax.Array,
    B_Wq: jax.Array,
    B_Wk: jax.Array,
    B_Wv: jax.Array,
    B_Wo: jax.Array,
    B_seg_len: int,
):
    del B_x
    assert B_seg_len == SEG
    assert A_x.shape == (1, S, D) and B_mem0.shape == (1, MEM, D)
    assert B_Wq.shape == (D, HB, DHB) and A_w_phi.shape == (HA, FA, FA)
    tr = lambda w: jnp.transpose(w, (1, 2, 0)).reshape(HB * DHB, D)
    hbm = pl.BlockSpec(memory_space=pl.ANY)
    out = pl.pallas_call(
        _kernel,
        out_shape=jax.ShapeDtypeStruct((S, D), bf16),
        in_specs=[hbm] * 9,
        out_specs=hbm,
        scratch_shapes=[
            pltpu.VMEM((S, D), bf16),
            pltpu.VMEM((3, D, D), bf16),
            pltpu.VMEM((FA, FA, HA), bf16),
            pltpu.VMEM((D, D), bf16),
            pltpu.VMEM((MEM, D), bf16),
            pltpu.VMEM((S, D), bf16),
            pltpu.VMEM((3, HB * DHB, D), bf16),
            pltpu.VMEM((NP, D // 2, 3 * PW), u32),
            pltpu.VMEM((HB * DHB, D), bf16),
            pltpu.VMEM((S, D), f32),
            pltpu.VMEM((S // 2, D), u32),
            pltpu.VMEM((64, D), f32),
            pltpu.VMEM((D // 2, D), u32),
            pltpu.VMEM((D // 2, D), u32),
            pltpu.VMEM((D // 2, D), u32),
            pltpu.VMEM((D // 2, D), u32),
            pltpu.VMEM((5, 8 * GR, 128), f32),
            pltpu.VMEM((2 * D, TB), f32),
            pltpu.VMEM((NG, 24, 128), u32),
            pltpu.VMEM((8, TB // 2, D), u32),
            pltpu.VMEM((MEM, D), f32),
            pltpu.VMEM((64, D), f32),
            pltpu.VMEM((NP, 8, 3 * PW), f32),
            pltpu.VMEM((NP, 8, PW), f32),
            pltpu.SemaphoreType.DMA((8 + 4 * NCH,)),
        ],
        compiler_params=pltpu.CompilerParams(vmem_limit_bytes=120 * 1024 * 1024),
        name="hedgehog_rmt",
    )(A_x.reshape(S, D), A_wqkv, jnp.transpose(A_w_phi, (1, 2, 0)), A_wo, B_mem0.reshape(MEM, D),
      tr(B_Wq), tr(B_Wk), tr(B_Wv), B_Wo.reshape(HB * DHB, D))
    return out.reshape(1, S, D)
```

```python
import contextlib
import functools

import jax
import jax.numpy as jnp
from jax import lax
import jax.experimental.pallas as pl
import jax.experimental.pallas.tpu as pltpu

f32, bf16, u32 = jnp.float32, jnp.bfloat16, jnp.uint32

S, D = 2048, 640
HA, FA = 32, 20
HB, DHB = 32, 192
MEM, SEG = 8, 32
L = MEM + SEG
NP = HB // 2
PW = 2 * DHB
TB = 128
NG = 16
GR = 2 * FA
NCH = 4
NT = (((1,), (1,)), ((), ()))
LOG2E = 1.4426950408889634


_scope = lambda name: contextlib.nullcontext()


def _dot(a, b):
    return jnp.dot(a, b, preferred_element_type=f32)


def _dot_nt(a, b):
    return lax.dot_general(a, b, NT, preferred_element_type=f32)


def _pack(x):
    return pltpu.bitcast(x.astype(bf16), u32)


def _unpack(x):
    return pltpu.bitcast(x, bf16)


def _recip(x):
    r = pl.reciprocal(x, approx=True)
    return r * (2.0 - x * r)


def _layernorm(x):
    m = jnp.mean(x, axis=-1, keepdims=True)
    xc = x - m
    v = jnp.mean(xc * xc, axis=-1, keepdims=True)
    return xc * lax.rsqrt(v + 1e-5)


def _iota(shape, dim):
    return lax.broadcasted_iota(jnp.int32, shape, dim)


def _kernel(x_hbm, wqkv_hbm, wphi_hbm, woa_hbm, mem0_hbm, wqt_hbm, wkt_hbm, wvt_hbm, wob_hbm,
            out_hbm,
            x_ref, wqkv_ref, wphi_ref, woa_ref, mem0_ref, out_ref,
            stage_ref, wb_ref, wob_ref, xres_ref, xna_ref, xnb_ref,
            wpqt_ref, wpkt_ref, wv_ref, wo_ref, acc_ref, z_ref, kvt_ref, o_ref,
            mem_ref, prev_ref, svq_ref, svo_ref, sems):
    XC = S // NCH
    WC = HB * DHB // NCH

    def cp_wqkv(m):
        return pltpu.make_async_copy(wqkv_hbm.at[:, pl.ds(m * D, D)], wqkv_ref.at[m], sems.at[m])

    def cp_x(i):
        rows = pl.ds(pl.multiple_of(i * XC, XC), XC)
        return pltpu.make_async_copy(x_hbm.at[rows, :], x_ref.at[rows, :], sems.at[8 + i])

    def cp_w(m, i):
        rows = pl.ds(pl.multiple_of(i * WC, WC), WC)
        return pltpu.make_async_copy((wqt_hbm, wkt_hbm, wvt_hbm)[m].at[rows, :], stage_ref.at[m, rows, :],
                                     sems.at[8 + NCH * (m + 1) + i])

    cp_phi = pltpu.make_async_copy(wphi_hbm, wphi_ref, sems.at[3])
    cp_woa = pltpu.make_async_copy(woa_hbm, woa_ref, sems.at[4])
    cp_mem = pltpu.make_async_copy(mem0_hbm, mem0_ref, sems.at[5])
    HW = HB * DHB // 2

    def cp_wo(i):
        rows = pl.ds(pl.multiple_of(i * (HW // NCH), HW // NCH), HW // NCH)
        return pltpu.make_async_copy(wob_hbm.at[rows, :], stage_ref.at[3, rows, :], sems.at[8 + 4 * NCH + i])

    cp_wob = pltpu.make_async_copy(wob_hbm.at[pl.ds(HW, HW), :], stage_ref.at[3, pl.ds(HW, HW), :], sems.at[6])
    cp_phi.start()
    cp_wqkv(1).start()
    cp_x(0).start()
    cp_wqkv(2).start()
    for i in range(1, NCH):
        cp_x(i).start()
    cp_wqkv(0).start()
    cp_woa.start()
    cp_mem.start()
    for i in range(NCH):
        for m in range(3):
            cp_w(m, i).start()
        cp_wo(i).start()
    cp_wob.start()

    def fold_phi(m, dst):
        wphi = wphi_ref[...].astype(f32)
        cat = jnp.concatenate([wphi[d] for d in range(FA)], axis=1)
        cat = jnp.concatenate([cat, jnp.zeros((32 - FA, D), f32)], axis=0).astype(bf16)
        p_row, p_col = _iota((D, D), 0), _iota((D, D), 1)
        spread = (FA * (p_row & 31) + (p_row >> 5) == p_col).astype(f32).astype(bf16)
        u = _dot(cat, spread).astype(bf16)
        dup = ((_iota((48, 32), 0) >> 1) == _iota((48, 32), 1)).astype(f32).astype(bf16)
        u2 = _dot(dup, u)[:GR]
        lane, par = _iota((GR, 128), 1), _iota((GR, 128), 0) & 1
        lhs = []
        for c in range(5):
            blocks = []
            for g in range(3 * c, 3 * c + 4):
                lo = GR * g - 128 * c + FA * par
                blocks.append(jnp.where((lane >= lo) & (lane < lo + FA), u2[:, 128 * c:128 * c + 128], 0.0))
            lhs.append(jnp.concatenate(blocks, axis=0).astype(bf16))
        cp_wqkv(m).wait()
        parts = [_dot_nt(lhs[c], wqkv_ref[m, :, 128 * c:128 * c + 128]) for c in range(5)]
        rows = []
        for c in range(5):
            first = parts[c][:GR] if c == 0 else parts[c][:GR] + parts[c - 1][3 * GR:]
            rows += [first, parts[c][GR:3 * GR]]
        rows.append(parts[4][3 * GR:])
        dst[...] = _pack(jnp.concatenate(rows, axis=0))

    def fold(x, op):
        r = op(op(op(x[:, 0], x[:, 1]), op(x[:, 2], x[:, 3])), x[:, 4])
        r = op(r, pltpu.roll(r, 2, 1))
        return op(r, pltpu.roll(r, 4, 1))

    def feature_map(pt):
        p = pt.reshape(-1, 5, 8, TB)
        ep = jnp.exp(p - fold(p, jnp.maximum)[:, None])
        en = jnp.exp(fold(p, jnp.minimum)[:, None] - p)
        ep = ep * _recip(fold(ep, jnp.add))[:, None]
        en = en * _recip(fold(en, jnp.add))[:, None]
        return jnp.concatenate([ep, en], axis=1)

    def half(r0):
        return pl.ds(pl.multiple_of(r0 // 2, TB // 2), TB // 2)

    CG = 4
    NC = NG // CG
    CR = CG * GR

    def kside_pass(load_x, nsub, pre=None):
        acc_ref[...] = jnp.zeros(acc_ref.shape, f32)
        z_ref[...] = jnp.zeros(z_ref.shape, f32)

        def body(i, c):
            xn, v, phi = {}, {}, {}
            if pre is not None:
                pre(i)

            def LN(j):
                r0 = pl.multiple_of((i * nsub + j) * TB, TB)
                if load_x is not None:
                    xn[j] = _layernorm(load_x(r0)).astype(bf16)
                    xna_ref[half(r0), :] = pltpu.bitcast(xn[j], u32)
                else:
                    xn[j] = _unpack(xna_ref[half(r0), :])

            def P(j, c):
                pk = _dot_nt(_unpack(wpkt_ref[c * CR // 2:(c + 1) * CR // 2, :]), xn[j])
                f = feature_map(pk).reshape(2 * CR, TB)
                z_ref[2 * CR * c:2 * CR * (c + 1), :] += f
                phi[j, c] = f

            def V(j, t):
                v[j, t] = _dot(xn[j], _unpack(wv_ref[:, 128 * t:128 * t + 128])).astype(bf16)

            def KV(j, t):
                f = jnp.concatenate([phi[j, c] for c in range(NC)], axis=0)
                acc_ref[t] += _dot(f[6 * GR * t:6 * GR * t + 8 * GR].astype(bf16), v[j, t])

            LN(0)
            for j in range(nsub):
                if j + 1 < nsub:
                    LN(j + 1)
                for c in range(NC):
                    P(j, c)
                for t in range(5):
                    V(j, t)
                for t in range(5):
                    KV(j, t)
            return c
        lax.fori_loop(0, S // (TB * nsub), body, 0)

    def finish_kv():
        z_ref[...] = jnp.broadcast_to(jnp.sum(z_ref[...], axis=1, keepdims=True), z_ref.shape)
        pad = jnp.zeros((128 - 2 * GR, 128), f32)
        tr = {}
        for t in range(5):
            for g in range(3 * t, 3 * t + 4):
                r = 2 * GR * (g - 3 * t)
                tr[t, g] = jnp.concatenate([acc_ref[t, r:r + 2 * GR, :], pad], axis=0).T
        same = (_iota((GR, 128), 0) >= FA) == ((_iota((GR, 128), 1) & 1) == 1)
        for g in range(NG):
            lo, hi = GR * g, GR * g + GR
            t0, t1 = lo // 128, (hi - 1) // 128
            if t0 == t1:
                blk = tr[t0, g][lo - 128 * t0:hi - 128 * t0]
            else:
                blk = jnp.concatenate([tr[t0, g][lo - 128 * t0:], tr[t1, g][:hi - 128 * t1]], axis=0)
            blk = jnp.where(same, blk, 0.0)
            kvt_ref[g] = _pack(jnp.concatenate([blk, jnp.zeros((8, 128), f32)], axis=0))

    def qside_pass(load_x, nsub, extra=None, pre=None):
        even = (_iota((CG, 8, TB), 1) & 1) == 0
        top = _iota((CG, 8, TB), 1) < 4

        def body(i, c):
            xn, phi, sc, ot, o, y = {}, {}, {}, {}, {}, {}
            if pre is not None:
                pre(i)

            def P(j, c):
                if c == 0:
                    xn[j] = _unpack(xna_ref[half(pl.multiple_of((i * nsub + j) * TB, TB)), :])
                pq = _dot_nt(_unpack(wpqt_ref[c * CR // 2:(c + 1) * CR // 2, :]), xn[j])
                f = feature_map(pq)
                pz = f * z_ref[2 * CR * c:2 * CR * (c + 1), :].reshape(CG, 10, 8, TB)
                rd = 1.0 / (fold(pz[:, :5] + pz[:, 5:], jnp.add) + 1e-6)
                rs = pltpu.roll(rd, 1, 1)
                r0_, r1_ = jnp.where(even, rd, rs), jnp.where(even, rs, rd)
                sc[j, c] = (r0_, jnp.where(top, r0_, r1_), r1_)
                phi[j, c] = f.reshape(2 * CR, TB)

            def N(j, c):
                r0_, rm, r1_ = sc[j, c]
                outs = []
                for g in range(CG):
                    num = _dot(_unpack(kvt_ref[CG * c + g])[:, :2 * GR], phi[j, c][2 * GR * g:2 * GR * (g + 1)].astype(bf16))[:GR]
                    outs.append(num * jnp.concatenate([r0_[g], r0_[g], rm[g], r1_[g], r1_[g]], axis=0))
                ot[j, c] = jnp.concatenate(outs, axis=0)

            def W(j, t):
                if t == 0:
                    o_ref[j] = pltpu.bitcast(jnp.concatenate([ot[j, c] for c in range(NC)], axis=0).astype(bf16).T, u32)
                    o[j] = _unpack(o_ref[j])
                y[j, t] = _dot(o[j], _unpack(wo_ref[:, 128 * t:128 * t + 128]))
                if t == 4:
                    r0 = pl.multiple_of((i * nsub + j) * TB, TB)
                    yy = load_x(r0) + jnp.concatenate([y[j, t] for t in range(5)], axis=1)
                    xres_ref[pl.ds(r0, TB), :] = yy
                    if extra is not None:
                        extra(i, j)

            for j in range(nsub + 1):
                if j < nsub:
                    for c in range(NC):
                        P(j, c)
                if j >= 1:
                    W(j - 1, 0), W(j - 1, 1)
                if j < nsub:
                    N(j, 0), N(j, 1)
                if j >= 1:
                    W(j - 1, 2), W(j - 1, 3), W(j - 1, 4)
                if j < nsub:
                    N(j, 2), N(j, 3)
            return c
        lax.fori_loop(0, S // (TB * nsub), body, 0)

    VPERM = [(h * DHB + 64 * c) for c in range(3) for h in range(2)]

    def retile_wo(j, parts):
        for c in parts:
            src = pl.ds(pl.multiple_of(j * PW + VPERM[c], 64), 64)
            wob_ref[j, 32 * c:32 * c + 32, :] = pltpu.bitcast(stage_ref[3, src, :], u32)

    def relayout_weights(i, jj):
        j = i * (NP // NCH) + jj
        retile_wo(i * 2 + jj // 2, range(3 * (jj % 2), 3 * (jj % 2) + 3))
        r0 = pl.multiple_of(j * PW, PW)
        for m in range(2):
            wb_ref[j, :, m * PW:(m + 1) * PW] = pltpu.bitcast(stage_ref[m, pl.ds(r0, PW), :].T, u32)
        for c in range(3):
            w = jnp.concatenate([stage_ref[2, pl.ds(pl.multiple_of(r0 + o, 64), 64), :] for o in VPERM[2 * c:2 * c + 2]], axis=0)
            wb_ref[j, :, 2 * PW + 128 * c:2 * PW + 128 * (c + 1)] = pltpu.bitcast(w.T, u32)

    scale = DHB ** -0.5
    NQ = 32
    row, col = _iota((2 * NQ, 2 * L), 0), _iota((2 * NQ, 2 * L), 1)
    same = (row < NQ) == (col < L)
    rr = jnp.where(row < NQ, row, row - NQ)
    kk = jnp.where(col < L, col, col - L)
    keep = same & ((rr < MEM) | (rr + 8 >= kk))
    fill = jnp.where(same, -1e9, -jnp.inf).astype(f32)
    lo = lambda n, w=128: (_iota((n, w), 1) & 64) == 0
    sub8 = _iota((8, 128), 0)

    def halves(x):
        m = lo(*x.shape)
        return jnp.concatenate([jnp.where(m, x, 0.0), jnp.where(m, 0.0, x)], axis=0).astype(bf16)

    def outer(x):
        return jnp.concatenate([x[:, 0:128], x[:, 256:384]], axis=0).astype(bf16)

    def scores(q, k):
        s1 = _dot_nt(outer(q), outer(k))
        s2 = _dot_nt(q[:, 128:256].astype(bf16), halves(k[:, 128:256]))
        s = s1 + jnp.concatenate([s2, s2], axis=0)
        s = jnp.where(keep, s * scale, fill)
        e = jnp.exp(s - jnp.max(s, axis=1, keepdims=True))
        return e, _recip(jnp.sum(e, axis=1, keepdims=True))

    def values(e, r, v):
        rab = jnp.where(lo(NQ), r[:NQ], r[NQ:])
        return _dot((e[:NQ] + e[NQ:]).astype(bf16), halves(v)) * jnp.concatenate([rab] * 3, axis=1)

    def head_attention(q, kv):
        q = q * (scale * LOG2E)
        q0, q2 = q[:, 0:128], q[:, 256:384]
        ql, qh = jnp.where(lo(8), q[:, 128:256], 0.0), jnp.where(lo(8), 0.0, q[:, 128:256])

        def bc(k, c):
            x = kv[8 * (k // 8):8 * (k // 8) + 8, 128 * c:128 * c + 128]
            return pltpu.roll(x, k % 8, 0) if k % 8 else x

        ss = []
        for k in range(16):
            k1 = bc(k, 1)
            a = jnp.sum(q0 * bc(k, 0) + ql * k1, axis=1, keepdims=True)
            b = jnp.sum(q2 * bc(k, 2) + qh * k1, axis=1, keepdims=True)
            x = jnp.where(lo(8), a, b)
            if k > MEM:
                x = jnp.where(sub8 >= k - MEM, x, -1e9 * LOG2E)
            ss.append(x)
        m = ss
        while len(m) > 1:
            m = [jnp.maximum(m[i], m[i + 1]) for i in range(0, len(m), 2)]
        acc = None
        for k in range(16):
            e = jnp.exp2(ss[k] - m[0])
            t = [e] + [e * bc(k, 3 + c) for c in range(3)]
            acc = t if acc is None else [u + w for u, w in zip(acc, t)]
        r = _recip(acc[0])
        return jnp.concatenate([acc[1] * r, acc[2] * r, acc[3] * r], axis=1)

    def bstep(lhs, first):
        qkv, ps, os_, ov = {}, {}, {}, {}
        acc = [None]
        nxt = [0]

        def QKV(t):
            r = _dot(lhs, _unpack(wb_ref[t]))
            if first:
                svq_ref[t] = r[L:L + 8]
                r = r[:L]
            else:
                r = jnp.concatenate([r[:MEM], svq_ref[t], r[MEM:]], axis=0)
            qkv[t] = r
            ov[t] = head_attention(r[8:16, :PW], r[:16, PW:])

        def SS(j):
            q = jnp.concatenate([qkv[j][:MEM, :PW], qkv[j][16:, :PW]], axis=0)
            ps[j] = scores(q, qkv[j][:, PW:2 * PW])

        def PV(j):
            o = values(*ps[j], qkv[j][:, 2 * PW:])
            if first:
                svo_ref[j] = o[24:32]
                o = jnp.concatenate([o[:24], ov[j]], axis=0)
            else:
                o = jnp.concatenate([o, ov[j], svo_ref[j]], axis=0)
            os_[j] = o.astype(bf16)

        def OO(n):
            for _ in range(n):
                j = nxt[0]
                c = _dot(os_[j], _unpack(wob_ref[j]))
                acc[0] = c if acc[0] is None else acc[0] + c
                nxt[0] += 1

        n1, n2, n3 = (2, 3, 2) if first else (2, 2, 1)
        nd = n1 + n2 + n3 + 1
        for t in range(NP):
            for op in ("QSOP" if first else "QOPS"):
                if op == "Q":
                    QKV(t)
                if op == "S" and t >= 1:
                    SS(t - 1)
                if op == "P" and t >= 2:
                    PV(t - 2)
                if op == "O" and 3 <= t < NP - 1 and nxt[0] < NP - nd:
                    OO(1)
        OO(n1)
        SS(NP - 1)
        PV(NP - 2)
        OO(n2)
        PV(NP - 1)
        OO(n3 + 1)
        return acc[0]

    def bpass(last):
        mem_ref[...] = mem0_ref[...].astype(f32)
        xnb_ref[...] = _layernorm(xres_ref[0:64, :])

        def body(i, c):
            r0 = pl.multiple_of(i * 64, 64)
            xa = xnb_ref[...]
            rn = pl.multiple_of(jnp.minimum(r0 + 64, S - 64), 64)
            xnext = _layernorm(xres_ref[pl.ds(rn, 64), :])
            ya = bstep(jnp.concatenate([mem_ref[...], xa[:L]], axis=0).astype(bf16), True)
            yb = bstep(jnp.concatenate([ya[:MEM], xa[L:]], axis=0).astype(bf16), False)
            mem_ref[...] = yb[:MEM]
            xnb_ref[...] = xnext
            y = xres_ref[pl.ds(r0, 64), :] + jnp.concatenate([ya[24:32], ya[MEM:24], yb[40:48], yb[32:40], yb[MEM:32]], axis=0)
            if last:
                out_ref[pl.ds(r0, 64), :] = y.astype(bf16)
                pltpu.make_async_copy(out_ref.at[pl.ds(r0, 64), :], out_hbm.at[pl.ds(r0, 64), :], sems.at[7]).start()
            else:
                xres_ref[pl.ds(r0, 64), :] = y
                rp = pl.multiple_of(jnp.maximum(r0 - 64, 0), 64)
                xna_ref[pl.ds(pl.multiple_of(rp // 2, 32), 32), :] = _pack(_layernorm(prev_ref[...]))
                prev_ref[...] = y
            return c
        if not last:
            prev_ref[...] = jnp.zeros(prev_ref.shape, f32)
        lax.fori_loop(0, S // 64, body, 0)
        if not last:
            xna_ref[(S - 64) // 2:, :] = _pack(_layernorm(prev_ref[...]))

    load_in = lambda r0: x_ref[pl.ds(r0, TB), :].astype(f32)
    load_res = lambda r0: xres_ref[pl.ds(r0, TB), :]

    def wait_w(i):
        for m in range(3):
            cp_w(m, i).wait()
        cp_wo(i).wait()

    with _scope("pro"):
        cp_phi.wait()
        fold_phi(1, wpkt_ref)
        cp_wqkv(2).wait()
        wv_ref[...] = pltpu.bitcast(wqkv_ref[2], u32)
    with _scope("k1"):
        kside_pass(load_in, S // (TB * NCH), pre=lambda i: cp_x(i).wait())
    with _scope("f1"):
        cp_woa.wait()
        cp_mem.wait()
        fold_phi(0, wpqt_ref)
        wo_ref[...] = pltpu.bitcast(woa_ref[...], u32)
        finish_kv()
    with _scope("q1"):
        qside_pass(load_in, S // (TB * NCH), relayout_weights, wait_w)
    with _scope("wait"):
        cp_wob.wait()
        for j in range(NP // 2, NP):
            retile_wo(j, range(6))
    with _scope("b1"):
        bpass(False)
    with _scope("k2"):
        kside_pass(None, 8)
    with _scope("f2"):
        finish_kv()
    with _scope("q2"):
        qside_pass(load_res, 8)
    with _scope("b2"):
        bpass(True)
    pltpu.make_async_copy(out_ref, out_hbm, sems.at[7]).wait()


@functools.partial(jax.jit, static_argnames=("B_seg_len",))
def pallas_interleave_layers__linear_kernel_hedgehog__memory_aug_recurrent_mem_tr__prompt_kernel(
    A_x: jax.Array,
    A_wqkv: jax.Array,
    A_w_phi: jax.Array,
    A_wo: jax.Array,
    B_x: jax.Array,
    B_mem0: jax.Array,
    B_Wq: jax.Array,
    B_Wk: jax.Array,
    B_Wv: jax.Array,
    B_Wo: jax.Array,
    B_seg_len: int,
):
    del B_x
    assert B_seg_len == SEG
    assert A_x.shape == (1, S, D) and B_mem0.shape == (1, MEM, D)
    assert B_Wq.shape == (D, HB, DHB) and A_w_phi.shape == (HA, FA, FA)
    tr = lambda w: jnp.transpose(w, (1, 2, 0)).reshape(HB * DHB, D)
    hbm = pl.BlockSpec(memory_space=pl.ANY)
    out = pl.pallas_call(
        _kernel,
        out_shape=jax.ShapeDtypeStruct((S, D), bf16),
        in_specs=[hbm] * 9,
        out_specs=hbm,
        scratch_shapes=[
            pltpu.VMEM((S, D), bf16),
            pltpu.VMEM((3, D, D), bf16),
            pltpu.VMEM((FA, FA, HA), bf16),
            pltpu.VMEM((D, D), bf16),
            pltpu.VMEM((MEM, D), bf16),
            pltpu.VMEM((S, D), bf16),
            pltpu.VMEM((4, HB * DHB, D), bf16),
            pltpu.VMEM((NP, D // 2, 3 * PW), u32),
            pltpu.VMEM((NP, PW // 2, D), u32),
            pltpu.VMEM((S, D), f32),
            pltpu.VMEM((S // 2, D), u32),
            pltpu.VMEM((64, D), f32),
            pltpu.VMEM((D // 2, D), u32),
            pltpu.VMEM((D // 2, D), u32),
            pltpu.VMEM((D // 2, D), u32),
            pltpu.VMEM((D // 2, D), u32),
            pltpu.VMEM((5, 8 * GR, 128), f32),
            pltpu.VMEM((2 * D, TB), f32),
            pltpu.VMEM((NG, 24, 128), u32),
            pltpu.VMEM((8, TB // 2, D), u32),
            pltpu.VMEM((MEM, D), f32),
            pltpu.VMEM((64, D), f32),
            pltpu.VMEM((NP, 8, 3 * PW), f32),
            pltpu.VMEM((NP, 8, PW), f32),
            pltpu.SemaphoreType.DMA((8 + 5 * NCH,)),
        ],
        compiler_params=pltpu.CompilerParams(vmem_limit_bytes=120 * 1024 * 1024),
        name="hedgehog_rmt",
    )(A_x.reshape(S, D), A_wqkv, jnp.transpose(A_w_phi, (1, 2, 0)), A_wo, B_mem0.reshape(MEM, D),
      tr(B_Wq), tr(B_Wk), tr(B_Wv), B_Wo.reshape(HB * DHB, D))
    return out.reshape(1, S, D)
```

```python
import contextlib
import functools

import jax
import jax.numpy as jnp
from jax import lax
import jax.experimental.pallas as pl
import jax.experimental.pallas.tpu as pltpu

f32, bf16, u32 = jnp.float32, jnp.bfloat16, jnp.uint32

S, D = 2048, 640
HA, FA = 32, 20
HB, DHB = 32, 192
MEM, SEG = 8, 32
L = MEM + SEG
NP = HB // 2
PW = 2 * DHB
TB = 128
NG = 16
GR = 2 * FA
NCH = 4
NT = (((1,), (1,)), ((), ()))
LOG2E = 1.4426950408889634
import os
_E = lambda k, d: type(d)(os.environ.get(k, d))
LN_AT = _E('LN_AT', 0)
LN_AT2 = _E('LN_AT2', 4)
NPR = _E('NPR', 1)
LEAD = _E('LEAD', 1)
KSPLIT = _E('KSPLIT', 8)
UNR = _E('UNR', 2)
A2MODE = _E('A2MODE', 1)


_scope = lambda name: contextlib.nullcontext()


def _dot(a, b):
    return jnp.dot(a, b, preferred_element_type=f32)


def _dot_nt(a, b):
    return lax.dot_general(a, b, NT, preferred_element_type=f32)


def _pack(x):
    return pltpu.bitcast(x.astype(bf16), u32)


def _unpack(x):
    return pltpu.bitcast(x, bf16)


def _recip(x):
    r = pl.reciprocal(x, approx=True)
    return r * (2.0 - x * r)


def _layernorm(x):
    m = jnp.mean(x, axis=-1, keepdims=True)
    xc = x - m
    v = jnp.mean(xc * xc, axis=-1, keepdims=True)
    return xc * lax.rsqrt(v + 1e-5)


def _iota(shape, dim):
    return lax.broadcasted_iota(jnp.int32, shape, dim)


def _kernel(x_hbm, wqkv_hbm, wphi_hbm, woa_hbm, mem0_hbm, wqt_hbm, wkt_hbm, wvt_hbm, wob_hbm,
            out_hbm,
            x_ref, wqkv_ref, wphi_ref, woa_ref, mem0_ref, out_ref,
            stage_ref, wb_ref, wob_ref, xres_ref, xna_ref, xnb_ref,
            wpqt_ref, wpkt_ref, wv_ref, wo_ref, acc_ref, z_ref, kvt_ref, o_ref,
            mem_ref, svq_ref, svo_ref, flag_ref, cnt_ref, sems):
    XC = S // NCH
    WC = HB * DHB // NCH

    def cp_wqkv(m):
        return pltpu.make_async_copy(wqkv_hbm.at[:, pl.ds(m * D, D)], wqkv_ref.at[m], sems.at[m])

    def cp_x(i):
        rows = pl.ds(pl.multiple_of(i * XC, XC), XC)
        return pltpu.make_async_copy(x_hbm.at[rows, :], x_ref.at[rows, :], sems.at[8 + i])

    def cp_w(m, i):
        rows = pl.ds(pl.multiple_of(i * WC, WC), WC)
        return pltpu.make_async_copy((wqt_hbm, wkt_hbm, wvt_hbm)[m].at[rows, :], stage_ref.at[m, rows, :],
                                     sems.at[8 + NCH * (m + 1) + i])

    cp_phi = pltpu.make_async_copy(wphi_hbm, wphi_ref, sems.at[3])
    cp_woa = pltpu.make_async_copy(woa_hbm, woa_ref, sems.at[4])
    cp_mem = pltpu.make_async_copy(mem0_hbm, mem0_ref, sems.at[5])
    HW = HB * DHB // 2

    def cp_wo(i):
        rows = pl.ds(pl.multiple_of(i * (HW // NCH), HW // NCH), HW // NCH)
        return pltpu.make_async_copy(wob_hbm.at[rows, :], stage_ref.at[3, rows, :], sems.at[8 + 4 * NCH + i])

    cp_wob = pltpu.make_async_copy(wob_hbm.at[pl.ds(HW, HW), :], stage_ref.at[3, pl.ds(HW, HW), :], sems.at[6])
    cp_phi.start()
    cp_wqkv(1).start()
    cp_x(0).start()
    cp_wqkv(2).start()
    for i in range(1, NCH):
        cp_x(i).start()
    cp_wqkv(0).start()
    cp_woa.start()
    cp_mem.start()
    for i in range(NCH):
        for m in range(3):
            cp_w(m, i).start()
        cp_wo(i).start()
    cp_wob.start()

    def fold_phi(m, dst):
        wphi = wphi_ref[...].astype(f32)
        cat = jnp.concatenate([wphi[d] for d in range(FA)], axis=1)
        cat = jnp.concatenate([cat, jnp.zeros((32 - FA, D), f32)], axis=0).astype(bf16)
        p_row, p_col = _iota((D, D), 0), _iota((D, D), 1)
        spread = (FA * (p_row & 31) + (p_row >> 5) == p_col).astype(f32).astype(bf16)
        u = _dot(cat, spread).astype(bf16)
        dup = ((_iota((48, 32), 0) >> 1) == _iota((48, 32), 1)).astype(f32).astype(bf16)
        u2 = _dot(dup, u)[:GR]
        lane, par = _iota((GR, 128), 1), _iota((GR, 128), 0) & 1
        lhs = []
        for c in range(5):
            blocks = []
            for g in range(3 * c, 3 * c + 4):
                lo = GR * g - 128 * c + FA * par
                blocks.append(jnp.where((lane >= lo) & (lane < lo + FA), u2[:, 128 * c:128 * c + 128], 0.0))
            lhs.append(jnp.concatenate(blocks, axis=0).astype(bf16))
        cp_wqkv(m).wait()
        parts = [_dot_nt(lhs[c], wqkv_ref[m, :, 128 * c:128 * c + 128]) for c in range(5)]
        rows = []
        for c in range(5):
            first = parts[c][:GR] if c == 0 else parts[c][:GR] + parts[c - 1][3 * GR:]
            rows += [first, parts[c][GR:3 * GR]]
        rows.append(parts[4][3 * GR:])
        dst[...] = _pack(jnp.concatenate(rows, axis=0))

    def fold(x, op):
        r = op(op(op(x[:, 0], x[:, 1]), op(x[:, 2], x[:, 3])), x[:, 4])
        r = op(r, pltpu.roll(r, 2, 1))
        return op(r, pltpu.roll(r, 4, 1))

    def feature_map(pt):
        p = pt.reshape(-1, 5, 8, TB)
        ep = jnp.exp(p - fold(p, jnp.maximum)[:, None])
        en = jnp.exp(fold(p, jnp.minimum)[:, None] - p)
        ep = ep * _recip(fold(ep, jnp.add))[:, None]
        en = en * _recip(fold(en, jnp.add))[:, None]
        return jnp.concatenate([ep, en], axis=1)

    def rows_of(b):
        if isinstance(b, int):
            return pl.ds(b * TB, TB), pl.ds(b * TB // 2, TB // 2)
        return pl.ds(pl.multiple_of(b * TB, TB), TB), pl.ds(pl.multiple_of(b * (TB // 2), TB // 2), TB // 2)

    CG = 4
    NC = NG // CG
    CR = CG * GR

    def k_blocks(blocks, load_x, init=False):
        xn, v, phi = {}, {}, {}

        def LN(j):
            rows, prows = rows_of(blocks[j])
            if load_x is not None:
                xn[j] = _layernorm(load_x(rows)).astype(bf16)
                xna_ref[prows, :] = pltpu.bitcast(xn[j], u32)
            else:
                xn[j] = _unpack(xna_ref[prows, :])

        def P(j, c):
            pk = _dot_nt(_unpack(wpkt_ref[c * CR // 2:(c + 1) * CR // 2, :]), xn[j])
            f = feature_map(pk).reshape(2 * CR, TB)
            if init and j == 0:
                z_ref[2 * CR * c:2 * CR * (c + 1), :] = f
            else:
                z_ref[2 * CR * c:2 * CR * (c + 1), :] += f
            phi[j, c] = f

        def V(j, t):
            v[j, t] = _dot(xn[j], _unpack(wv_ref[:, 128 * t:128 * t + 128])).astype(bf16)

        def KV(j, t):
            f = jnp.concatenate([phi[j, c] for c in range(NC)], axis=0)[6 * GR * t:6 * GR * t + 8 * GR]
            if j == len(blocks) - 1:
                r = jnp.concatenate([_dot(f[2 * GR * g:2 * GR * (g + 1)].astype(bf16), v[j, t]) for g in range(4)], axis=0)
            else:
                r = _dot(f.astype(bf16), v[j, t])
            if init and j == 0:
                acc_ref[t] = r
            else:
                acc_ref[t] += r

        LN(0)
        for j in range(len(blocks)):
            if j + 1 < len(blocks):
                LN(j + 1)
            for c in range(NC):
                P(j, c)
            for t in range(5):
                V(j, t)
            for t in range(5):
                KV(j, t)

    def kside_pass(load_x, nsub, pre=None):
        acc_ref[...] = jnp.zeros(acc_ref.shape, f32)
        z_ref[...] = jnp.zeros(z_ref.shape, f32)

        def body(i, carry):
            if pre is not None:
                pre(i)
            k_blocks([i * nsub + j for j in range(nsub)], load_x)
            return carry
        lax.fori_loop(0, S // (TB * nsub), body, 0)

    def finish_kv():
        pad = jnp.zeros((128 - 2 * GR, 128), f32)
        lane = _iota((2 * GR, 128), 1)
        r48, odd = _iota((48, 128), 0), (_iota((48, 128), 1) & 1) == 1
        same = (((r48 >= FA) & (r48 < GR)) | (r48 >= GR + 4)) == odd
        for g in range(NG):
            lo, hi = GR * g, GR * g + GR
            t0, t1 = lo // 128, (hi - 1) // 128
            blk = lambda t: acc_ref[t, 2 * GR * (g - 3 * t):2 * GR * (g - 3 * t + 1), :]
            z = jnp.sum(z_ref[2 * GR * g:2 * GR * (g + 1), :], axis=1, keepdims=True)
            zc = 120 if lo - 128 * t0 < 8 else 0
            a = jnp.where((lane >= zc) & (lane < zc + 8), z, blk(t0))
            a = jnp.concatenate([a, pad], axis=0).T
            parts = [a[lo - 128 * t0:min(hi - 128 * t0, 128)]]
            if t1 != t0:
                parts.append(jnp.concatenate([blk(t1), pad], axis=0).T[:hi - 128 * t1])
            parts.append(a[zc:zc + 8])
            kvt_ref[g] = _pack(jnp.where(same, jnp.concatenate(parts, axis=0), 0.0))

    def q_blocks(blocks, load_x, extra=None, between=None):
        top = _iota((8, TB), 0) < 4
        phi, ot, o, y = {}, {}, {}, {}
        n = len(blocks)

        def P(j):
            xn = _unpack(xna_ref[rows_of(blocks[j])[1], :])
            for c in range(NC):
                f = feature_map(_dot_nt(_unpack(wpqt_ref[c * CR // 2:(c + 1) * CR // 2, :]), xn)).reshape(2 * CR, TB)
                for g in range(CG):
                    phi[j, CG * c + g] = f[2 * GR * g:2 * GR * (g + 1)].astype(bf16)

        def N(j):
            outs = []
            for g in range(NG):
                num = _dot(_unpack(kvt_ref[g])[:, :2 * GR], phi[j, g])
                rm = 1.0 / (num[GR:] + 1e-6)
                rs = pltpu.roll(rm, 4, 0)
                r0, r1 = jnp.where(top, rm, rs), jnp.where(top, rs, rm)
                outs.append(num[:GR] * jnp.concatenate([r0, r0, rm, r1, r1], axis=0))
            ot[j] = jnp.concatenate(outs, axis=0)

        def W(j, t):
            if t == 0:
                o_ref[j] = pltpu.bitcast(ot[j].astype(bf16).T, u32)
                o[j] = _unpack(o_ref[j])
            y[j, t] = _dot(o[j], _unpack(wo_ref[:, 128 * t:128 * t + 128]))
            if t == 4:
                rows = rows_of(blocks[j])[0]
                xres_ref[rows, :] = load_x(rows) + jnp.concatenate([y[j, t] for t in range(5)], axis=1)
                if extra is not None:
                    extra(j)

        WW = lambda j: [W(j, t) for t in range(5)]
        P(0), P(1)
        if between is not None:
            between()
        N(0), P(2), N(1), WW(0), N(2)
        for j in range(3, n):
            P(j), WW(j - 2), N(j)
        WW(n - 2), WW(n - 1)

    def qside_pass(load_x, nsub, extra=None, pre=None):
        def body(i, carry):
            if pre is not None:
                pre(i)
            q_blocks([i * nsub + j for j in range(nsub)], load_x,
                     None if extra is None else functools.partial(extra, i))
            return carry
        lax.fori_loop(0, S // (TB * nsub), body, 0)

    VPERM = [(h * DHB + 64 * c) for c in range(3) for h in range(2)]

    def retile_wo(j, parts):
        for c in parts:
            src = pl.ds(pl.multiple_of(j * PW + VPERM[c], 64), 64)
            wob_ref[j, 32 * c:32 * c + 32, :] = pltpu.bitcast(stage_ref[3, src, :], u32)

    def relayout_weights(i, jj):
        j = i * (NP // NCH) + jj
        retile_wo(i * 2 + jj // 2, range(3 * (jj % 2), 3 * (jj % 2) + 3))
        r0 = pl.multiple_of(j * PW, PW)
        for m in range(2):
            wb_ref[j, :, m * PW:(m + 1) * PW] = pltpu.bitcast(stage_ref[m, pl.ds(r0, PW), :].T, u32)
        for c in range(3):
            w = jnp.concatenate([stage_ref[2, pl.ds(pl.multiple_of(r0 + o, 64), 64), :] for o in VPERM[2 * c:2 * c + 2]], axis=0)
            wb_ref[j, :, 2 * PW + 128 * c:2 * PW + 128 * (c + 1)] = pltpu.bitcast(w.T, u32)

    scale = DHB ** -0.5
    NQ = 32
    row, col = _iota((2 * NQ, 2 * L), 0), _iota((2 * NQ, 2 * L), 1)
    same = (row < NQ) == (col < L)
    rr = jnp.where(row < NQ, row, row - NQ)
    kk = jnp.where(col < L, col, col - L)
    keep = same & ((rr < MEM) | (rr + 8 >= kk))
    fill = jnp.where(same, -1e9, -jnp.inf).astype(f32)
    lo = lambda n, w=128: (_iota((n, w), 1) & 64) == 0
    sub8 = _iota((8, 128), 0)

    def halves(x):
        m = lo(*x.shape)
        return jnp.concatenate([jnp.where(m, x, 0.0), jnp.where(m, 0.0, x)], axis=0).astype(bf16)

    def outer(x):
        return jnp.concatenate([x[:, 0:128], x[:, 256:384]], axis=0).astype(bf16)

    def scores(q, k):
        s1 = _dot_nt(outer(q), outer(k))
        s2 = _dot_nt(q[:, 128:256].astype(bf16), halves(k[:, 128:256]))
        s = s1 + jnp.concatenate([s2, s2], axis=0)
        s = jnp.where(keep, s * scale, fill)
        e = jnp.exp(s - jnp.max(s, axis=1, keepdims=True))
        return e, _recip(jnp.sum(e, axis=1, keepdims=True))

    def values(e, r, v):
        rab = jnp.where(lo(NQ), r[:NQ], r[NQ:])
        return _dot((e[:NQ] + e[NQ:]).astype(bf16), halves(v)) * jnp.concatenate([rab] * 3, axis=1)

    def head_attention(q, kv):
        rot = lambda x, r: pltpu.roll(x, r % 8, 0) if r % 8 else x
        tile = lambda x, c: x[:, 128 * c:128 * c + 128]
        q = q * (scale * LOG2E)
        ks = []
        for b in range(2):
            kb = kv[8 * b:8 * b + 8]
            ks.append((tile(kb, 0), jnp.where(lo(8), tile(kb, 1), 0.0), jnp.where(lo(8), 0.0, tile(kb, 1)), tile(kb, 2)))
        ss, m = {}, None
        for r in range(7, -1, -1):
            qr = [rot(tile(q, c), 8 - r) for c in range(3)]
            for b in range(2):
                k0, kl, kh, k2 = ks[b]
                sa = jnp.sum(qr[0] * k0 + qr[1] * kl, axis=1, keepdims=True)
                sb = jnp.sum(qr[2] * k2 + qr[1] * kh, axis=1, keepdims=True)
                x = jnp.where(lo(8), sa, sb)
                if b == 1 and r > 0:
                    x = jnp.where(sub8 <= 7 - r, x, -1e9 * LOG2E)
                ss[b, r] = x
            mx = jnp.maximum(ss[0, r], ss[1, r])
            m = mx if m is None else jnp.maximum(rot(m, 1), mx)
        acc = None
        for r in range(7, -1, -1):
            mr = rot(m, 8 - r)
            e0, e1 = jnp.exp2(ss[0, r] - mr), jnp.exp2(ss[1, r] - mr)
            t = [e0 + e1] + [e0 * tile(kv[0:8], 3 + c) + e1 * tile(kv[8:16], 3 + c) for c in range(3)]
            acc = t if acc is None else [rot(u, 1) + w for u, w in zip(acc, t)]
        r = _recip(acc[0])
        return jnp.concatenate([acc[1] * r, acc[2] * r, acc[3] * r], axis=1)

    def bstep(h, first, never, early, chained_in, chained_out):
        qkv, ps, os_, ov = {}, {}, {}, {}
        acc = [None]
        nxt = [0]
        lhs = h.astype(bf16)

        def QKV(t):
            if t == 0 and chained_in:
                r = None
                for k in range(5):
                    c = _dot(h[:, 128 * k:128 * k + 128].astype(bf16), _unpack(wb_ref[t, 64 * k:64 * k + 64, :]))
                    r = c if r is None else r + c
            else:
                r = _dot(lhs, _unpack(wb_ref[t]))
            if first:
                svq_ref[t] = r[L:L + 8]
                r = r[:L]
            else:
                r = jnp.concatenate([r[:MEM], svq_ref[t], r[MEM:]], axis=0)
            qkv[t] = r
            ov[t] = head_attention(r[8:16, :PW], r[:16, PW:])

        def SS(j):
            q = jnp.concatenate([qkv[j][:MEM, :PW], qkv[j][16:, :PW]], axis=0)
            ps[j] = scores(q, qkv[j][:, PW:2 * PW])

        def PV(j):
            e, r = ps[j]
            if j >= 1:
                e = jnp.concatenate([jnp.where(never, ov[j - 1][:, 128 * c:128 * c + 2 * L], e[8 * c:8 * c + 8])
                                     for c in range(3)] + [e[24:]], axis=0)
            if j in early:
                e = jnp.concatenate([e[:24], jnp.where(never, early[j][:, :2 * L], e[24:32]), e[32:]], axis=0)
            o = values(e, r, qkv[j][:, 2 * PW:])
            if first:
                svo_ref[j] = o[24:32]
                o = jnp.concatenate([o[:24], ov[j]], axis=0)
            else:
                o = jnp.concatenate([o, ov[j], svo_ref[j]], axis=0)
            os_[j] = o

        def OO(n, merge=1):
            for _ in range(n):
                js = range(nxt[0], nxt[0] + merge)
                c = _dot(jnp.concatenate([os_[j] for j in js], axis=1).astype(bf16),
                         _unpack(jnp.concatenate([wob_ref[j] for j in js], axis=0)))
                acc[0] = c if acc[0] is None else acc[0] + c
                nxt[0] += merge

        n1, n2, n3, nl = (3, 3, 2, 2) if first else (2, 2, 1, 2 if chained_out else 1)
        nd = n1 + n2 + n3 + nl
        for t in range(NP):
            for op in ("QSOP" if first else "QOPS"):
                if op == "Q":
                    QKV(t)
                if op == "S" and t >= 1:
                    SS(t - 1)
                if op == "P" and t >= 2:
                    PV(t - 2)
                if op == "O" and 4 <= t < NP - 1 and nxt[0] < NP - nd:
                    OO(1)
        OO(n1)
        SS(NP - 1)
        PV(NP - 2)
        OO(n2)
        PV(NP - 1)
        OO(n3)
        OO(1, nl)
        return acc[0]

    def bpass(last):
        R = 64 * UNR
        mem_ref[...] = mem0_ref[...].astype(f32)
        xnb_ref[...] = _layernorm(xres_ref[0:R, :])

        def body(i, c):
            never = flag_ref[:, :2 * L] > 0
            probe = lambda x, g: x[8 * g:8 * g + 8, 0:128]
            mem = mem_ref[...]
            xall = xnb_ref[...]
            for u in range(UNR):
                r0 = pl.multiple_of(i * R + 64 * u, 64)
                xa = xall[64 * u:64 * u + 64]
                rn = pl.multiple_of(jnp.minimum(r0 + R, S - 64), 64)
                xn = _layernorm(xres_ref[pl.ds(rn, 64), :])
                xnb_ref[64 * u:64 * u + 64, :] = xn
                early = {LN_AT + g: probe(xn, g) for g in range(8)}
                if not last:
                    rp = pl.multiple_of(jnp.maximum(r0 - 64, 0), 64)
                    xn = _layernorm(xres_ref[pl.ds(rp, 64), :])
                    xna_ref[pl.ds(pl.multiple_of(rp // 2, 32), 32), :] = _pack(xn)
                    for g in range(8):
                        j = LN_AT2 + g
                        early[j] = jnp.maximum(early[j], probe(xn, g)) if j in early else probe(xn, g)
                ya = bstep(jnp.concatenate([mem, xa[:L]], axis=0), True, never, early, u > 0, True)
                yb = bstep(jnp.concatenate([ya[:MEM], xa[L:]], axis=0), False, never, {}, True, u < UNR - 1)
                mem = yb[:MEM]
                y = xres_ref[pl.ds(r0, 64), :] + jnp.concatenate([ya[24:32], ya[MEM:24], yb[40:48], yb[32:40], yb[MEM:32]], axis=0)
                if last:
                    out_ref[pl.ds(r0, 64), :] = y.astype(bf16)
                else:
                    xres_ref[pl.ds(r0, 64), :] = y
            mem_ref[...] = mem
            if last:
                rows = pl.ds(pl.multiple_of(i * R, R), R)
                pltpu.make_async_copy(out_ref.at[rows, :], out_hbm.at[rows, :], sems.at[7]).start()
            return c
        lax.fori_loop(0, S // R, body, 0)

    load_in = lambda rows: x_ref[rows, :].astype(f32)
    load_res = lambda rows: xres_ref[rows, :]

    def wait_w(i):
        for m in range(3):
            cp_w(m, i).wait()
        cp_wo(i).wait()

    with _scope("pro"):
        flag_ref[...] = jnp.zeros(flag_ref.shape, jnp.int32)
        cnt_ref[0] = 0
        cp_phi.wait()
        fold_phi(1, wpkt_ref)
        cp_wqkv(2).wait()
        wv_ref[...] = pltpu.bitcast(wqkv_ref[2], u32)
    with _scope("k1"):
        kside_pass(load_in, S // (TB * NCH), pre=lambda i: cp_x(i).wait())
    with _scope("f1"):
        cp_woa.wait()
        cp_mem.wait()
        fold_phi(0, wpqt_ref)
        wo_ref[...] = pltpu.bitcast(woa_ref[...], u32)
        finish_kv()
    with _scope("q1"):
        qside_pass(load_in, S // (TB * NCH), relayout_weights, wait_w)
    with _scope("wait"):
        cp_wob.wait()
        for j in range(NP // 2, NP):
            retile_wo(j, range(6))
    with _scope("b1"):
        bpass(False)
    if True:
        with _scope("a2"):
            pl.when(cnt_ref[0] == 0)(lambda: k_blocks(list(range(KSPLIT)), None, init=True))
            xna_ref[(S - 64) // 2:, :] = _pack(_layernorm(xres_ref[S - 64:, :]))
            k_blocks(list(range(KSPLIT, 16)), None)
            q_blocks(list(range(16)), load_res, between=finish_kv)
    with _scope("b2"):
        bpass(True)
    pltpu.make_async_copy(out_ref, out_hbm, sems.at[7]).wait()


@functools.partial(jax.jit, static_argnames=("B_seg_len",))
def pallas_interleave_layers__linear_kernel_hedgehog__memory_aug_recurrent_mem_tr__prompt_kernel(
    A_x: jax.Array,
    A_wqkv: jax.Array,
    A_w_phi: jax.Array,
    A_wo: jax.Array,
    B_x: jax.Array,
    B_mem0: jax.Array,
    B_Wq: jax.Array,
    B_Wk: jax.Array,
    B_Wv: jax.Array,
    B_Wo: jax.Array,
    B_seg_len: int,
):
    del B_x
    assert B_seg_len == SEG
    assert A_x.shape == (1, S, D) and B_mem0.shape == (1, MEM, D)
    assert B_Wq.shape == (D, HB, DHB) and A_w_phi.shape == (HA, FA, FA)
    tr = lambda w: jnp.transpose(w, (1, 2, 0)).reshape(HB * DHB, D)
    hbm = pl.BlockSpec(memory_space=pl.ANY)
    out = pl.pallas_call(
        _kernel,
        out_shape=jax.ShapeDtypeStruct((S, D), bf16),
        in_specs=[hbm] * 9,
        out_specs=hbm,
        scratch_shapes=[
            pltpu.VMEM((S, D), bf16),
            pltpu.VMEM((3, D, D), bf16),
            pltpu.VMEM((FA, FA, HA), bf16),
            pltpu.VMEM((D, D), bf16),
            pltpu.VMEM((MEM, D), bf16),
            pltpu.VMEM((S, D), bf16),
            pltpu.VMEM((4, HB * DHB, D), bf16),
            pltpu.VMEM((NP, D // 2, 3 * PW), u32),
            pltpu.VMEM((NP, PW // 2, D), u32),
            pltpu.VMEM((S, D), f32),
            pltpu.VMEM((S // 2, D), u32),
            pltpu.VMEM((64 * UNR, D), f32),
            pltpu.VMEM((D // 2, D), u32),
            pltpu.VMEM((D // 2, D), u32),
            pltpu.VMEM((D // 2, D), u32),
            pltpu.VMEM((D // 2, D), u32),
            pltpu.VMEM((5, 8 * GR, 128), f32),
            pltpu.VMEM((2 * D, TB), f32),
            pltpu.VMEM((NG, 24, 128), u32),
            pltpu.VMEM((16, TB // 2, D), u32),
            pltpu.VMEM((MEM, D), f32),
            pltpu.VMEM((NP, 8, 3 * PW), f32),
            pltpu.VMEM((NP, 8, PW), f32),
            pltpu.VMEM((8, 128), jnp.int32),
            pltpu.SMEM((1,), jnp.int32),
            pltpu.SemaphoreType.DMA((8 + 5 * NCH,)),
        ],
        compiler_params=pltpu.CompilerParams(vmem_limit_bytes=120 * 1024 * 1024),
        name="hedgehog_rmt",
    )(A_x.reshape(S, D), A_wqkv, jnp.transpose(A_w_phi, (1, 2, 0)), A_wo, B_mem0.reshape(MEM, D),
      tr(B_Wq), tr(B_Wk), tr(B_Wv), B_Wo.reshape(HB * DHB, D))
    return out.reshape(1, S, D)
```

```python
import contextlib
import functools

import jax
import jax.numpy as jnp
from jax import lax
import jax.experimental.pallas as pl
import jax.experimental.pallas.tpu as pltpu

f32, bf16, u32 = jnp.float32, jnp.bfloat16, jnp.uint32

S, D = 2048, 640
HA, FA = 32, 20
HB, DHB = 32, 192
MEM, SEG = 8, 32
L = MEM + SEG
NP = HB // 2
PW = 2 * DHB
TB = 128
NG = 16
GR = 2 * FA
NCH = 4
WO_CUTS = (NCH, 13, 15, 16)
NT = (((1,), (1,)), ((), ()))
LOG2E = 1.4426950408889634
import os
_E = lambda k, d: type(d)(os.environ.get(k, d))
LN_AT = _E('LN_AT', 0)
LN_AT2 = _E('LN_AT2', 4)
NPR = _E('NPR', 1)
LEAD = _E('LEAD', 1)
KSPLIT = _E('KSPLIT', 8)
UNR1 = _E('UNR1', 1)
FLIP = [int(v) for v in _E('FLIP', '0,1,2,3,4,13,14,15').split(',') if v]
FLIPM = [int(v) for v in _E('FLIPM', '2').split(',') if v]
ORD_A, ORD_B = _E('OA', 'QSPO'), _E('OB', 'QOPS')
TAIL_A, TAIL_B = _E('TLA', 'OOOSPOOOPOO'), _E('TLB', 'OOSPOOPO')
TAIL_C = _E('TLC', 'OOSPOOPO')
OLAG = _E('OLAG', 4)
OLAG_B = _E('OLAGB', 4)
NLA, NLC = _E('NLA', 3), _E('NLC', 1)
PORD_A = [int(c) for c in _E('PA', '120')]
PORD_B = [int(c) for c in _E('PB', '012')]
ONLYB = _E('ONLYB', 0)
A2MODE = _E('A2MODE', 1)


_scope = lambda name: contextlib.nullcontext()


def _dot(a, b):
    return jnp.dot(a, b, preferred_element_type=f32)


def _dot_nt(a, b):
    return lax.dot_general(a, b, NT, preferred_element_type=f32)


def _pack(x):
    return pltpu.bitcast(x.astype(bf16), u32)


def _unpack(x):
    return pltpu.bitcast(x, bf16)


def _recip(x):
    r = pl.reciprocal(x, approx=True)
    return r * (2.0 - x * r)


def _layernorm(x):
    m = jnp.mean(x, axis=-1, keepdims=True)
    xc = x - m
    v = jnp.mean(xc * xc, axis=-1, keepdims=True)
    return xc * lax.rsqrt(v + 1e-5)


def _iota(shape, dim):
    return lax.broadcasted_iota(jnp.int32, shape, dim)


def _kernel(x_hbm, wqkv_hbm, wphi_hbm, woa_hbm, mem0_hbm, wqt_hbm, wkt_hbm, wvt_hbm, wob_hbm,
            out_hbm,
            x_ref, wqkv_ref, wphi_ref, woa_ref, mem0_ref, out_ref,
            stage_ref, wb_ref, wob_ref, xres_ref, xna_ref, xnb_ref,
            wpqt_ref, wpkt_ref, wv_ref, wo_ref, acc_ref, z_ref, kvt_ref, o_ref,
            mem_ref, svq_ref, svo_ref, flag_ref, cnt_ref, sems):
    XC = S // NCH
    WC = HB * DHB // NCH

    def cp_wqkv(m):
        return pltpu.make_async_copy(wqkv_hbm.at[:, pl.ds(m * D, D)], wqkv_ref.at[m], sems.at[m])

    def cp_x(i):
        rows = pl.ds(pl.multiple_of(i * XC, XC), XC)
        return pltpu.make_async_copy(x_hbm.at[rows, :], x_ref.at[rows, :], sems.at[8 + i])

    def cp_w(m, i):
        rows = pl.ds(pl.multiple_of(i * WC, WC), WC)
        return pltpu.make_async_copy((wqt_hbm, wkt_hbm, wvt_hbm)[m].at[rows, :], stage_ref.at[m, rows, :],
                                     sems.at[8 + NCH * (m + 1) + i])

    cp_phi = pltpu.make_async_copy(wphi_hbm, wphi_ref, sems.at[3])
    cp_woa = pltpu.make_async_copy(woa_hbm, woa_ref, sems.at[4])
    cp_mem = pltpu.make_async_copy(mem0_hbm, mem0_ref, sems.at[5])
    def cp_wo(i):
        rows = pl.ds(pl.multiple_of(i * PW, PW), PW)
        return pltpu.make_async_copy(wob_hbm.at[rows, :], stage_ref.at[3, rows, :], sems.at[8 + 4 * NCH + i])

    def cp_wo_tail(n):
        rows = pl.ds(WO_CUTS[n] * PW, (WO_CUTS[n + 1] - WO_CUTS[n]) * PW)
        return pltpu.make_async_copy(wob_hbm.at[rows, :], stage_ref.at[3, rows, :], sems.at[8 + 5 * NCH + n])

    cp_phi.start()
    cp_wqkv(1).start()
    cp_x(0).start()
    cp_wqkv(2).start()
    for i in range(1, NCH):
        cp_x(i).start()
    cp_wqkv(0).start()
    cp_woa.start()
    cp_mem.start()
    for i in range(NCH):
        for m in range(3):
            cp_w(m, i).start()
        cp_wo(i).start()
    for n in range(len(WO_CUTS) - 1):
        cp_wo_tail(n).start()

    def fold_phi(m, dst):
        wphi = wphi_ref[...].astype(f32)
        cat = jnp.concatenate([wphi[d] for d in range(FA)], axis=1)
        cat = jnp.concatenate([cat, jnp.zeros((32 - FA, D), f32)], axis=0).astype(bf16)
        p_row, p_col = _iota((D, D), 0), _iota((D, D), 1)
        spread = (FA * (p_row & 31) + (p_row >> 5) == p_col).astype(f32).astype(bf16)
        u = _dot(cat, spread).astype(bf16)
        dup = ((_iota((48, 32), 0) >> 1) == _iota((48, 32), 1)).astype(f32).astype(bf16)
        u2 = _dot(dup, u)[:GR]
        lane, par = _iota((GR, 128), 1), _iota((GR, 128), 0) & 1
        lhs = []
        for c in range(5):
            blocks = []
            for g in range(3 * c, 3 * c + 4):
                lo = GR * g - 128 * c + FA * par
                blocks.append(jnp.where((lane >= lo) & (lane < lo + FA), u2[:, 128 * c:128 * c + 128], 0.0))
            lhs.append(jnp.concatenate(blocks, axis=0).astype(bf16))
        cp_wqkv(m).wait()
        parts = [_dot_nt(lhs[c], wqkv_ref[m, :, 128 * c:128 * c + 128]) for c in range(5)]
        rows = []
        for c in range(5):
            first = parts[c][:GR] if c == 0 else parts[c][:GR] + parts[c - 1][3 * GR:]
            rows += [first, parts[c][GR:3 * GR]]
        rows.append(parts[4][3 * GR:])
        dst[...] = _pack(jnp.concatenate(rows, axis=0))

    def fold(x, op):
        r = op(op(op(x[:, 0], x[:, 1]), op(x[:, 2], x[:, 3])), x[:, 4])
        r = op(r, pltpu.roll(r, 2, 1))
        return op(r, pltpu.roll(r, 4, 1))

    def feature_map(pt):
        p = pt.reshape(-1, 5, 8, TB)
        ep = jnp.exp(p - fold(p, jnp.maximum)[:, None])
        en = jnp.exp(fold(p, jnp.minimum)[:, None] - p)
        ep = ep * _recip(fold(ep, jnp.add))[:, None]
        en = en * _recip(fold(en, jnp.add))[:, None]
        return jnp.concatenate([ep, en], axis=1)

    def rows_of(b):
        if isinstance(b, int):
            return pl.ds(b * TB, TB), pl.ds(b * TB // 2, TB // 2)
        return pl.ds(pl.multiple_of(b * TB, TB), TB), pl.ds(pl.multiple_of(b * (TB // 2), TB // 2), TB // 2)

    CG = 4
    NC = NG // CG
    CR = CG * GR

    def k_blocks(blocks, load_x, init=False):
        xn, v, phi = {}, {}, {}

        def LN(j):
            rows, prows = rows_of(blocks[j])
            if load_x is not None:
                xn[j] = _layernorm(load_x(rows)).astype(bf16)
                xna_ref[prows, :] = pltpu.bitcast(xn[j], u32)
            else:
                xn[j] = _unpack(xna_ref[prows, :])

        def P(j, c):
            pk = _dot_nt(_unpack(wpkt_ref[c * CR // 2:(c + 1) * CR // 2, :]), xn[j])
            f = feature_map(pk).reshape(2 * CR, TB)
            if init and j == 0:
                z_ref[2 * CR * c:2 * CR * (c + 1), :] = f
            else:
                z_ref[2 * CR * c:2 * CR * (c + 1), :] += f
            phi[j, c] = f

        def V(j, t):
            v[j, t] = _dot(xn[j], _unpack(wv_ref[:, 128 * t:128 * t + 128])).astype(bf16)

        def KV(j, t):
            f = jnp.concatenate([phi[j, c] for c in range(NC)], axis=0)[6 * GR * t:6 * GR * t + 8 * GR]
            if j == len(blocks) - 1:
                r = jnp.concatenate([_dot(f[2 * GR * g:2 * GR * (g + 1)].astype(bf16), v[j, t]) for g in range(4)], axis=0)
            else:
                r = _dot(f.astype(bf16), v[j, t])
            if init and j == 0:
                acc_ref[t] = r
            else:
                acc_ref[t] += r

        LN(0)
        for j in range(len(blocks)):
            if j + 1 < len(blocks):
                LN(j + 1)
            for c in range(NC):
                P(j, c)
            for t in range(5):
                V(j, t)
            for t in range(5):
                KV(j, t)

    def kside_pass(load_x, nsub, pre=None):
        acc_ref[...] = jnp.zeros(acc_ref.shape, f32)
        z_ref[...] = jnp.zeros(z_ref.shape, f32)

        def body(i, carry):
            if pre is not None:
                pre(i)
            k_blocks([i * nsub + j for j in range(nsub)], load_x)
            return carry
        lax.fori_loop(0, S // (TB * nsub), body, 0)

    def finish_kv():
        pad = jnp.zeros((128 - 2 * GR, 128), f32)
        lane = _iota((2 * GR, 128), 1)
        r48, odd = _iota((48, 128), 0), (_iota((48, 128), 1) & 1) == 1
        same = (((r48 >= FA) & (r48 < GR)) | (r48 >= GR + 4)) == odd
        for g in range(NG):
            lo, hi = GR * g, GR * g + GR
            t0, t1 = lo // 128, (hi - 1) // 128
            blk = lambda t: acc_ref[t, 2 * GR * (g - 3 * t):2 * GR * (g - 3 * t + 1), :]
            z = jnp.sum(z_ref[2 * GR * g:2 * GR * (g + 1), :], axis=1, keepdims=True)
            zc = 120 if lo - 128 * t0 < 8 else 0
            a = jnp.where((lane >= zc) & (lane < zc + 8), z, blk(t0))
            a = jnp.concatenate([a, pad], axis=0).T
            parts = [a[lo - 128 * t0:min(hi - 128 * t0, 128)]]
            if t1 != t0:
                parts.append(jnp.concatenate([blk(t1), pad], axis=0).T[:hi - 128 * t1])
            parts.append(a[zc:zc + 8])
            kvt_ref[g] = _pack(jnp.where(same, jnp.concatenate(parts, axis=0), 0.0))

    def q_blocks(blocks, load_x, extra=None, between=None):
        top = _iota((8, TB), 0) < 4
        phi, ot, o, y = {}, {}, {}, {}
        n = len(blocks)

        def P(j):
            xn = _unpack(xna_ref[rows_of(blocks[j])[1], :])
            for c in range(NC):
                f = feature_map(_dot_nt(_unpack(wpqt_ref[c * CR // 2:(c + 1) * CR // 2, :]), xn)).reshape(2 * CR, TB)
                for g in range(CG):
                    phi[j, CG * c + g] = f[2 * GR * g:2 * GR * (g + 1)].astype(bf16)

        def N(j):
            outs = []
            for g in range(NG):
                num = _dot(_unpack(kvt_ref[g])[:, :2 * GR], phi[j, g])
                rm = 1.0 / (num[GR:] + 1e-6)
                rs = pltpu.roll(rm, 4, 0)
                r0, r1 = jnp.where(top, rm, rs), jnp.where(top, rs, rm)
                outs.append(num[:GR] * jnp.concatenate([r0, r0, rm, r1, r1], axis=0))
            ot[j] = jnp.concatenate(outs, axis=0)

        def W(j, t):
            if t == 0:
                o_ref[j] = pltpu.bitcast(ot[j].astype(bf16).T, u32)
                o[j] = _unpack(o_ref[j])
            y[j, t] = _dot(o[j], _unpack(wo_ref[:, 128 * t:128 * t + 128]))
            if t == 4:
                rows = rows_of(blocks[j])[0]
                xres_ref[rows, :] = load_x(rows) + jnp.concatenate([y[j, t] for t in range(5)], axis=1)
                if extra is not None:
                    extra(j)

        WW = lambda j: [W(j, t) for t in range(5)]
        P(0), P(1)
        if between is not None:
            between()
        N(0), P(2), N(1), WW(0), N(2)
        for j in range(3, n):
            P(j), WW(j - 2), N(j)
        WW(n - 2), WW(n - 1)

    def qside_pass(load_x, nsub, extra=None, pre=None):
        def body(i, carry):
            if pre is not None:
                pre(i)
            q_blocks([i * nsub + j for j in range(nsub)], load_x,
                     None if extra is None else functools.partial(extra, i))
            return carry
        lax.fori_loop(0, S // (TB * nsub), body, 0)

    VPERM = [(h * DHB + 64 * c) for c in range(3) for h in range(2)]

    def retile_wo(j, parts):
        for c in parts:
            src = pl.ds(pl.multiple_of(j * PW + VPERM[c], 64), 64)
            wob_ref[j, 32 * c:32 * c + 32, :] = pltpu.bitcast(stage_ref[3, src, :], u32)

    def relayout_weights(i, jj):
        j = i * (NP // NCH) + jj
        retile_wo(i, range(2 * jj, min(2 * jj + 2, 6)))
        r0 = pl.multiple_of(j * PW, PW)
        for m in range(2):
            wb_ref[j, :, m * PW:(m + 1) * PW] = pltpu.bitcast(stage_ref[m, pl.ds(r0, PW), :].T, u32)
        for c in range(3):
            w = jnp.concatenate([stage_ref[2, pl.ds(pl.multiple_of(r0 + o, 64), 64), :] for o in VPERM[2 * c:2 * c + 2]], axis=0)
            wb_ref[j, :, 2 * PW + 128 * c:2 * PW + 128 * (c + 1)] = pltpu.bitcast(w.T, u32)

    scale = DHB ** -0.5
    NQ = 32
    row, col = _iota((2 * NQ, 2 * L), 0), _iota((2 * NQ, 2 * L), 1)
    same = (row < NQ) == (col < L)
    rr = jnp.where(row < NQ, row, row - NQ)
    kk = jnp.where(col < L, col, col - L)
    keep = same & ((rr < MEM) | (rr >= kk) | (kk >= NQ))
    fill = jnp.where(same, -1e9 / scale, -jnp.inf).astype(f32)
    lo = lambda n, w=128: (_iota((n, w), 1) & 64) == 0
    sub8 = _iota((8, 128), 0)

    def halves(x):
        m = lo(*x.shape)
        return jnp.concatenate([jnp.where(m, x, 0.0), jnp.where(m, 0.0, x)], axis=0).astype(bf16)

    def outer(x):
        return jnp.concatenate([x[:, 0:128], x[:, 256:384]], axis=0).astype(bf16)

    def scores(q, k):
        s1 = _dot_nt(outer(q), outer(k))
        s2 = _dot_nt(q[:, 128:256].astype(bf16), halves(k[:, 128:256]))
        s = s1 + jnp.concatenate([s2, s2], axis=0)
        s = jnp.where(keep, s, fill)
        e = jnp.exp2((s - jnp.max(s, axis=1, keepdims=True)) * (scale * LOG2E))
        return e, jnp.sum(e, axis=1, keepdims=True)

    def values(e, l, v):
        rab = _recip(jnp.where(lo(NQ), l[:NQ], l[NQ:]))
        return _dot((e[:NQ] + e[NQ:]).astype(bf16), halves(v)) * jnp.concatenate([rab] * 3, axis=1)

    def head_attention(q, kv):
        rot = lambda x, r: pltpu.roll(x, r % 8, 0) if r % 8 else x
        tile = lambda x, c: x[:, 128 * c:128 * c + 128]
        q = q * (scale * LOG2E)
        ks = []
        for b in range(2):
            kb = kv[8 * b:8 * b + 8]
            ks.append((tile(kb, 0), jnp.where(lo(8), tile(kb, 1), 0.0), jnp.where(lo(8), 0.0, tile(kb, 1)), tile(kb, 2)))
        ss, m = {}, None
        for r in range(7, -1, -1):
            qr = [rot(tile(q, c), 8 - r) for c in range(3)]
            for b in range(2):
                k0, kl, kh, k2 = ks[b]
                sa = jnp.sum(qr[0] * k0 + qr[1] * kl, axis=1, keepdims=True)
                sb = jnp.sum(qr[2] * k2 + qr[1] * kh, axis=1, keepdims=True)
                x = jnp.where(lo(8), sa, sb)
                if b == 1 and r > 0:
                    x = jnp.where(sub8 <= 7 - r, x, -1e9 * LOG2E)
                ss[b, r] = x
            mx = jnp.maximum(ss[0, r], ss[1, r])
            m = mx if m is None else jnp.maximum(rot(m, 1), mx)
        acc = None
        for r in range(7, -1, -1):
            mr = rot(m, 8 - r)
            e0, e1 = jnp.exp2(ss[0, r] - mr), jnp.exp2(ss[1, r] - mr)
            t = [e0 + e1] + [e0 * tile(kv[0:8], 3 + c) + e1 * tile(kv[8:16], 3 + c) for c in range(3)]
            acc = t if acc is None else [rot(u, 1) + w for u, w in zip(acc, t)]
        r = _recip(acc[0])
        return jnp.concatenate([acc[1] * r, acc[2] * r, acc[3] * r], axis=1)

    def is_long(first, t, m):
        return first != (m in FLIPM and t in FLIP)

    def bstep(h, first, never, early, chained_in, chained_out):
        qkv, ps, os_, ov = {}, {}, {}, {}
        acc = [None]
        nxt = [0]

        def PR(t, ms):
            hs = {m: h if is_long(first, t, m) else h[:NQ] for m in ms}
            if t == 0 and chained_in:
                rs = {}
                for k in range(5):
                    for m in ms:
                        c = _dot(hs[m][:, 128 * k:128 * k + 128].astype(bf16),
                                 _unpack(wb_ref[t, 64 * k:64 * k + 64, m * PW:(m + 1) * PW]))
                        rs[m] = c if k == 0 else rs[m] + c
            else:
                rs = {m: _dot(hs[m].astype(bf16), _unpack(wb_ref[t, :, m * PW:(m + 1) * PW])) for m in ms}
            for m in ms:
                if is_long(first, t, m):
                    svq_ref[t, :, m * PW:(m + 1) * PW] = rs[m][L:]
                    qkv[t, m] = rs[m][:L]
                else:
                    qkv[t, m] = jnp.concatenate([rs[m], svq_ref[t, :, m * PW:(m + 1) * PW]], axis=0)
            if 2 in ms:
                kv = jnp.concatenate([qkv[t, 1], qkv[t, 2]], axis=1)
                ov[t] = head_attention(qkv[t, 0][NQ:], jnp.concatenate([kv[:MEM], kv[NQ:]], axis=0))

        def SS(j):
            ps[j] = scores(qkv[j, 0][:NQ], qkv[j, 1])

        def PV(j):
            e, l = ps[j]
            if j >= 1:
                e = jnp.concatenate([jnp.where(never, ov[j - 1][:, 128 * c:128 * c + 2 * L], e[8 * c:8 * c + 8])
                                     for c in range(3)] + [e[24:]], axis=0)
            if j in early:
                e = jnp.concatenate([e[:24], jnp.where(never, early[j][:, :2 * L], e[24:32]), e[32:]], axis=0)
            o = values(e, l, qkv[j, 2])
            if first:
                svo_ref[j] = o[24:32]
                o = jnp.concatenate([o[:24], ov[j]], axis=0)
            else:
                o = jnp.concatenate([o, ov[j], svo_ref[j]], axis=0)
            os_[j] = o

        def OO(merge=1):
            js = range(nxt[0], nxt[0] + merge)
            c = _dot(jnp.concatenate([os_[j] for j in js], axis=1).astype(bf16),
                     _unpack(jnp.concatenate([wob_ref[j] for j in js], axis=0)))
            acc[0] = c if acc[0] is None else acc[0] + c
            nxt[0] += merge

        order, tail, olag = (ORD_A, TAIL_A, OLAG) if first else (ORD_B, TAIL_C if chained_out else TAIL_B, OLAG_B)
        nl = (NLA if first else NLC) if chained_out else 1
        nd = tail.count("O") + nl
        for t in range(NP):
            for op in order:
                if op == "Q":
                    PR(t, [m for m in (PORD_A if first else PORD_B) if m != 2 or "V" not in order])
                if op == "V" and t >= 1:
                    PR(t - 1, [2])
                if op == "S" and t >= 1:
                    SS(t - 1)
                if op == "P" and t >= 2:
                    PV(t - 2)
                if op == "O" and olag <= t < NP - 1 and nxt[0] < NP - nd:
                    OO()
        p = NP - 2
        for op in tail:
            if op == "O":
                OO()
            if op == "S":
                SS(NP - 1)
            if op == "V":
                PR(NP - 1, [2])
            if op == "P":
                PV(p)
                p += 1
        OO(nl)
        assert nxt[0] == NP and p == NP
        return acc[0]

    def bpass_init(UNR):
        R = 64 * UNR
        mem_ref[...] = mem0_ref[...].astype(f32)
        x0 = _layernorm(xres_ref[0:R, :])
        xnb_ref[0:R, :] = x0
        for t in FLIP:
            for m in FLIPM:
                svq_ref[t, :, m * PW:(m + 1) * PW] = _dot(x0[0:16].astype(bf16), _unpack(wb_ref[t, :, m * PW:(m + 1) * PW]))[:8]

    def bpass(last, UNR):
        R = 64 * UNR

        def body(i, c):
            never = flag_ref[:, :2 * L] > 0
            probe = lambda x, g: x[8 * g:8 * g + 8, 0:128]
            mem = mem_ref[...]
            xall = xnb_ref[0:R, :]
            for u in range(UNR):
                r0 = pl.multiple_of(i * R + 64 * u, 64)
                xa = xall[64 * u:64 * u + 64]
                rn = pl.multiple_of(jnp.minimum(r0 + R, S - 64), 64)
                xn = _layernorm(xres_ref[pl.ds(rn, 64), :])
                xnb_ref[64 * u:64 * u + 64, :] = xn
                if u == 0:
                    head_next = xn[0:8]
                early = {LN_AT + g: probe(xn, g) for g in range(8)}
                if not last:
                    rp = pl.multiple_of(jnp.maximum(r0 - 64, 0), 64)
                    xn = _layernorm(xres_ref[pl.ds(rp, 64), :])
                    xna_ref[pl.ds(pl.multiple_of(rp // 2, 32), 32), :] = _pack(xn)
                    for g in range(8):
                        j = LN_AT2 + g
                        early[j] = jnp.maximum(early[j], probe(xn, g)) if j in early else probe(xn, g)
                nxt8 = head_next if u == UNR - 1 else xall[64 * u + 64:64 * u + 72]
                ya = bstep(jnp.concatenate([mem, xa[8:32], xa[0:8], xa[32:40]], axis=0), True, never, early, u > 0, True)
                yb = bstep(jnp.concatenate([ya[:MEM], xa[40:64], xa[32:40], nxt8], axis=0), False, never, {}, True, u < UNR - 1)
                mem = yb[:MEM]
                y = xres_ref[pl.ds(r0, 64), :] + jnp.concatenate([ya[24:32], ya[MEM:24], yb[40:48], yb[32:40], yb[MEM:32]], axis=0)
                if last:
                    out_ref[pl.ds(r0, 64), :] = y.astype(bf16)
                else:
                    xres_ref[pl.ds(r0, 64), :] = y
            mem_ref[...] = mem
            if last:
                rows = pl.ds(pl.multiple_of(i * R, R), R)
                pltpu.make_async_copy(out_ref.at[rows, :], out_hbm.at[rows, :], sems.at[7]).start()
            return c
        lax.fori_loop(0, S // R, body, 0)

    load_in = lambda rows: x_ref[rows, :].astype(f32)
    load_res = lambda rows: xres_ref[rows, :]

    def wait_w(i):
        for m in range(3):
            cp_w(m, i).wait()
        cp_wo(i).wait()

    with _scope("pro"):
        flag_ref[...] = jnp.zeros(flag_ref.shape, jnp.int32)
        cnt_ref[0] = 0
        cp_phi.wait()
        fold_phi(1, wpkt_ref)
        cp_wqkv(2).wait()
        wv_ref[...] = pltpu.bitcast(wqkv_ref[2], u32)
    with _scope("k1"):
        kside_pass(load_in, S // (TB * NCH), pre=lambda i: cp_x(i).wait())
    with _scope("f1"):
        cp_woa.wait()
        cp_mem.wait()
        fold_phi(0, wpqt_ref)
        wo_ref[...] = pltpu.bitcast(woa_ref[...], u32)
        finish_kv()
    with _scope("q1"):
        qside_pass(load_in, S // (TB * NCH), relayout_weights, wait_w)
    with _scope("wait"):
        for n in range(len(WO_CUTS) - 1):
            cp_wo_tail(n).wait()
            if n == 0:
                bpass_init(UNR1)
            for j in range(WO_CUTS[n], WO_CUTS[n + 1]):
                retile_wo(j, range(6))
    with _scope("b1"):
        bpass(False, UNR1)
    if not ONLYB:
        with _scope("a2"):
            lax.fori_loop(0, cnt_ref[0] + 1, lambda i, c: (k_blocks(list(range(KSPLIT)), None, init=True), c)[1], 0)
            xna_ref[(S - 64) // 2:, :] = _pack(_layernorm(xres_ref[S - 64:, :]))
            k_blocks(list(range(KSPLIT, 16)), None)
            q_blocks(list(range(16)), load_res, between=finish_kv)
    with _scope("b2"):
        bpass_init(2)
        bpass(True, 2)
    pltpu.make_async_copy(out_ref, out_hbm, sems.at[7]).wait()


@functools.partial(jax.jit, static_argnames=("B_seg_len",))
def pallas_interleave_layers__linear_kernel_hedgehog__memory_aug_recurrent_mem_tr__prompt_kernel(
    A_x: jax.Array,
    A_wqkv: jax.Array,
    A_w_phi: jax.Array,
    A_wo: jax.Array,
    B_x: jax.Array,
    B_mem0: jax.Array,
    B_Wq: jax.Array,
    B_Wk: jax.Array,
    B_Wv: jax.Array,
    B_Wo: jax.Array,
    B_seg_len: int,
):
    del B_x
    assert B_seg_len == SEG
    assert A_x.shape == (1, S, D) and B_mem0.shape == (1, MEM, D)
    assert B_Wq.shape == (D, HB, DHB) and A_w_phi.shape == (HA, FA, FA)
    tr = lambda w: jnp.transpose(w, (1, 2, 0)).reshape(HB * DHB, D)
    hbm = pl.BlockSpec(memory_space=pl.ANY)
    out = pl.pallas_call(
        _kernel,
        out_shape=jax.ShapeDtypeStruct((S, D), bf16),
        in_specs=[hbm] * 9,
        out_specs=hbm,
        scratch_shapes=[
            pltpu.VMEM((S, D), bf16),
            pltpu.VMEM((3, D, D), bf16),
            pltpu.VMEM((FA, FA, HA), bf16),
            pltpu.VMEM((D, D), bf16),
            pltpu.VMEM((MEM, D), bf16),
            pltpu.VMEM((S, D), bf16),
            pltpu.VMEM((4, HB * DHB, D), bf16),
            pltpu.VMEM((NP, D // 2, 3 * PW), u32),
            pltpu.VMEM((NP, PW // 2, D), u32),
            pltpu.VMEM((S, D), f32),
            pltpu.VMEM((S // 2, D), u32),
            pltpu.VMEM((128, D), f32),
            pltpu.VMEM((D // 2, D), u32),
            pltpu.VMEM((D // 2, D), u32),
            pltpu.VMEM((D // 2, D), u32),
            pltpu.VMEM((D // 2, D), u32),
            pltpu.VMEM((5, 8 * GR, 128), f32),
            pltpu.VMEM((2 * D, TB), f32),
            pltpu.VMEM((NG, 24, 128), u32),
            pltpu.VMEM((16, TB // 2, D), u32),
            pltpu.VMEM((MEM, D), f32),
            pltpu.VMEM((NP, 8, 3 * PW), f32),
            pltpu.VMEM((NP, 8, PW), f32),
            pltpu.VMEM((8, 128), jnp.int32),
            pltpu.SMEM((1,), jnp.int32),
            pltpu.SemaphoreType.DMA((8 + 5 * NCH + len(WO_CUTS) - 1,)),
        ],
        compiler_params=pltpu.CompilerParams(vmem_limit_bytes=120 * 1024 * 1024),
        name="hedgehog_rmt",
    )(A_x.reshape(S, D), A_wqkv, jnp.transpose(A_w_phi, (1, 2, 0)), A_wo, B_mem0.reshape(MEM, D),
      tr(B_Wq), tr(B_Wk), tr(B_Wv), B_Wo.reshape(HB * DHB, D))
    return out.reshape(1, S, D)
```

```python
import contextlib
import functools

import jax
import jax.numpy as jnp
from jax import lax
import jax.experimental.pallas as pl
import jax.experimental.pallas.tpu as pltpu

f32, bf16, u32 = jnp.float32, jnp.bfloat16, jnp.uint32

S, D = 2048, 640
HA, FA = 32, 20
HB, DHB = 32, 192
MEM, SEG = 8, 32
L = MEM + SEG
NP = HB // 2
PW = 2 * DHB
TB = 128
NG = 16
GR = 2 * FA
NCH = 4
NT = (((1,), (1,)), ((), ()))
LOG2E = 1.4426950408889634
import os
_E = lambda k, d: type(d)(os.environ.get(k, d))
LN_AT = _E('LN_AT', 0)
LN_AT2 = _E('LN_AT2', 4)
NPR = _E('NPR', 1)
LEAD = _E('LEAD', 1)
KSPLIT = _E('KSPLIT', 8)
KB = _E('KB', 3)
PRE1, PRE2 = _E('PRE1', 1), _E('PRE2', 3)
FLIP = [int(v) for v in _E('FLIP', '0,1,2,3,4,13,14,15').split(',') if v]
FLIPM = [int(v) for v in _E('FLIPM', '2').split(',') if v]
ORD_A, ORD_B = _E('OA', 'QSPO'), _E('OB', 'QOPS')
TAIL_A, TAIL_B = _E('TLA', 'OOOSPOOOPOO'), _E('TLB', 'OOSPOOPO')
TAIL_C = _E('TLC', 'OOSPOOPO')
OLAG = _E('OLAG', 4)
OLAG_B = _E('OLAGB', 4)
NLA, NLC = _E('NLA', 3), _E('NLC', 1)
PORD_A = [int(c) for c in _E('PA', '120')]
PORD_B = [int(c) for c in _E('PB', '012')]
ONLYB = _E('ONLYB', 0)
A2MODE = _E('A2MODE', 1)


_scope = lambda name: contextlib.nullcontext()


def _dot(a, b):
    return jnp.dot(a, b, preferred_element_type=f32)


def _dot_nt(a, b):
    return lax.dot_general(a, b, NT, preferred_element_type=f32)


def _pack(x):
    return pltpu.bitcast(x.astype(bf16), u32)


def _unpack(x):
    return pltpu.bitcast(x, bf16)


def _recip(x):
    r = pl.reciprocal(x, approx=True)
    return r * (2.0 - x * r)


def _layernorm(x):
    m = jnp.mean(x, axis=-1, keepdims=True)
    xc = x - m
    v = jnp.mean(xc * xc, axis=-1, keepdims=True)
    return xc * lax.rsqrt(v + 1e-5)


def _iota(shape, dim):
    return lax.broadcasted_iota(jnp.int32, shape, dim)


def _kernel(x_hbm, wqkv_hbm, wphi_hbm, woa_hbm, mem0_hbm, wqt_hbm, wkt_hbm, wvt_hbm, wob_hbm,
            out_hbm,
            x_ref, wqkv_ref, wphi_ref, woa_ref, mem0_ref, out_ref,
            stage_ref, wb_ref, wob_ref, xres_ref, xna_ref, xnb_ref,
            wpqt_ref, wpkt_ref, acc_ref, z_ref, kvt_ref, o_ref,
            mem_ref, svq_ref, pre_ref, svo_ref, flag_ref, cnt_ref, sems):
    WC = HB * DHB // NCH
    X_CUTS = (0, 2 * TB, (2 + KB) * TB, S)

    def cp_wqkv(m):
        return pltpu.make_async_copy(wqkv_hbm.at[:, pl.ds(m * D, D)], wqkv_ref.at[m], sems.at[m])

    def cp_x(n):
        rows = pl.ds(X_CUTS[n], X_CUTS[n + 1] - X_CUTS[n])
        return pltpu.make_async_copy(x_hbm.at[rows, :], x_ref.at[rows, :], sems.at[8 + n])

    def cp_w(m, i):
        rows = pl.ds(pl.multiple_of(i * WC, WC), WC)
        return pltpu.make_async_copy((wqt_hbm, wkt_hbm, wvt_hbm)[m].at[rows, :], stage_ref.at[m, rows, :],
                                     sems.at[11 + NCH * m + i])

    cp_phi = pltpu.make_async_copy(wphi_hbm, wphi_ref, sems.at[3])
    cp_woa = pltpu.make_async_copy(woa_hbm, woa_ref, sems.at[4])
    cp_mem = pltpu.make_async_copy(mem0_hbm, mem0_ref, sems.at[5])
    cp_wob = pltpu.make_async_copy(wob_hbm, stage_ref.at[3], sems.at[6])
    cp_phi.start()
    cp_x(0).start()
    cp_wqkv(1).start()
    cp_wqkv(2).start()
    cp_x(1).start()
    cp_x(2).start()
    cp_wqkv(0).start()
    cp_woa.start()
    cp_mem.start()
    for i in range(NCH):
        for m in range(3):
            cp_w(m, i).start()
    cp_wob.start()

    def phi_blocks():
        wphi = wphi_ref[...].astype(f32)
        cat = jnp.concatenate([wphi[d] for d in range(FA)], axis=1)
        cat = jnp.concatenate([cat, jnp.zeros((32 - FA, D), f32)], axis=0).astype(bf16)
        p_row, p_col = _iota((D, D), 0), _iota((D, D), 1)
        spread = (FA * (p_row & 31) + (p_row >> 5) == p_col).astype(f32).astype(bf16)
        u = _dot(cat, spread).astype(bf16)
        dup = ((_iota((48, 32), 0) >> 1) == _iota((48, 32), 1)).astype(f32).astype(bf16)
        u2 = _dot(dup, u)[:GR]
        lane, par = _iota((GR, 128), 1), _iota((GR, 128), 0) & 1
        lhs = []
        for c in range(5):
            blocks = []
            for g in range(3 * c, 3 * c + 4):
                lo = GR * g - 128 * c + FA * par
                blocks.append(jnp.where((lane >= lo) & (lane < lo + FA), u2[:, 128 * c:128 * c + 128], 0.0))
            lhs.append(jnp.concatenate(blocks, axis=0).astype(bf16))
        return lhs

    def fold_phi(lhs, m, dst):
        parts = [_dot_nt(lhs[c], wqkv_ref[m, :, 128 * c:128 * c + 128]) for c in range(5)]
        rows = []
        for c in range(5):
            first = parts[c][:GR] if c == 0 else parts[c][:GR] + parts[c - 1][3 * GR:]
            rows += [first, parts[c][GR:3 * GR]]
        rows.append(parts[4][3 * GR:])
        dst[...] = _pack(jnp.concatenate(rows, axis=0))

    def fold(x, op):
        r = op(op(op(x[:, 0], x[:, 1]), op(x[:, 2], x[:, 3])), x[:, 4])
        r = op(r, pltpu.roll(r, 2, 1))
        return op(r, pltpu.roll(r, 4, 1))

    def feature_map(pt):
        p = pt.reshape(-1, 5, 8, TB)
        ep = jnp.exp(p - fold(p, jnp.maximum)[:, None])
        en = jnp.exp(fold(p, jnp.minimum)[:, None] - p)
        ep = ep * _recip(fold(ep, jnp.add))[:, None]
        en = en * _recip(fold(en, jnp.add))[:, None]
        return jnp.concatenate([ep, en], axis=1)

    def rows_of(b):
        if isinstance(b, int):
            return pl.ds(b * TB, TB), pl.ds(b * TB // 2, TB // 2)
        return pl.ds(pl.multiple_of(b * TB, TB), TB), pl.ds(pl.multiple_of(b * (TB // 2), TB // 2), TB // 2)

    CG = 4
    NC = NG // CG
    CR = CG * GR

    def k_blocks(blocks, load_x=None, ahead=None, init=False, mid=None):
        xn, v, phi = {}, {}, {}

        def LN(j):
            rows, prows = rows_of(blocks[j] if j < len(blocks) else ahead)
            if load_x is not None and j > 0:
                xn[j] = _layernorm(load_x(rows)).astype(bf16)
                xna_ref[prows, :] = pltpu.bitcast(xn[j], u32)
            else:
                xn[j] = _unpack(xna_ref[prows, :])

        def P(j, c):
            pk = _dot_nt(_unpack(wpkt_ref[c * CR // 2:(c + 1) * CR // 2, :]), xn[j])
            f = feature_map(pk).reshape(2 * CR, TB)
            if init and j == 0:
                z_ref[2 * CR * c:2 * CR * (c + 1), :] = f
            else:
                z_ref[2 * CR * c:2 * CR * (c + 1), :] += f
            phi[j, c] = f

        def V(j, t):
            v[j, t] = _dot(xn[j], wqkv_ref[2, :, 128 * t:128 * t + 128]).astype(bf16)

        def KV(j, t):
            f = jnp.concatenate([phi[j, c] for c in range(NC)], axis=0)[6 * GR * t:6 * GR * t + 8 * GR]
            if j == len(blocks) - 1:
                r = jnp.concatenate([_dot(f[2 * GR * g:2 * GR * (g + 1)].astype(bf16), v[j, t]) for g in range(4)], axis=0)
            else:
                r = _dot(f.astype(bf16), v[j, t])
            if init and j == 0:
                acc_ref[t] = r
            else:
                acc_ref[t] += r

        LN(0)
        for j in range(len(blocks)):
            if j + 1 < len(blocks) or ahead is not None:
                LN(j + 1)
            for c in range(NC):
                P(j, c)
            if mid is not None:
                mid()
            for t in range(5):
                V(j, t)
            for t in range(5):
                KV(j, t)

    def finish_kv():
        pad = jnp.zeros((128 - 2 * GR, 128), f32)
        lane = _iota((2 * GR, 128), 1)
        r48, odd = _iota((48, 128), 0), (_iota((48, 128), 1) & 1) == 1
        same = (((r48 >= FA) & (r48 < GR)) | (r48 >= GR + 4)) == odd
        for g in range(NG):
            lo, hi = GR * g, GR * g + GR
            t0, t1 = lo // 128, (hi - 1) // 128
            blk = lambda t: acc_ref[t, 2 * GR * (g - 3 * t):2 * GR * (g - 3 * t + 1), :]
            z = jnp.sum(z_ref[2 * GR * g:2 * GR * (g + 1), :], axis=1, keepdims=True)
            zc = 120 if lo - 128 * t0 < 8 else 0
            a = jnp.where((lane >= zc) & (lane < zc + 8), z, blk(t0))
            a = jnp.concatenate([a, pad], axis=0).T
            parts = [a[lo - 128 * t0:min(hi - 128 * t0, 128)]]
            if t1 != t0:
                parts.append(jnp.concatenate([blk(t1), pad], axis=0).T[:hi - 128 * t1])
            parts.append(a[zc:zc + 8])
            kvt_ref[g] = _pack(jnp.where(same, jnp.concatenate(parts, axis=0), 0.0))

    def q_blocks(blocks, load_x, between=None, hooks=None):
        top = _iota((8, TB), 0) < 4
        phi, ot, o, y = {}, {}, {}, {}
        n = len(blocks)

        def P(j):
            xn = _unpack(xna_ref[rows_of(blocks[j])[1], :])
            for c in range(NC):
                f = feature_map(_dot_nt(_unpack(wpqt_ref[c * CR // 2:(c + 1) * CR // 2, :]), xn)).reshape(2 * CR, TB)
                for g in range(CG):
                    phi[j, CG * c + g] = f[2 * GR * g:2 * GR * (g + 1)].astype(bf16)

        def N(j):
            outs = []
            for g in range(NG):
                num = _dot(_unpack(kvt_ref[g])[:, :2 * GR], phi[j, g])
                rm = 1.0 / (num[GR:] + 1e-6)
                rs = pltpu.roll(rm, 4, 0)
                r0, r1 = jnp.where(top, rm, rs), jnp.where(top, rs, rm)
                outs.append(num[:GR] * jnp.concatenate([r0, r0, rm, r1, r1], axis=0))
            ot[j] = jnp.concatenate(outs, axis=0)

        def W(j, t):
            if t == 0:
                o_ref[j] = pltpu.bitcast(ot[j].astype(bf16).T, u32)
                o[j] = _unpack(o_ref[j])
            y[j, t] = _dot(o[j], woa_ref[:, 128 * t:128 * t + 128])
            if t == 4:
                rows = rows_of(blocks[j])[0]
                xres_ref[rows, :] = load_x(rows) + jnp.concatenate([y[j, t] for t in range(5)], axis=1)

        def WW(j):
            for t in range(5):
                W(j, t)
            if hooks is not None:
                hooks[j]()

        P(0), P(1)
        if between is not None:
            between()
        N(0), P(2), N(1), WW(0), N(2)
        for j in range(3, n):
            P(j), WW(j - 2), N(j)
        WW(n - 2), WW(n - 1)

    VPERM = [(h * DHB + 64 * c) for c in range(3) for h in range(2)]

    def relayout_weights(j):
        r0 = pl.multiple_of(j * PW, PW)
        for m in range(2):
            wb_ref[j, :, m * PW:(m + 1) * PW] = pltpu.bitcast(stage_ref[m, pl.ds(r0, PW), :].T, u32)
        for c in range(3):
            w = jnp.concatenate([stage_ref[2, pl.ds(pl.multiple_of(r0 + o, 64), 64), :] for o in VPERM[2 * c:2 * c + 2]], axis=0)
            wb_ref[j, :, 2 * PW + 128 * c:2 * PW + 128 * (c + 1)] = pltpu.bitcast(w.T, u32)

    scale = DHB ** -0.5
    NQ = 32
    row, col = _iota((2 * NQ, 2 * L), 0), _iota((2 * NQ, 2 * L), 1)
    same = (row < NQ) == (col < L)
    rr = jnp.where(row < NQ, row, row - NQ)
    kk = jnp.where(col < L, col, col - L)
    keep = same & ((rr < MEM) | (rr >= kk) | (kk >= NQ))
    fill = jnp.where(same, -1e9 / scale, -jnp.inf).astype(f32)
    lo = lambda n, w=128: (_iota((n, w), 1) & 64) == 0
    sub8 = _iota((8, 128), 0)

    def halves(x):
        m = lo(*x.shape)
        return jnp.concatenate([jnp.where(m, x, 0.0), jnp.where(m, 0.0, x)], axis=0).astype(bf16)

    def outer(x):
        return jnp.concatenate([x[:, 0:128], x[:, 256:384]], axis=0).astype(bf16)

    def scores(q, k):
        s1 = _dot_nt(outer(q), outer(k))
        s2 = _dot_nt(q[:, 128:256].astype(bf16), halves(k[:, 128:256]))
        s = s1 + jnp.concatenate([s2, s2], axis=0)
        s = jnp.where(keep, s, fill)
        e = jnp.exp2((s - jnp.max(s, axis=1, keepdims=True)) * (scale * LOG2E))
        return e, jnp.sum(e, axis=1, keepdims=True)

    def values(e, l, v):
        rab = _recip(jnp.where(lo(NQ), l[:NQ], l[NQ:]))
        return _dot((e[:NQ] + e[NQ:]).astype(bf16), halves(v)) * jnp.concatenate([rab] * 3, axis=1)

    def head_attention(q, kv):
        rot = lambda x, r: pltpu.roll(x, r % 8, 0) if r % 8 else x
        tile = lambda x, c: x[:, 128 * c:128 * c + 128]
        q = q * (scale * LOG2E)
        ks = []
        for b in range(2):
            kb = kv[8 * b:8 * b + 8]
            ks.append((tile(kb, 0), jnp.where(lo(8), tile(kb, 1), 0.0), jnp.where(lo(8), 0.0, tile(kb, 1)), tile(kb, 2)))
        ss, m = {}, None
        for r in range(7, -1, -1):
            qr = [rot(tile(q, c), 8 - r) for c in range(3)]
            for b in range(2):
                k0, kl, kh, k2 = ks[b]
                sa = jnp.sum(qr[0] * k0 + qr[1] * kl, axis=1, keepdims=True)
                sb = jnp.sum(qr[2] * k2 + qr[1] * kh, axis=1, keepdims=True)
                x = jnp.where(lo(8), sa, sb)
                if b == 1 and r > 0:
                    x = jnp.where(sub8 <= 7 - r, x, -1e9 * LOG2E)
                ss[b, r] = x
            mx = jnp.maximum(ss[0, r], ss[1, r])
            m = mx if m is None else jnp.maximum(rot(m, 1), mx)
        acc = None
        for r in range(7, -1, -1):
            mr = rot(m, 8 - r)
            e0, e1 = jnp.exp2(ss[0, r] - mr), jnp.exp2(ss[1, r] - mr)
            t = [e0 + e1] + [e0 * tile(kv[0:8], 3 + c) + e1 * tile(kv[8:16], 3 + c) for c in range(3)]
            acc = t if acc is None else [rot(u, 1) + w for u, w in zip(acc, t)]
        r = _recip(acc[0])
        return jnp.concatenate([acc[1] * r, acc[2] * r, acc[3] * r], axis=1)

    def bstep(h, first, never, early, chained_in, chained_out, pre=None):
        qkv, ps, os_, ov = {}, {}, {}, {}
        acc = [None]
        nxt = [0]

        def is_long(first, t, m):
            flipped = m in FLIPM and t in FLIP
            return (flipped and not first) if pre is not None else first != flipped

        def PR(t, ms):
            hs = {m: h if is_long(first, t, m) else h[:NQ] for m in ms}
            if t == 0 and chained_in:
                rs = {}
                for k in range(5):
                    for m in ms:
                        c = _dot(hs[m][:, 128 * k:128 * k + 128].astype(bf16),
                                 _unpack(wb_ref[t, 64 * k:64 * k + 64, m * PW:(m + 1) * PW]))
                        rs[m] = c if k == 0 else rs[m] + c
            else:
                rs = {m: _dot(hs[m].astype(bf16), _unpack(wb_ref[t, :, m * PW:(m + 1) * PW])) for m in ms}
            for m in ms:
                if is_long(first, t, m):
                    svq_ref[t, :, m * PW:(m + 1) * PW] = rs[m][L:]
                    qkv[t, m] = rs[m][:L]
                else:
                    cols = slice(m * PW, (m + 1) * PW)
                    saved = svq_ref[t, :, cols] if pre is None else pre_ref[t, pl.ds(pl.multiple_of(pre * 8, 8), 8), cols]
                    qkv[t, m] = jnp.concatenate([rs[m], saved], axis=0)
            if 2 in ms:
                kv = jnp.concatenate([qkv[t, 1], qkv[t, 2]], axis=1)
                ov[t] = head_attention(qkv[t, 0][NQ:], jnp.concatenate([kv[:MEM], kv[NQ:]], axis=0))

        def SS(j):
            ps[j] = scores(qkv[j, 0][:NQ], qkv[j, 1])

        def PV(j):
            e, l = ps[j]
            if j >= 1:
                e = jnp.concatenate([jnp.where(never, ov[j - 1][:, 128 * c:128 * c + 2 * L], e[8 * c:8 * c + 8])
                                     for c in range(3)] + [e[24:]], axis=0)
            if j in early:
                e = jnp.concatenate([e[:24], jnp.where(never, early[j][:, :2 * L], e[24:32]), e[32:]], axis=0)
            o = values(e, l, qkv[j, 2])
            if first:
                svo_ref[j] = o[24:32]
                o = jnp.concatenate([o[:24], ov[j]], axis=0)
            else:
                o = jnp.concatenate([o, ov[j], svo_ref[j]], axis=0)
            os_[j] = o

        def OO(merge=1):
            js = range(nxt[0], nxt[0] + merge)
            ws = []
            for j in js:
                if pre is not None:
                    ws.append(jnp.concatenate(
                        [pltpu.bitcast(stage_ref[3, j * PW + o:j * PW + o + 64, :], u32) for o in VPERM], axis=0))
                    if not first:
                        wob_ref[j] = ws[-1]
                else:
                    ws.append(wob_ref[j])
            c = _dot(jnp.concatenate([os_[j] for j in js], axis=1).astype(bf16), _unpack(jnp.concatenate(ws, axis=0)))
            acc[0] = c if acc[0] is None else acc[0] + c
            nxt[0] += merge

        order, tail, olag = (ORD_A, TAIL_A, OLAG) if first else (ORD_B, TAIL_C if chained_out else TAIL_B, OLAG_B)
        nl = (NLA if first else NLC) if chained_out else 1
        nd = tail.count("O") + nl
        for t in range(NP):
            for op in order:
                if op == "Q":
                    PR(t, [m for m in (PORD_A if first else PORD_B) if m != 2 or "V" not in order])
                if op == "V" and t >= 1:
                    PR(t - 1, [2])
                if op == "S" and t >= 1:
                    SS(t - 1)
                if op == "P" and t >= 2:
                    PV(t - 2)
                if op == "O" and olag <= t < NP - 1 and nxt[0] < NP - nd:
                    OO()
        p = NP - 2
        for op in tail:
            if op == "O":
                OO()
            if op == "S":
                SS(NP - 1)
            if op == "V":
                PR(NP - 1, [2])
            if op == "P":
                PV(p)
                p += 1
        OO(nl)
        assert nxt[0] == NP and p == NP
        return acc[0]

    def bpass(last, lo_it, hi_it, warm=False):
        def body(i, c):
            never = flag_ref[:, :2 * L] > 0
            probe = lambda x, g: x[8 * g:8 * g + 8, 0:128]
            mem = mem_ref[...]
            if warm:
                slots = [pl.ds(pl.multiple_of(i * 64, 64), 64)]
                heads = [xnb_ref[pl.ds(pl.multiple_of((1 - i) * 64, 64), 8), :]]
            else:
                slots = [pl.ds(0, 64), pl.ds(64, 64)]
            xs = [xnb_ref[sl, :] for sl in slots]
            n = len(slots)
            for u in range(n):
                r0 = pl.multiple_of((i * n + u) * 64, 64)
                xa = xs[u]
                rn = pl.multiple_of(jnp.minimum(r0 + 128, S - 64), 64)
                xn = _layernorm(xres_ref[pl.ds(rn, 64), :])
                xnb_ref[slots[u], :] = xn
                if not warm and u == 0:
                    heads = [xs[1][0:8], xn[0:8]]
                early = {LN_AT + g: probe(xn, g) for g in range(8)}
                if not last:
                    rp = pl.multiple_of(jnp.maximum(r0 - 64, 0), 64)
                    xn = _layernorm(xres_ref[pl.ds(rp, 64), :])
                    xna_ref[pl.ds(pl.multiple_of(rp // 2, 32), 32), :] = _pack(xn)
                    for g in range(8):
                        j = LN_AT2 + g
                        early[j] = jnp.maximum(early[j], probe(xn, g)) if j in early else probe(xn, g)
                ya = bstep(jnp.concatenate([mem, xa[8:32], xa[0:8], xa[32:40]], axis=0), True, never, early,
                           u > 0, True, 2 * i if warm else None)
                yb = bstep(jnp.concatenate([ya[:MEM], xa[40:64], xa[32:40], heads[u]], axis=0), False, never, {},
                           True, u < n - 1, 2 * i + 1 if warm else None)
                mem = yb[:MEM]
                y = xres_ref[pl.ds(r0, 64), :] + jnp.concatenate([ya[24:32], ya[MEM:24], yb[40:48], yb[32:40], yb[MEM:32]], axis=0)
                if last:
                    out_ref[pl.ds(r0, 64), :] = y.astype(bf16)
                else:
                    xres_ref[pl.ds(r0, 64), :] = y
            mem_ref[...] = mem
            if last:
                rows = pl.ds(pl.multiple_of(i * 128, 128), 128)
                pltpu.make_async_copy(out_ref.at[rows, :], out_hbm.at[rows, :], sems.at[7]).start()
            return c
        lax.fori_loop(lo_it, hi_it, body, 0)

    load_in = lambda rows: x_ref[rows, :].astype(f32)
    load_res = lambda rows: xres_ref[rows, :]
    NB = S // (TB * NCH)

    def k1_body(i, c):
        pl.when(i == 1)(lambda: cp_x(2).wait())
        k_blocks([1 + i * KB + j for j in range(KB)], load_in, jnp.minimum(1 + i * KB + KB, S // TB - 1))
        return c

    def q1_body(i, c):
        for m in range(3):
            cp_w(m, i).wait()
        pairs = [i * (NP // NCH) + j for j in range(NP // NCH)]
        for j in pairs:
            relayout_weights(j)
        head = []

        def norm_first():
            x0 = _layernorm(xres_ref[0:128, :])
            xnb_ref[...] = x0
            head.append(jnp.concatenate([x0[32 * sg:32 * sg + 8] for sg in range(4)], axis=0).astype(bf16))

        def project(js):
            for j in js:
                pre_ref[j] = _dot(head[0], _unpack(wb_ref[j]))

        q_blocks([i * NB + j for j in range(NB)], load_in,
                 hooks=[norm_first, lambda: project(pairs[:PRE1]), lambda: project(pairs[PRE1:PRE2]), lambda: project(pairs[PRE2:])])
        return c

    with _scope("pro"):
        flag_ref[...] = jnp.zeros(flag_ref.shape, jnp.int32)
        cnt_ref[0] = 0
        cp_phi.wait()
        cp_x(0).wait()
        phi_lhs = phi_blocks()
        xna_ref[0:TB, :] = _pack(_layernorm(load_in(pl.ds(0, 2 * TB))))
        cp_wqkv(1).wait()
        fold_phi(phi_lhs, 1, wpkt_ref)
        k_blocks([0], init=True, mid=lambda: cp_wqkv(2).wait())
        cp_x(1).wait()
    with _scope("k1"):
        lax.fori_loop(0, (S // TB - 1) // KB, k1_body, 0)
    with _scope("f1"):
        cp_wqkv(0).wait()
        cp_woa.wait()
        cp_mem.wait()
        fold_phi(phi_lhs, 0, wpqt_ref)
        finish_kv()
        mem_ref[...] = mem0_ref[...].astype(f32)
    with _scope("q1"):
        lax.fori_loop(0, NCH, q1_body, 0)
    with _scope("wait"):
        cp_wob.wait()
    with _scope("b1w"):
        bpass(False, 0, 2, warm=True)
    with _scope("b1"):
        bpass(False, 1, S // 128)
    if not ONLYB:
        with _scope("a2"):
            lax.fori_loop(0, cnt_ref[0] + 1, lambda i, c: (k_blocks(list(range(KSPLIT)), init=True), c)[1], 0)
            xna_ref[(S - 64) // 2:, :] = _pack(_layernorm(xres_ref[S - 64:, :]))
            k_blocks(list(range(KSPLIT, 16)))
            q_blocks(list(range(16)), load_res, between=finish_kv)
    with _scope("b2"):
        mem_ref[...] = mem0_ref[...].astype(f32)
        x0 = _layernorm(xres_ref[0:128, :])
        xnb_ref[...] = x0
        for t in FLIP:
            for m in FLIPM:
                svq_ref[t, :, m * PW:(m + 1) * PW] = _dot(x0[0:16].astype(bf16), _unpack(wb_ref[t, :, m * PW:(m + 1) * PW]))[:8]
        bpass(True, 0, S // 128)
    pltpu.make_async_copy(out_ref, out_hbm, sems.at[7]).wait()


@functools.partial(jax.jit, static_argnames=("B_seg_len",))
def pallas_interleave_layers__linear_kernel_hedgehog__memory_aug_recurrent_mem_tr__prompt_kernel(
    A_x: jax.Array,
    A_wqkv: jax.Array,
    A_w_phi: jax.Array,
    A_wo: jax.Array,
    B_x: jax.Array,
    B_mem0: jax.Array,
    B_Wq: jax.Array,
    B_Wk: jax.Array,
    B_Wv: jax.Array,
    B_Wo: jax.Array,
    B_seg_len: int,
):
    del B_x
    assert B_seg_len == SEG
    assert A_x.shape == (1, S, D) and B_mem0.shape == (1, MEM, D)
    assert B_Wq.shape == (D, HB, DHB) and A_w_phi.shape == (HA, FA, FA)
    tr = lambda w: jnp.transpose(w, (1, 2, 0)).reshape(HB * DHB, D)
    hbm = pl.BlockSpec(memory_space=pl.ANY)
    out = pl.pallas_call(
        _kernel,
        out_shape=jax.ShapeDtypeStruct((S, D), bf16),
        in_specs=[hbm] * 9,
        out_specs=hbm,
        scratch_shapes=[
            pltpu.VMEM((S, D), bf16),
            pltpu.VMEM((3, D, D), bf16),
            pltpu.VMEM((FA, FA, HA), bf16),
            pltpu.VMEM((D, D), bf16),
            pltpu.VMEM((MEM, D), bf16),
            pltpu.VMEM((S, D), bf16),
            pltpu.VMEM((4, HB * DHB, D), bf16),
            pltpu.VMEM((NP, D // 2, 3 * PW), u32),
            pltpu.VMEM((NP, PW // 2, D), u32),
            pltpu.VMEM((S, D), f32),
            pltpu.VMEM((S // 2, D), u32),
            pltpu.VMEM((128, D), f32),
            pltpu.VMEM((D // 2, D), u32),
            pltpu.VMEM((D // 2, D), u32),
            pltpu.VMEM((5, 8 * GR, 128), f32),
            pltpu.VMEM((2 * D, TB), f32),
            pltpu.VMEM((NG, 24, 128), u32),
            pltpu.VMEM((16, TB // 2, D), u32),
            pltpu.VMEM((MEM, D), f32),
            pltpu.VMEM((NP, 8, 3 * PW), f32),
            pltpu.VMEM((NP, 32, 3 * PW), f32),
            pltpu.VMEM((NP, 8, PW), f32),
            pltpu.VMEM((8, 128), jnp.int32),
            pltpu.SMEM((1,), jnp.int32),
            pltpu.SemaphoreType.DMA((11 + 3 * NCH,)),
        ],
        compiler_params=pltpu.CompilerParams(vmem_limit_bytes=120 * 1024 * 1024),
        name="hedgehog_rmt",
    )(A_x.reshape(S, D), A_wqkv, jnp.transpose(A_w_phi, (1, 2, 0)), A_wo, B_mem0.reshape(MEM, D),
      tr(B_Wq), tr(B_Wk), tr(B_Wv), B_Wo.reshape(HB * DHB, D))
    return out.reshape(1, S, D)
```

```python
import contextlib
import functools

import jax
import jax.numpy as jnp
from jax import lax
import jax.experimental.pallas as pl
import jax.experimental.pallas.tpu as pltpu

f32, bf16, u32 = jnp.float32, jnp.bfloat16, jnp.uint32

S, D = 2048, 640
HA, FA = 32, 20
HB, DHB = 32, 192
MEM, SEG = 8, 32
L = MEM + SEG
NP = HB // 2
PW = 2 * DHB
TB = 128
NG = 16
GR = 2 * FA
NCH = 4
NT = (((1,), (1,)), ((), ()))
LOG2E = 1.4426950408889634
import os
_E = lambda k, d: type(d)(os.environ.get(k, d))
LN_AT = _E('LN_AT', 0)
LN_AT2 = _E('LN_AT2', 4)
NPR = _E('NPR', 1)
LEAD = _E('LEAD', 1)
KSPLIT = _E('KSPLIT', 8)
KB = _E('KB', 3)
TAIL_W = _E('TLW', 'SOOOOPOOOPOOOOOO')
PRE1, PRE2 = _E('PRE1', 1), _E('PRE2', 3)
FLIP = [int(v) for v in _E('FLIP', '0,1,2,3,4,13,14,15').split(',') if v]
FLIPM = [int(v) for v in _E('FLIPM', '2').split(',') if v]
ORD_A, ORD_B = _E('OA', 'QSPO'), _E('OB', 'QOPS')
TAIL_A, TAIL_B = _E('TLA', 'OOOSPOOOPOO'), _E('TLB', 'OOSPOOPO')
TAIL_C = _E('TLC', 'OOSPOOPO')
OLAG = _E('OLAG', 4)
OLAG_B = _E('OLAGB', 4)
NLA, NLC = _E('NLA', 3), _E('NLC', 1)
PORD_A = [int(c) for c in _E('PA', '120')]
PORD_B = [int(c) for c in _E('PB', '012')]
ONLYB = _E('ONLYB', 0)
A2MODE = _E('A2MODE', 1)


_scope = lambda name: contextlib.nullcontext()


def _dot(a, b):
    return jnp.dot(a, b, preferred_element_type=f32)


def _dot_nt(a, b):
    return lax.dot_general(a, b, NT, preferred_element_type=f32)


def _pack(x):
    return pltpu.bitcast(x.astype(bf16), u32)


def _unpack(x):
    return pltpu.bitcast(x, bf16)


def _recip(x):
    r = pl.reciprocal(x, approx=True)
    return r * (2.0 - x * r)


def _layernorm(x):
    m = jnp.mean(x, axis=-1, keepdims=True)
    xc = x - m
    v = jnp.mean(xc * xc, axis=-1, keepdims=True)
    return xc * lax.rsqrt(v + 1e-5)


def _iota(shape, dim):
    return lax.broadcasted_iota(jnp.int32, shape, dim)


def _kernel(x_hbm, wqkv_hbm, wphi_hbm, woa_hbm, mem0_hbm, wqt_hbm, wkt_hbm, wvt_hbm, wob_hbm,
            out_hbm,
            x_ref, wqkv_ref, wphi_ref, woa_ref, mem0_ref, out_ref,
            stage_ref, wb_ref, wob_ref, xres_ref, xna_ref, xnb_ref,
            wpqt_ref, wpkt_ref, wvt_ref, acc_ref, kvt_ref, o_ref,
            mem_ref, svq_ref, pre_ref, svo_ref, flag_ref, cnt_ref, sems):
    WC = HB * DHB // NCH
    X_CUTS = (0, TB, 2 * TB, (2 + KB) * TB, S)

    def cp_wqkv(m):
        return pltpu.make_async_copy(wqkv_hbm.at[:, pl.ds(m * D, D)], wqkv_ref.at[m], sems.at[m])

    def cp_x(n):
        rows = pl.ds(X_CUTS[n], X_CUTS[n + 1] - X_CUTS[n])
        return pltpu.make_async_copy(x_hbm.at[rows, :], x_ref.at[rows, :], sems.at[8 + n])

    def cp_w(m, i):
        rows = pl.ds(pl.multiple_of(i * WC, WC), WC)
        return pltpu.make_async_copy((wqt_hbm, wkt_hbm, wvt_hbm)[m].at[rows, :], stage_ref.at[m, rows, :],
                                     sems.at[12 + NCH * m + i])

    cp_phi = pltpu.make_async_copy(wphi_hbm, wphi_ref, sems.at[3])
    cp_woa = pltpu.make_async_copy(woa_hbm, woa_ref, sems.at[4])
    cp_mem = pltpu.make_async_copy(mem0_hbm, mem0_ref, sems.at[5])
    cp_wob = pltpu.make_async_copy(wob_hbm, stage_ref.at[3], sems.at[6])
    cp_phi.start()
    cp_x(0).start()
    cp_wqkv(1).start()
    cp_wqkv(2).start()
    cp_x(1).start()
    cp_x(2).start()
    cp_x(3).start()
    cp_wqkv(0).start()
    cp_woa.start()
    cp_mem.start()
    for i in range(NCH):
        for m in range(3):
            cp_w(m, i).start()
    cp_wob.start()

    def phi_blocks():
        wphi = wphi_ref[...].astype(f32)
        cat = jnp.concatenate([wphi[d] for d in range(FA)], axis=1)
        cat = jnp.concatenate([cat, jnp.zeros((32 - FA, D), f32)], axis=0).astype(bf16)
        p_row, p_col = _iota((D, D), 0), _iota((D, D), 1)
        spread = (FA * (p_row & 31) + (p_row >> 5) == p_col).astype(f32).astype(bf16)
        u = _dot(cat, spread).astype(bf16)
        dup = ((_iota((48, 32), 0) >> 1) == _iota((48, 32), 1)).astype(f32).astype(bf16)
        u2 = _dot(dup, u)[:GR]
        lane, par = _iota((GR, 128), 1), _iota((GR, 128), 0) & 1
        lhs = []
        for c in range(5):
            blocks = []
            for g in range(3 * c, 3 * c + 4):
                lo = GR * g - 128 * c + FA * par
                blocks.append(jnp.where((lane >= lo) & (lane < lo + FA), u2[:, 128 * c:128 * c + 128], 0.0))
            lhs.append(jnp.concatenate(blocks, axis=0).astype(bf16))
        return lhs

    def fold_phi(lhs, m, dst):
        parts = [_dot_nt(lhs[c], wqkv_ref[m, :, 128 * c:128 * c + 128]) for c in range(5)]
        rows = []
        for c in range(5):
            first = parts[c][:GR] if c == 0 else parts[c][:GR] + parts[c - 1][3 * GR:]
            rows += [first, parts[c][GR:3 * GR]]
        rows.append(parts[4][3 * GR:])
        dst[...] = _pack(jnp.concatenate(rows, axis=0))

    def fold(x, op):
        r = op(op(op(x[:, 0], x[:, 1]), op(x[:, 2], x[:, 3])), x[:, 4])
        r = op(r, pltpu.roll(r, 2, 1))
        return op(r, pltpu.roll(r, 4, 1))

    def feature_map(pt):
        p = pt.reshape(-1, 5, 8, TB)
        ep = jnp.exp(p - fold(p, jnp.maximum)[:, None])
        en = jnp.exp(fold(p, jnp.minimum)[:, None] - p)
        ep = ep * _recip(fold(ep, jnp.add))[:, None]
        en = en * _recip(fold(en, jnp.add))[:, None]
        return jnp.concatenate([ep, en], axis=1)

    def rows_of(b):
        if isinstance(b, int):
            return pl.ds(b * TB, TB), pl.ds(b * TB // 2, TB // 2)
        return pl.ds(pl.multiple_of(b * TB, TB), TB), pl.ds(pl.multiple_of(b * (TB // 2), TB // 2), TB // 2)

    CG = 4
    NC = NG // CG
    CR = CG * GR

    def k_blocks(blocks, load_x=None, ahead=None, init=False, mid=None):
        xn, v, phi = {}, {}, {}

        def LN(j):
            rows, prows = rows_of(blocks[j] if j < len(blocks) else ahead)
            if load_x is not None and j > 0:
                xn[j] = _layernorm(load_x(rows)).astype(bf16)
                xna_ref[prows, :] = pltpu.bitcast(xn[j], u32)
            else:
                xn[j] = _unpack(xna_ref[prows, :])

        def P(j, c):
            pk = _dot_nt(_unpack(wpkt_ref[c * CR // 2:(c + 1) * CR // 2, :]), xn[j])
            f = feature_map(pk).reshape(2 * CR, TB)
            for g in range(CG):
                phi[j, CG * c + g] = f[2 * GR * g:2 * GR * (g + 1)].astype(bf16)

        def V(j, c):
            vt = _dot_nt(_unpack(wvt_ref[c * CR // 2:(c + 1) * CR // 2, :]), xn[j])
            for g in range(CG):
                v[j, CG * c + g] = jnp.concatenate([vt[GR * g:GR * (g + 1)], jnp.ones((8, TB), f32)], axis=0).astype(bf16)

        def KV(j):
            for g in range(NG):
                r = _dot_nt(v[j, g], phi[j, g])
                if init and j == 0:
                    acc_ref[g] = r
                else:
                    acc_ref[g] += r

        LN(0)
        for j in range(len(blocks)):
            if j + 1 < len(blocks) or ahead is not None:
                LN(j + 1)
            for c in range(NC):
                P(j, c)
            if mid is not None:
                mid()
            for c in range(NC):
                V(j, c)
            KV(j)

    def finish_kv():
        r48, odd = _iota((48, 2 * GR), 0), (_iota((48, 2 * GR), 1) & 1) == 1
        same = (((r48 >= FA) & (r48 < GR)) | (r48 >= GR + 4)) == odd
        for g in range(NG):
            kvt_ref[g] = _pack(jnp.where(same, acc_ref[g], 0.0))

    def q_blocks(blocks, load_x, between=None, hooks=None):
        top = _iota((8, TB), 0) < 4
        phi, ot, o, y = {}, {}, {}, {}
        n = len(blocks)

        def P(j):
            xn = _unpack(xna_ref[rows_of(blocks[j])[1], :])
            for c in range(NC):
                f = feature_map(_dot_nt(_unpack(wpqt_ref[c * CR // 2:(c + 1) * CR // 2, :]), xn)).reshape(2 * CR, TB)
                for g in range(CG):
                    phi[j, CG * c + g] = f[2 * GR * g:2 * GR * (g + 1)].astype(bf16)

        def N(j):
            outs = []
            for g in range(NG):
                num = _dot(_unpack(kvt_ref[g]), phi[j, g])
                rm = 1.0 / (num[GR:] + 1e-6)
                rs = pltpu.roll(rm, 4, 0)
                r0, r1 = jnp.where(top, rm, rs), jnp.where(top, rs, rm)
                outs.append(num[:GR] * jnp.concatenate([r0, r0, rm, r1, r1], axis=0))
            ot[j] = jnp.concatenate(outs, axis=0)

        def W(j, t):
            if t == 0:
                o_ref[j] = pltpu.bitcast(ot[j].astype(bf16).T, u32)
                o[j] = _unpack(o_ref[j])
            y[j, t] = _dot(o[j], woa_ref[:, 128 * t:128 * t + 128])
            if t == 4:
                rows = rows_of(blocks[j])[0]
                xres_ref[rows, :] = load_x(rows) + jnp.concatenate([y[j, t] for t in range(5)], axis=1)

        def WW(j):
            for t in range(5):
                W(j, t)
            if hooks is not None:
                hooks[j]()

        P(0), P(1)
        if between is not None:
            between()
        N(0), P(2), N(1), WW(0), N(2)
        for j in range(3, n):
            P(j), WW(j - 2), N(j)
        WW(n - 2), WW(n - 1)

    VPERM = [(h * DHB + 64 * c) for c in range(3) for h in range(2)]

    def relayout_weights(j):
        r0 = pl.multiple_of(j * PW, PW)
        for m in range(2):
            wb_ref[j, :, m * PW:(m + 1) * PW] = pltpu.bitcast(stage_ref[m, pl.ds(r0, PW), :].T, u32)
        for c in range(3):
            w = jnp.concatenate([stage_ref[2, pl.ds(pl.multiple_of(r0 + o, 64), 64), :] for o in VPERM[2 * c:2 * c + 2]], axis=0)
            wb_ref[j, :, 2 * PW + 128 * c:2 * PW + 128 * (c + 1)] = pltpu.bitcast(w.T, u32)

    scale = DHB ** -0.5
    NQ = 32
    row, col = _iota((2 * NQ, 2 * L), 0), _iota((2 * NQ, 2 * L), 1)
    same = (row < NQ) == (col < L)
    rr = jnp.where(row < NQ, row, row - NQ)
    kk = jnp.where(col < L, col, col - L)
    keep = same & ((rr < MEM) | (rr >= kk) | (kk >= NQ))
    fill = jnp.where(same, -1e9 / scale, -jnp.inf).astype(f32)
    lo = lambda n, w=128: (_iota((n, w), 1) & 64) == 0
    sub8 = _iota((8, 128), 0)

    def halves(x):
        m = lo(*x.shape)
        return jnp.concatenate([jnp.where(m, x, 0.0), jnp.where(m, 0.0, x)], axis=0).astype(bf16)

    def outer(x):
        return jnp.concatenate([x[:, 0:128], x[:, 256:384]], axis=0).astype(bf16)

    def scores(q, k):
        s1 = _dot_nt(outer(q), outer(k))
        s2 = _dot_nt(q[:, 128:256].astype(bf16), halves(k[:, 128:256]))
        s = s1 + jnp.concatenate([s2, s2], axis=0)
        s = jnp.where(keep, s, fill)
        e = jnp.exp2((s - jnp.max(s, axis=1, keepdims=True)) * (scale * LOG2E))
        return e, jnp.sum(e, axis=1, keepdims=True)

    def values(e, l, v):
        rab = _recip(jnp.where(lo(NQ), l[:NQ], l[NQ:]))
        return _dot((e[:NQ] + e[NQ:]).astype(bf16), halves(v)) * jnp.concatenate([rab] * 3, axis=1)

    def head_attention(q, kv):
        rot = lambda x, r: pltpu.roll(x, r % 8, 0) if r % 8 else x
        tile = lambda x, c: x[:, 128 * c:128 * c + 128]
        q = q * (scale * LOG2E)
        ks = []
        for b in range(2):
            kb = kv[8 * b:8 * b + 8]
            ks.append((tile(kb, 0), jnp.where(lo(8), tile(kb, 1), 0.0), jnp.where(lo(8), 0.0, tile(kb, 1)), tile(kb, 2)))
        ss, m = {}, None
        for r in range(7, -1, -1):
            qr = [rot(tile(q, c), 8 - r) for c in range(3)]
            for b in range(2):
                k0, kl, kh, k2 = ks[b]
                sa = jnp.sum(qr[0] * k0 + qr[1] * kl, axis=1, keepdims=True)
                sb = jnp.sum(qr[2] * k2 + qr[1] * kh, axis=1, keepdims=True)
                x = jnp.where(lo(8), sa, sb)
                if b == 1 and r > 0:
                    x = jnp.where(sub8 <= 7 - r, x, -1e9 * LOG2E)
                ss[b, r] = x
            mx = jnp.maximum(ss[0, r], ss[1, r])
            m = mx if m is None else jnp.maximum(rot(m, 1), mx)
        acc = None
        for r in range(7, -1, -1):
            mr = rot(m, 8 - r)
            e0, e1 = jnp.exp2(ss[0, r] - mr), jnp.exp2(ss[1, r] - mr)
            t = [e0 + e1] + [e0 * tile(kv[0:8], 3 + c) + e1 * tile(kv[8:16], 3 + c) for c in range(3)]
            acc = t if acc is None else [rot(u, 1) + w for u, w in zip(acc, t)]
        r = _recip(acc[0])
        return jnp.concatenate([acc[1] * r, acc[2] * r, acc[3] * r], axis=1)

    def bstep(h, first, never, early, chained_in, chained_out, pre=None):
        qkv, ps, os_, ov = {}, {}, {}, {}
        acc = [None]
        nxt = [0]

        split = pre is not None and first

        def is_long(first, t, m):
            flipped = m in FLIPM and t in FLIP
            return (flipped and not first) if pre is not None else first != flipped

        def PR(t, ms):
            hs = {m: h if is_long(first, t, m) else h[:NQ] for m in ms}
            if t == 0 and chained_in:
                rs = {}
                for k in range(5):
                    for m in ms:
                        c = _dot(hs[m][:, 128 * k:128 * k + 128].astype(bf16),
                                 _unpack(wb_ref[t, 64 * k:64 * k + 64, m * PW:(m + 1) * PW]))
                        rs[m] = c if k == 0 else rs[m] + c
            else:
                rs = {m: _dot(hs[m].astype(bf16), _unpack(wb_ref[t, :, m * PW:(m + 1) * PW])) for m in ms}
            for m in ms:
                if is_long(first, t, m):
                    svq_ref[t, :, m * PW:(m + 1) * PW] = rs[m][L:]
                    qkv[t, m] = rs[m][:L]
                else:
                    cols = slice(m * PW, (m + 1) * PW)
                    saved = svq_ref[t, :, cols] if pre is None else pre_ref[t, pl.ds(pl.multiple_of(pre * 8, 8), 8), cols]
                    qkv[t, m] = jnp.concatenate([rs[m], saved], axis=0)
            if 2 in ms and not (split and t >= NP - 2):
                HA_(t)

        def HA_(t):
            kv = jnp.concatenate([qkv[t, 1], qkv[t, 2]], axis=1)
            ov[t] = head_attention(qkv[t, 0][NQ:], jnp.concatenate([kv[:MEM], kv[NQ:]], axis=0))

        def SS(j):
            ps[j] = scores(qkv[j, 0][:NQ], qkv[j, 1])

        def PV(j):
            e, l = ps[j]
            if j >= 1:
                e = jnp.concatenate([jnp.where(never, ov[j - 1][:, 128 * c:128 * c + 2 * L], e[8 * c:8 * c + 8])
                                     for c in range(3)] + [e[24:]], axis=0)
            if j in early:
                e = jnp.concatenate([e[:24], jnp.where(never, early[j][:, :2 * L], e[24:32]), e[32:]], axis=0)
            o = values(e, l, qkv[j, 2])
            if first:
                svo_ref[j] = o[24:32]
                o = jnp.concatenate([o[:24], ov[j]], axis=0)
            else:
                o = jnp.concatenate([o, ov[j], svo_ref[j]], axis=0)
            os_[j] = o

        def OO(merge=1):
            js = range(nxt[0], nxt[0] + merge)
            ws = []
            for j in js:
                if pre is not None:
                    ws.append(jnp.concatenate(
                        [pltpu.bitcast(stage_ref[3, j * PW + o:j * PW + o + 64, :], u32) for o in VPERM], axis=0))
                    if not first:
                        wob_ref[j] = ws[-1]
                else:
                    ws.append(wob_ref[j])
            c = _dot(jnp.concatenate([os_[j] for j in js], axis=1).astype(bf16), _unpack(jnp.concatenate(ws, axis=0)))
            acc[0] = c if acc[0] is None else acc[0] + c
            nxt[0] += merge

        order, tail, olag = (ORD_A, TAIL_A, OLAG) if first else (ORD_B, TAIL_C if chained_out else TAIL_B, OLAG_B)
        nl = (NLA if first else NLC) if chained_out else 1
        if split:
            tail = TAIL_W
        nd = tail.count("O") + nl
        for t in range(NP):
            for op in order:
                if op == "Q":
                    PR(t, [m for m in (PORD_A if first else PORD_B) if m != 2 or "V" not in order])
                    if split and t == NP - 1:
                        pl.when(pre == 0)(lambda: cp_wob.wait())
                        HA_(NP - 2), HA_(NP - 1)
                if op == "V" and t >= 1:
                    PR(t - 1, [2])
                if op == "S" and t >= 1:
                    SS(t - 1)
                if op == "P" and t >= 2:
                    PV(t - 2)
                if op == "O" and olag <= t < NP - 1 and nxt[0] < NP - nd:
                    OO()
        p = NP - 2
        for op in tail:
            if op == "O":
                OO()
            if op == "S":
                SS(NP - 1)
            if op == "V":
                PR(NP - 1, [2])
            if op == "P":
                PV(p)
                p += 1
        OO(nl)
        assert nxt[0] == NP and p == NP
        return acc[0]

    def bpass(last, lo_it, hi_it, warm=False):
        def body(i, c):
            never = flag_ref[:, :2 * L] > 0
            probe = lambda x, g: x[8 * g:8 * g + 8, 0:128]
            mem = mem_ref[...]
            if warm:
                slots = [pl.ds(pl.multiple_of(i * 64, 64), 64)]
                heads = [xnb_ref[pl.ds(pl.multiple_of((1 - i) * 64, 64), 8), :]]
            else:
                slots = [pl.ds(0, 64), pl.ds(64, 64)]
            xs = [xnb_ref[sl, :] for sl in slots]
            n = len(slots)
            for u in range(n):
                r0 = pl.multiple_of((i * n + u) * 64, 64)
                xa = xs[u]
                rn = pl.multiple_of(jnp.minimum(r0 + 128, S - 64), 64)
                xn = _layernorm(xres_ref[pl.ds(rn, 64), :])
                xnb_ref[slots[u], :] = xn
                if not warm and u == 0:
                    heads = [xs[1][0:8], xn[0:8]]
                early = {LN_AT + g: probe(xn, g) for g in range(8)}
                if not last:
                    rp = pl.multiple_of(jnp.maximum(r0 - 64, 0), 64)
                    xn = _layernorm(xres_ref[pl.ds(rp, 64), :])
                    xna_ref[pl.ds(pl.multiple_of(rp // 2, 32), 32), :] = _pack(xn)
                    for g in range(8):
                        j = LN_AT2 + g
                        early[j] = jnp.maximum(early[j], probe(xn, g)) if j in early else probe(xn, g)
                ya = bstep(jnp.concatenate([mem, xa[8:32], xa[0:8], xa[32:40]], axis=0), True, never, early,
                           u > 0, True, 2 * i if warm else None)
                yb = bstep(jnp.concatenate([ya[:MEM], xa[40:64], xa[32:40], heads[u]], axis=0), False, never, {},
                           True, u < n - 1, 2 * i + 1 if warm else None)
                mem = yb[:MEM]
                y = xres_ref[pl.ds(r0, 64), :] + jnp.concatenate([ya[24:32], ya[MEM:24], yb[40:48], yb[32:40], yb[MEM:32]], axis=0)
                if last:
                    out_ref[pl.ds(r0, 64), :] = y.astype(bf16)
                else:
                    xres_ref[pl.ds(r0, 64), :] = y
            mem_ref[...] = mem
            if last:
                rows = pl.ds(pl.multiple_of(i * 128, 128), 128)
                pltpu.make_async_copy(out_ref.at[rows, :], out_hbm.at[rows, :], sems.at[7]).start()
            return c
        lax.fori_loop(lo_it, hi_it, body, 0)

    load_in = lambda rows: x_ref[rows, :].astype(f32)
    load_res = lambda rows: xres_ref[rows, :]
    NB = S // (TB * NCH)

    def k1_body(i, c):
        pl.when(i == 1)(lambda: cp_x(3).wait())
        k_blocks([1 + i * KB + j for j in range(KB)], load_in, jnp.minimum(1 + i * KB + KB, S // TB - 1))
        return c

    def q1_body(i, c):
        for m in range(3):
            cp_w(m, i).wait()
        pairs = [i * (NP // NCH) + j for j in range(NP // NCH)]
        for j in pairs:
            relayout_weights(j)
        head = []

        def norm_first():
            x0 = _layernorm(xres_ref[0:128, :])
            xnb_ref[...] = x0
            head.append(jnp.concatenate([x0[32 * sg:32 * sg + 8] for sg in range(4)], axis=0).astype(bf16))

        def project(js):
            for j in js:
                pre_ref[j] = _dot(head[0], _unpack(wb_ref[j]))

        q_blocks([i * NB + j for j in range(NB)], load_in,
                 hooks=[norm_first, lambda: project(pairs[:PRE1]), lambda: project(pairs[PRE1:PRE2]), lambda: project(pairs[PRE2:])])
        return c

    with _scope("pro"):
        flag_ref[...] = jnp.zeros(flag_ref.shape, jnp.int32)
        cnt_ref[0] = 0
        cp_phi.wait()
        cp_x(0).wait()
        phi_lhs = phi_blocks()
        xna_ref[0:TB // 2, :] = _pack(_layernorm(load_in(pl.ds(0, TB))))
        cp_wqkv(1).wait()
        fold_phi(phi_lhs, 1, wpkt_ref)

        def values_ready():
            cp_wqkv(2).wait()
            cp_x(1).wait()
            wvt_ref[...] = pltpu.bitcast(wqkv_ref[2].T, u32)
            xna_ref[TB // 2:TB, :] = _pack(_layernorm(load_in(pl.ds(TB, TB))))

        k_blocks([0], init=True, mid=values_ready)
        cp_x(2).wait()
    with _scope("k1"):
        lax.fori_loop(0, (S // TB - 1) // KB, k1_body, 0)
    with _scope("f1"):
        cp_wqkv(0).wait()
        cp_woa.wait()
        cp_mem.wait()
        fold_phi(phi_lhs, 0, wpqt_ref)
        finish_kv()
        mem_ref[...] = mem0_ref[...].astype(f32)
    with _scope("q1"):
        lax.fori_loop(0, NCH, q1_body, 0)
    with _scope("b1w"):
        bpass(False, 0, 2, warm=True)
    with _scope("b1"):
        bpass(False, 1, S // 128)
    if not ONLYB:
        with _scope("a2"):
            lax.fori_loop(0, cnt_ref[0] + 1, lambda i, c: (k_blocks(list(range(KSPLIT)), init=True), c)[1], 0)
            xna_ref[(S - 64) // 2:, :] = _pack(_layernorm(xres_ref[S - 64:, :]))
            k_blocks(list(range(KSPLIT, 16)))
            q_blocks(list(range(16)), load_res, between=finish_kv)
    with _scope("b2"):
        mem_ref[...] = mem0_ref[...].astype(f32)
        x0 = _layernorm(xres_ref[0:128, :])
        xnb_ref[...] = x0
        for t in FLIP:
            for m in FLIPM:
                svq_ref[t, :, m * PW:(m + 1) * PW] = _dot(x0[0:16].astype(bf16), _unpack(wb_ref[t, :, m * PW:(m + 1) * PW]))[:8]
        bpass(True, 0, S // 128)
    pltpu.make_async_copy(out_ref, out_hbm, sems.at[7]).wait()


@functools.partial(jax.jit, static_argnames=("B_seg_len",))
def pallas_interleave_layers__linear_kernel_hedgehog__memory_aug_recurrent_mem_tr__prompt_kernel(
    A_x: jax.Array,
    A_wqkv: jax.Array,
    A_w_phi: jax.Array,
    A_wo: jax.Array,
    B_x: jax.Array,
    B_mem0: jax.Array,
    B_Wq: jax.Array,
    B_Wk: jax.Array,
    B_Wv: jax.Array,
    B_Wo: jax.Array,
    B_seg_len: int,
):
    del B_x
    assert B_seg_len == SEG
    assert A_x.shape == (1, S, D) and B_mem0.shape == (1, MEM, D)
    assert B_Wq.shape == (D, HB, DHB) and A_w_phi.shape == (HA, FA, FA)
    tr = lambda w: jnp.transpose(w, (1, 2, 0)).reshape(HB * DHB, D)
    hbm = pl.BlockSpec(memory_space=pl.ANY)
    out = pl.pallas_call(
        _kernel,
        out_shape=jax.ShapeDtypeStruct((S, D), bf16),
        in_specs=[hbm] * 9,
        out_specs=hbm,
        scratch_shapes=[
            pltpu.VMEM((S, D), bf16),
            pltpu.VMEM((3, D, D), bf16),
            pltpu.VMEM((FA, FA, HA), bf16),
            pltpu.VMEM((D, D), bf16),
            pltpu.VMEM((MEM, D), bf16),
            pltpu.VMEM((S, D), bf16),
            pltpu.VMEM((4, HB * DHB, D), bf16),
            pltpu.VMEM((NP, D // 2, 3 * PW), u32),
            pltpu.VMEM((NP, PW // 2, D), u32),
            pltpu.VMEM((S, D), f32),
            pltpu.VMEM((S // 2, D), u32),
            pltpu.VMEM((128, D), f32),
            pltpu.VMEM((D // 2, D), u32),
            pltpu.VMEM((D // 2, D), u32),
            pltpu.VMEM((D // 2, D), u32),
            pltpu.VMEM((NG, 48, 2 * GR), f32),
            pltpu.VMEM((NG, 24, 2 * GR), u32),
            pltpu.VMEM((16, TB // 2, D), u32),
            pltpu.VMEM((MEM, D), f32),
            pltpu.VMEM((NP, 8, 3 * PW), f32),
            pltpu.VMEM((NP, 32, 3 * PW), f32),
            pltpu.VMEM((NP, 8, PW), f32),
            pltpu.VMEM((8, 128), jnp.int32),
            pltpu.SMEM((1,), jnp.int32),
            pltpu.SemaphoreType.DMA((12 + 3 * NCH,)),
        ],
        compiler_params=pltpu.CompilerParams(vmem_limit_bytes=120 * 1024 * 1024),
        name="hedgehog_rmt",
    )(A_x.reshape(S, D), A_wqkv, jnp.transpose(A_w_phi, (1, 2, 0)), A_wo, B_mem0.reshape(MEM, D),
      tr(B_Wq), tr(B_Wk), tr(B_Wv), B_Wo.reshape(HB * DHB, D))
    return out.reshape(1, S, D)
```

```python
import contextlib
import functools

import jax
import jax.numpy as jnp
from jax import lax
import jax.experimental.pallas as pl
import jax.experimental.pallas.tpu as pltpu

f32, bf16, u32 = jnp.float32, jnp.bfloat16, jnp.uint32

S, D = 2048, 640
HA, FA = 32, 20
HB, DHB = 32, 192
MEM, SEG = 8, 32
L = MEM + SEG
NP = HB // 2
PW = 2 * DHB
TB = 128
NG = 16
GR = 2 * FA
NCH = 4
NT = (((1,), (1,)), ((), ()))
LOG2E = 1.4426950408889634

FLIP, FLIPM = (0, 1, 2, 3, 4, 13, 14, 15), (2,)
ORD_A, ORD_B = "QSPO", "QOPS"
TAIL_A, TAIL_B, TAIL_W = "OOOSPOOOPOO", "OOSPOOPO", "SOOOOPOOOPOOOOOO"
PORD_A, PORD_B = (1, 2, 0), (0, 1, 2)
OLAG = 4
LN_AT, LN_AT2 = 0, 4
KB = 3
KSPLIT = 8


_scope = lambda name: contextlib.nullcontext()


def _dot(a, b):
    return jnp.dot(a, b, preferred_element_type=f32)


def _dot_nt(a, b):
    return lax.dot_general(a, b, NT, preferred_element_type=f32)


def _pack(x):
    return pltpu.bitcast(x.astype(bf16), u32)


def _unpack(x):
    return pltpu.bitcast(x, bf16)


def _recip(x):
    r = pl.reciprocal(x, approx=True)
    return r * (2.0 - x * r)


def _layernorm(x):
    m = jnp.mean(x, axis=-1, keepdims=True)
    xc = x - m
    v = jnp.mean(xc * xc, axis=-1, keepdims=True)
    return xc * lax.rsqrt(v + 1e-5)


def _iota(shape, dim):
    return lax.broadcasted_iota(jnp.int32, shape, dim)


def _kernel(x_hbm, wqkv_hbm, wphi_hbm, woa_hbm, mem0_hbm, wqt_hbm, wkt_hbm, wvt_hbm, wob_hbm,
            out_hbm,
            x_ref, wqkv_ref, wphi_ref, woa_ref, mem0_ref, out_ref,
            stage_ref, wb_ref, wob_ref, xres_ref, xna_ref, xnb_ref,
            wpqt_ref, wpkt_ref, wvt_ref, acc_ref, kvt_ref, o_ref,
            mem_ref, svq_ref, pre_ref, svo_ref, flag_ref, cnt_ref, sems):
    WC = HB * DHB // NCH
    X_CUTS = (0, TB, 2 * TB, (2 + KB) * TB, S)

    def cp_wqkv(m):
        return pltpu.make_async_copy(wqkv_hbm.at[:, pl.ds(m * D, D)], wqkv_ref.at[m], sems.at[m])

    def cp_x(n):
        rows = pl.ds(X_CUTS[n], X_CUTS[n + 1] - X_CUTS[n])
        return pltpu.make_async_copy(x_hbm.at[rows, :], x_ref.at[rows, :], sems.at[8 + n])

    def cp_w(m, i):
        rows = pl.ds(pl.multiple_of(i * WC, WC), WC)
        return pltpu.make_async_copy((wqt_hbm, wkt_hbm, wvt_hbm)[m].at[rows, :], stage_ref.at[m, rows, :],
                                     sems.at[12 + NCH * m + i])

    cp_phi = pltpu.make_async_copy(wphi_hbm, wphi_ref, sems.at[3])
    cp_woa = pltpu.make_async_copy(woa_hbm, woa_ref, sems.at[4])
    cp_mem = pltpu.make_async_copy(mem0_hbm, mem0_ref, sems.at[5])
    cp_wob = pltpu.make_async_copy(wob_hbm, stage_ref.at[3], sems.at[6])
    cp_phi.start()
    cp_x(0).start()
    cp_wqkv(1).start()
    cp_wqkv(2).start()
    cp_x(1).start()
    cp_x(2).start()
    cp_x(3).start()
    cp_wqkv(0).start()
    cp_woa.start()
    cp_mem.start()
    for i in range(NCH):
        for m in range(3):
            cp_w(m, i).start()
    cp_wob.start()

    def phi_blocks():
        wphi = wphi_ref[...].astype(f32)
        cat = jnp.concatenate([wphi[d] for d in range(FA)], axis=1)
        cat = jnp.concatenate([cat, jnp.zeros((32 - FA, D), f32)], axis=0).astype(bf16)
        p_row, p_col = _iota((D, D), 0), _iota((D, D), 1)
        spread = (FA * (p_row & 31) + (p_row >> 5) == p_col).astype(f32).astype(bf16)
        u = _dot(cat, spread).astype(bf16)
        dup = ((_iota((48, 32), 0) >> 1) == _iota((48, 32), 1)).astype(f32).astype(bf16)
        u2 = _dot(dup, u)[:GR]
        lane, par = _iota((GR, 128), 1), _iota((GR, 128), 0) & 1
        lhs = []
        for c in range(5):
            blocks = []
            for g in range(3 * c, 3 * c + 4):
                lo = GR * g - 128 * c + FA * par
                blocks.append(jnp.where((lane >= lo) & (lane < lo + FA), u2[:, 128 * c:128 * c + 128], 0.0))
            lhs.append(jnp.concatenate(blocks, axis=0).astype(bf16))
        return lhs

    def fold_phi(lhs, m, dst):
        parts = [_dot_nt(lhs[c], wqkv_ref[m, :, 128 * c:128 * c + 128]) for c in range(5)]
        rows = []
        for c in range(5):
            first = parts[c][:GR] if c == 0 else parts[c][:GR] + parts[c - 1][3 * GR:]
            rows += [first, parts[c][GR:3 * GR]]
        rows.append(parts[4][3 * GR:])
        dst[...] = _pack(jnp.concatenate(rows, axis=0))

    def fold(x, op):
        r = op(op(op(x[:, 0], x[:, 1]), op(x[:, 2], x[:, 3])), x[:, 4])
        r = op(r, pltpu.roll(r, 2, 1))
        return op(r, pltpu.roll(r, 4, 1))

    def feature_map(pt):
        p = pt.reshape(-1, 5, 8, TB)
        ep = jnp.exp(p - fold(p, jnp.maximum)[:, None])
        en = jnp.exp(fold(p, jnp.minimum)[:, None] - p)
        ep = ep * _recip(fold(ep, jnp.add))[:, None]
        en = en * _recip(fold(en, jnp.add))[:, None]
        return jnp.concatenate([ep, en], axis=1)

    def rows_of(b):
        if isinstance(b, int):
            return pl.ds(b * TB, TB), pl.ds(b * TB // 2, TB // 2)
        return pl.ds(pl.multiple_of(b * TB, TB), TB), pl.ds(pl.multiple_of(b * (TB // 2), TB // 2), TB // 2)

    CG = 4
    NC = NG // CG
    CR = CG * GR

    def k_blocks(blocks, load_x=None, ahead=None, init=False, mid=None):
        xn, v, phi = {}, {}, {}

        def LN(j):
            rows, prows = rows_of(blocks[j] if j < len(blocks) else ahead)
            if load_x is not None and j > 0:
                xn[j] = _layernorm(load_x(rows)).astype(bf16)
                xna_ref[prows, :] = pltpu.bitcast(xn[j], u32)
            else:
                xn[j] = _unpack(xna_ref[prows, :])

        def P(j, c):
            pk = _dot_nt(_unpack(wpkt_ref[c * CR // 2:(c + 1) * CR // 2, :]), xn[j])
            f = feature_map(pk).reshape(2 * CR, TB)
            for g in range(CG):
                phi[j, CG * c + g] = f[2 * GR * g:2 * GR * (g + 1)].astype(bf16)

        def V(j, c):
            vt = _dot_nt(_unpack(wvt_ref[c * CR // 2:(c + 1) * CR // 2, :]), xn[j])
            for g in range(CG):
                v[j, CG * c + g] = jnp.concatenate([vt[GR * g:GR * (g + 1)], jnp.ones((8, TB), f32)], axis=0).astype(bf16)

        def KV(j):
            for g in range(NG):
                r = _dot_nt(v[j, g], phi[j, g])
                if init and j == 0:
                    acc_ref[g] = r
                else:
                    acc_ref[g] += r

        LN(0)
        for j in range(len(blocks)):
            if j + 1 < len(blocks) or ahead is not None:
                LN(j + 1)
            for c in range(NC):
                P(j, c)
            if mid is not None:
                mid()
            for c in range(NC):
                V(j, c)
            KV(j)

    def finish_kv():
        r48, odd = _iota((48, 2 * GR), 0), (_iota((48, 2 * GR), 1) & 1) == 1
        same = (((r48 >= FA) & (r48 < GR)) | (r48 >= GR + 4)) == odd
        for g in range(NG):
            kvt_ref[g] = _pack(jnp.where(same, acc_ref[g], 0.0))

    def q_blocks(blocks, load_x, between=None, hooks=None):
        top = _iota((8, TB), 0) < 4
        phi, ot, o, y = {}, {}, {}, {}
        n = len(blocks)

        def P(j):
            xn = _unpack(xna_ref[rows_of(blocks[j])[1], :])
            for c in range(NC):
                f = feature_map(_dot_nt(_unpack(wpqt_ref[c * CR // 2:(c + 1) * CR // 2, :]), xn)).reshape(2 * CR, TB)
                for g in range(CG):
                    phi[j, CG * c + g] = f[2 * GR * g:2 * GR * (g + 1)].astype(bf16)

        def N(j):
            outs = []
            for g in range(NG):
                num = _dot(_unpack(kvt_ref[g]), phi[j, g])
                rm = 1.0 / (num[GR:] + 1e-6)
                rs = pltpu.roll(rm, 4, 0)
                r0, r1 = jnp.where(top, rm, rs), jnp.where(top, rs, rm)
                outs.append(num[:GR] * jnp.concatenate([r0, r0, rm, r1, r1], axis=0))
            ot[j] = jnp.concatenate(outs, axis=0)

        def W(j, t):
            if t == 0:
                o_ref[j] = pltpu.bitcast(ot[j].astype(bf16).T, u32)
                o[j] = _unpack(o_ref[j])
            y[j, t] = _dot(o[j], woa_ref[:, 128 * t:128 * t + 128])
            if t == 4:
                rows = rows_of(blocks[j])[0]
                xres_ref[rows, :] = load_x(rows) + jnp.concatenate([y[j, t] for t in range(5)], axis=1)

        def WW(j):
            for t in range(5):
                W(j, t)
            if hooks is not None:
                hooks[j]()

        P(0), P(1)
        if between is not None:
            between()
        N(0), P(2), N(1), WW(0), N(2)
        for j in range(3, n):
            P(j), WW(j - 2), N(j)
        WW(n - 2), WW(n - 1)

    VPERM = [(h * DHB + 64 * c) for c in range(3) for h in range(2)]

    def relayout_weights(j):
        r0 = pl.multiple_of(j * PW, PW)
        for m in range(2):
            wb_ref[j, :, m * PW:(m + 1) * PW] = pltpu.bitcast(stage_ref[m, pl.ds(r0, PW), :].T, u32)
        for c in range(3):
            w = jnp.concatenate([stage_ref[2, pl.ds(pl.multiple_of(r0 + o, 64), 64), :] for o in VPERM[2 * c:2 * c + 2]], axis=0)
            wb_ref[j, :, 2 * PW + 128 * c:2 * PW + 128 * (c + 1)] = pltpu.bitcast(w.T, u32)

    scale = DHB ** -0.5
    NQ = 32
    row, col = _iota((2 * NQ, 2 * L), 0), _iota((2 * NQ, 2 * L), 1)
    same = (row < NQ) == (col < L)
    rr = jnp.where(row < NQ, row, row - NQ)
    kk = jnp.where(col < L, col, col - L)
    keep = same & ((rr < MEM) | (rr >= kk) | (kk >= NQ))
    fill = jnp.where(same, -1e9 / scale, -jnp.inf).astype(f32)
    lo = lambda n, w=128: (_iota((n, w), 1) & 64) == 0
    sub8 = _iota((8, 128), 0)

    def halves(x):
        m = lo(*x.shape)
        return jnp.concatenate([jnp.where(m, x, 0.0), jnp.where(m, 0.0, x)], axis=0).astype(bf16)

    def outer(x):
        return jnp.concatenate([x[:, 0:128], x[:, 256:384]], axis=0).astype(bf16)

    def scores(q, k):
        s1 = _dot_nt(outer(q), outer(k))
        s2 = _dot_nt(q[:, 128:256].astype(bf16), halves(k[:, 128:256]))
        s = s1 + jnp.concatenate([s2, s2], axis=0)
        s = jnp.where(keep, s, fill)
        e = jnp.exp2((s - jnp.max(s, axis=1, keepdims=True)) * (scale * LOG2E))
        return e, jnp.sum(e, axis=1, keepdims=True)

    def values(e, l, v):
        rab = _recip(jnp.where(lo(NQ), l[:NQ], l[NQ:]))
        return _dot((e[:NQ] + e[NQ:]).astype(bf16), halves(v)) * jnp.concatenate([rab] * 3, axis=1)

    def head_attention(q, kv):
        rot = lambda x, r: pltpu.roll(x, r % 8, 0) if r % 8 else x
        tile = lambda x, c: x[:, 128 * c:128 * c + 128]
        q = q * (scale * LOG2E)
        ks = []
        for b in range(2):
            kb = kv[8 * b:8 * b + 8]
            ks.append((tile(kb, 0), jnp.where(lo(8), tile(kb, 1), 0.0), jnp.where(lo(8), 0.0, tile(kb, 1)), tile(kb, 2)))
        ss, m = {}, None
        for r in range(7, -1, -1):
            qr = [rot(tile(q, c), 8 - r) for c in range(3)]
            for b in range(2):
                k0, kl, kh, k2 = ks[b]
                sa = jnp.sum(qr[0] * k0 + qr[1] * kl, axis=1, keepdims=True)
                sb = jnp.sum(qr[2] * k2 + qr[1] * kh, axis=1, keepdims=True)
                x = jnp.where(lo(8), sa, sb)
                if b == 1 and r > 0:
                    x = jnp.where(sub8 <= 7 - r, x, -1e9 * LOG2E)
                ss[b, r] = x
            mx = jnp.maximum(ss[0, r], ss[1, r])
            m = mx if m is None else jnp.maximum(rot(m, 1), mx)
        acc = None
        for r in range(7, -1, -1):
            mr = rot(m, 8 - r)
            e0, e1 = jnp.exp2(ss[0, r] - mr), jnp.exp2(ss[1, r] - mr)
            t = [e0 + e1] + [e0 * tile(kv[0:8], 3 + c) + e1 * tile(kv[8:16], 3 + c) for c in range(3)]
            acc = t if acc is None else [rot(u, 1) + w for u, w in zip(acc, t)]
        r = _recip(acc[0])
        return jnp.concatenate([acc[1] * r, acc[2] * r, acc[3] * r], axis=1)

    def bstep(h, first, never, early, chained_in, pre=None):
        qkv, ps, os_, ov = {}, {}, {}, {}
        acc = [None]
        nxt = [0]

        split = pre is not None and first

        def is_long(first, t, m):
            flipped = m in FLIPM and t in FLIP
            return (flipped and not first) if pre is not None else first != flipped

        def PR(t, ms):
            hs = {m: h if is_long(first, t, m) else h[:NQ] for m in ms}
            if t == 0 and chained_in:
                rs = {}
                for k in range(5):
                    for m in ms:
                        c = _dot(hs[m][:, 128 * k:128 * k + 128].astype(bf16),
                                 _unpack(wb_ref[t, 64 * k:64 * k + 64, m * PW:(m + 1) * PW]))
                        rs[m] = c if k == 0 else rs[m] + c
            else:
                rs = {m: _dot(hs[m].astype(bf16), _unpack(wb_ref[t, :, m * PW:(m + 1) * PW])) for m in ms}
            for m in ms:
                if is_long(first, t, m):
                    svq_ref[t, :, m * PW:(m + 1) * PW] = rs[m][L:]
                    qkv[t, m] = rs[m][:L]
                else:
                    cols = slice(m * PW, (m + 1) * PW)
                    saved = svq_ref[t, :, cols] if pre is None else pre_ref[t, pl.ds(pl.multiple_of(pre * 8, 8), 8), cols]
                    qkv[t, m] = jnp.concatenate([rs[m], saved], axis=0)
            if not (split and t >= NP - 2):
                HA_(t)

        def HA_(t):
            kv = jnp.concatenate([qkv[t, 1], qkv[t, 2]], axis=1)
            ov[t] = head_attention(qkv[t, 0][NQ:], jnp.concatenate([kv[:MEM], kv[NQ:]], axis=0))

        def SS(j):
            ps[j] = scores(qkv[j, 0][:NQ], qkv[j, 1])

        def PV(j):
            e, l = ps[j]
            if j >= 1:
                e = jnp.concatenate([jnp.where(never, ov[j - 1][:, 128 * c:128 * c + 2 * L], e[8 * c:8 * c + 8])
                                     for c in range(3)] + [e[24:]], axis=0)
            if j in early:
                e = jnp.concatenate([e[:24], jnp.where(never, early[j][:, :2 * L], e[24:32]), e[32:]], axis=0)
            o = values(e, l, qkv[j, 2])
            if first:
                svo_ref[j] = o[24:32]
                o = jnp.concatenate([o[:24], ov[j]], axis=0)
            else:
                o = jnp.concatenate([o, ov[j], svo_ref[j]], axis=0)
            os_[j] = o

        def OO(merge=1):
            js = range(nxt[0], nxt[0] + merge)
            ws = []
            for j in js:
                if pre is not None:
                    ws.append(jnp.concatenate(
                        [pltpu.bitcast(stage_ref[3, j * PW + o:j * PW + o + 64, :], u32) for o in VPERM], axis=0))
                    if not first:
                        wob_ref[j] = ws[-1]
                else:
                    ws.append(wob_ref[j])
            c = _dot(jnp.concatenate([os_[j] for j in js], axis=1).astype(bf16), _unpack(jnp.concatenate(ws, axis=0)))
            acc[0] = c if acc[0] is None else acc[0] + c
            nxt[0] += merge

        order, tail = (ORD_A, TAIL_W if split else TAIL_A) if first else (ORD_B, TAIL_B)
        nl = 3 if first else 1
        nd = tail.count("O") + nl
        for t in range(NP):
            for op in order:
                if op == "Q":
                    PR(t, PORD_A if first else PORD_B)
                    if split and t == NP - 1:
                        pl.when(pre == 0)(lambda: cp_wob.wait())
                        HA_(NP - 2), HA_(NP - 1)
                if op == "S" and t >= 1:
                    SS(t - 1)
                if op == "P" and t >= 2:
                    PV(t - 2)
                if op == "O" and OLAG <= t < NP - 1 and nxt[0] < NP - nd:
                    OO()
        p = NP - 2
        for op in tail:
            if op == "O":
                OO()
            if op == "S":
                SS(NP - 1)
            if op == "P":
                PV(p)
                p += 1
        OO(nl)
        assert nxt[0] == NP and p == NP
        return acc[0]

    def bpass(last, lo_it, hi_it, warm=False):
        def body(i, c):
            never = flag_ref[:, :2 * L] > 0
            probe = lambda x, g: x[8 * g:8 * g + 8, 0:128]
            mem = mem_ref[...]
            if warm:
                slots = [pl.ds(pl.multiple_of(i * 64, 64), 64)]
                heads = [xnb_ref[pl.ds(pl.multiple_of((1 - i) * 64, 64), 8), :]]
            else:
                slots = [pl.ds(0, 64), pl.ds(64, 64)]
            xs = [xnb_ref[sl, :] for sl in slots]
            n = len(slots)
            for u in range(n):
                r0 = pl.multiple_of((i * n + u) * 64, 64)
                xa = xs[u]
                rn = pl.multiple_of(jnp.minimum(r0 + 128, S - 64), 64)
                xn = _layernorm(xres_ref[pl.ds(rn, 64), :])
                xnb_ref[slots[u], :] = xn
                if not warm and u == 0:
                    heads = [xs[1][0:8], xn[0:8]]
                early = {LN_AT + g: probe(xn, g) for g in range(8)}
                if not last:
                    rp = pl.multiple_of(jnp.maximum(r0 - 64, 0), 64)
                    xn = _layernorm(xres_ref[pl.ds(rp, 64), :])
                    xna_ref[pl.ds(pl.multiple_of(rp // 2, 32), 32), :] = _pack(xn)
                    for g in range(8):
                        j = LN_AT2 + g
                        early[j] = jnp.maximum(early[j], probe(xn, g)) if j in early else probe(xn, g)
                ya = bstep(jnp.concatenate([mem, xa[8:32], xa[0:8], xa[32:40]], axis=0), True, never, early,
                           u > 0, 2 * i if warm else None)
                yb = bstep(jnp.concatenate([ya[:MEM], xa[40:64], xa[32:40], heads[u]], axis=0), False, never, {},
                           True, 2 * i + 1 if warm else None)
                mem = yb[:MEM]
                y = xres_ref[pl.ds(r0, 64), :] + jnp.concatenate([ya[24:32], ya[MEM:24], yb[40:48], yb[32:40], yb[MEM:32]], axis=0)
                if last:
                    out_ref[pl.ds(r0, 64), :] = y.astype(bf16)
                else:
                    xres_ref[pl.ds(r0, 64), :] = y
            mem_ref[...] = mem
            if last:
                rows = pl.ds(pl.multiple_of(i * 128, 128), 128)
                pltpu.make_async_copy(out_ref.at[rows, :], out_hbm.at[rows, :], sems.at[7]).start()
            return c
        lax.fori_loop(lo_it, hi_it, body, 0)

    load_in = lambda rows: x_ref[rows, :].astype(f32)
    load_res = lambda rows: xres_ref[rows, :]
    NB = S // (TB * NCH)

    def k1_body(i, c):
        pl.when(i == 1)(lambda: cp_x(3).wait())
        k_blocks([1 + i * KB + j for j in range(KB)], load_in, jnp.minimum(1 + i * KB + KB, S // TB - 1))
        return c

    def q1_body(i, c):
        for m in range(3):
            cp_w(m, i).wait()
        pairs = [i * (NP // NCH) + j for j in range(NP // NCH)]
        for j in pairs:
            relayout_weights(j)
        head = []

        def norm_first():
            x0 = _layernorm(xres_ref[0:128, :])
            xnb_ref[...] = x0
            head.append(jnp.concatenate([x0[32 * sg:32 * sg + 8] for sg in range(4)], axis=0).astype(bf16))

        def project(js):
            for j in js:
                pre_ref[j] = _dot(head[0], _unpack(wb_ref[j]))

        q_blocks([i * NB + j for j in range(NB)], load_in,
                 hooks=[norm_first, lambda: project(pairs[:1]), lambda: project(pairs[1:3]), lambda: project(pairs[3:])])
        return c

    with _scope("pro"):
        flag_ref[...] = jnp.zeros(flag_ref.shape, jnp.int32)
        cnt_ref[0] = 0
        cp_phi.wait()
        cp_x(0).wait()
        phi_lhs = phi_blocks()
        xna_ref[0:TB // 2, :] = _pack(_layernorm(load_in(pl.ds(0, TB))))
        cp_wqkv(1).wait()
        fold_phi(phi_lhs, 1, wpkt_ref)

        def values_ready():
            cp_wqkv(2).wait()
            cp_x(1).wait()
            wvt_ref[...] = pltpu.bitcast(wqkv_ref[2].T, u32)
            xna_ref[TB // 2:TB, :] = _pack(_layernorm(load_in(pl.ds(TB, TB))))

        k_blocks([0], init=True, mid=values_ready)
        cp_x(2).wait()
    with _scope("k1"):
        lax.fori_loop(0, (S // TB - 1) // KB, k1_body, 0)
    with _scope("f1"):
        cp_wqkv(0).wait()
        cp_woa.wait()
        cp_mem.wait()
        fold_phi(phi_lhs, 0, wpqt_ref)
        finish_kv()
        mem_ref[...] = mem0_ref[...].astype(f32)
    with _scope("q1"):
        lax.fori_loop(0, NCH, q1_body, 0)
    with _scope("b1w"):
        bpass(False, 0, 2, warm=True)
    with _scope("b1"):
        bpass(False, 1, S // 128)
    with _scope("a2"):
        lax.fori_loop(0, cnt_ref[0] + 1, lambda i, c: (k_blocks(list(range(KSPLIT)), init=True), c)[1], 0)
        xna_ref[(S - 64) // 2:, :] = _pack(_layernorm(xres_ref[S - 64:, :]))
        k_blocks(list(range(KSPLIT, S // TB)))
        q_blocks(list(range(S // TB)), load_res, between=finish_kv)
    with _scope("b2"):
        mem_ref[...] = mem0_ref[...].astype(f32)
        x0 = _layernorm(xres_ref[0:128, :])
        xnb_ref[...] = x0
        for t in FLIP:
            for m in FLIPM:
                svq_ref[t, :, m * PW:(m + 1) * PW] = _dot(x0[0:16].astype(bf16), _unpack(wb_ref[t, :, m * PW:(m + 1) * PW]))[:8]
        bpass(True, 0, S // 128)
    pltpu.make_async_copy(out_ref, out_hbm, sems.at[7]).wait()


@functools.partial(jax.jit, static_argnames=("B_seg_len",))
def pallas_interleave_layers__linear_kernel_hedgehog__memory_aug_recurrent_mem_tr__prompt_kernel(
    A_x: jax.Array,
    A_wqkv: jax.Array,
    A_w_phi: jax.Array,
    A_wo: jax.Array,
    B_x: jax.Array,
    B_mem0: jax.Array,
    B_Wq: jax.Array,
    B_Wk: jax.Array,
    B_Wv: jax.Array,
    B_Wo: jax.Array,
    B_seg_len: int,
):
    del B_x
    assert B_seg_len == SEG
    assert A_x.shape == (1, S, D) and B_mem0.shape == (1, MEM, D)
    assert B_Wq.shape == (D, HB, DHB) and A_w_phi.shape == (HA, FA, FA)
    tr = lambda w: jnp.transpose(w, (1, 2, 0)).reshape(HB * DHB, D)
    hbm = pl.BlockSpec(memory_space=pl.ANY)
    out = pl.pallas_call(
        _kernel,
        out_shape=jax.ShapeDtypeStruct((S, D), bf16),
        in_specs=[hbm] * 9,
        out_specs=hbm,
        scratch_shapes=[
            pltpu.VMEM((S, D), bf16),
            pltpu.VMEM((3, D, D), bf16),
            pltpu.VMEM((FA, FA, HA), bf16),
            pltpu.VMEM((D, D), bf16),
            pltpu.VMEM((MEM, D), bf16),
            pltpu.VMEM((S, D), bf16),
            pltpu.VMEM((4, HB * DHB, D), bf16),
            pltpu.VMEM((NP, D // 2, 3 * PW), u32),
            pltpu.VMEM((NP, PW // 2, D), u32),
            pltpu.VMEM((S, D), f32),
            pltpu.VMEM((S // 2, D), u32),
            pltpu.VMEM((128, D), f32),
            pltpu.VMEM((D // 2, D), u32),
            pltpu.VMEM((D // 2, D), u32),
            pltpu.VMEM((D // 2, D), u32),
            pltpu.VMEM((NG, 48, 2 * GR), f32),
            pltpu.VMEM((NG, 24, 2 * GR), u32),
            pltpu.VMEM((S // TB, TB // 2, D), u32),
            pltpu.VMEM((MEM, D), f32),
            pltpu.VMEM((NP, 8, 3 * PW), f32),
            pltpu.VMEM((NP, 32, 3 * PW), f32),
            pltpu.VMEM((NP, 8, PW), f32),
            pltpu.VMEM((8, 128), jnp.int32),
            pltpu.SMEM((1,), jnp.int32),
            pltpu.SemaphoreType.DMA((12 + 3 * NCH,)),
        ],
        compiler_params=pltpu.CompilerParams(vmem_limit_bytes=120 * 1024 * 1024),
        name="hedgehog_rmt",
    )(A_x.reshape(S, D), A_wqkv, jnp.transpose(A_w_phi, (1, 2, 0)), A_wo, B_mem0.reshape(MEM, D),
      tr(B_Wq), tr(B_Wk), tr(B_Wv), B_Wo.reshape(HB * DHB, D))
    return out.reshape(1, S, D)
```

```python
import contextlib
import functools

import jax
import jax.numpy as jnp
from jax import lax
import jax.experimental.pallas as pl
import jax.experimental.pallas.tpu as pltpu

f32, bf16, u32 = jnp.float32, jnp.bfloat16, jnp.uint32

S, D = 2048, 640
HA, FA = 32, 20
HB, DHB = 32, 192
MEM, SEG = 8, 32
L = MEM + SEG
NP = HB // 2
PW = 2 * DHB
TB = 128
NG = 16
GR = 2 * FA
NCH = 4
NT = (((1,), (1,)), ((), ()))
LOG2E = 1.4426950408889634

FLIP, FLIPM = (0, 1, 2, 3, 4, 13, 14, 15), (2,)
ORD_A, ORD_B = "QSPO", "QOPS"
TAIL_A, TAIL_B, TAIL_W = "OOOSPOOOPOO", "OOSPOOPO", "SOOOOPOOOPOOOOOO"
PORD_A, PORD_B = (1, 2, 0), (0, 1, 2)
OLAG = 4
LN_AT, LN_AT2 = 0, 4
KB = 3
KSPLIT = 7


_scope = lambda name: contextlib.nullcontext()


def _dot(a, b):
    return jnp.dot(a, b, preferred_element_type=f32)


def _dot_nt(a, b):
    return lax.dot_general(a, b, NT, preferred_element_type=f32)


def _pack(x):
    return pltpu.bitcast(x.astype(bf16), u32)


def _unpack(x):
    return pltpu.bitcast(x, bf16)


def _recip(x):
    r = pl.reciprocal(x, approx=True)
    return r * (2.0 - x * r)


def _layernorm(x):
    m = jnp.mean(x, axis=-1, keepdims=True)
    xc = x - m
    v = jnp.mean(xc * xc, axis=-1, keepdims=True)
    return xc * lax.rsqrt(v + 1e-5)


def _iota(shape, dim):
    return lax.broadcasted_iota(jnp.int32, shape, dim)


def _kernel(x_hbm, wqkv_hbm, wphi_hbm, woa_hbm, mem0_hbm, wqt_hbm, wkt_hbm, wvt_hbm, wob_hbm,
            out_hbm,
            x_ref, wqkv_ref, wphi_ref, woa_ref, mem0_ref, out_ref,
            stage_ref, wb_ref, wob_ref, xres_ref, xna_ref, xnb_ref,
            wpqt_ref, wpkt_ref, wvt_ref, acc_ref, kvt_ref, o_ref,
            mem_ref, svq_ref, pre_ref, svo_ref, flag_ref, cnt_ref, sems):
    WC = HB * DHB // NCH
    X_CUTS = (0, TB, 2 * TB, (2 + KB) * TB, S)

    def cp_wqkv(m):
        return pltpu.make_async_copy(wqkv_hbm.at[:, pl.ds(m * D, D)], wqkv_ref.at[m], sems.at[m])

    def cp_x(n):
        rows = pl.ds(X_CUTS[n], X_CUTS[n + 1] - X_CUTS[n])
        return pltpu.make_async_copy(x_hbm.at[rows, :], x_ref.at[rows, :], sems.at[8 + n])

    def cp_w(m, i):
        rows = pl.ds(pl.multiple_of(i * WC, WC), WC)
        return pltpu.make_async_copy((wqt_hbm, wkt_hbm, wvt_hbm)[m].at[rows, :], stage_ref.at[m, rows, :],
                                     sems.at[12 + NCH * m + i])

    cp_phi = pltpu.make_async_copy(wphi_hbm, wphi_ref, sems.at[3])
    cp_woa = pltpu.make_async_copy(woa_hbm, woa_ref, sems.at[4])
    cp_mem = pltpu.make_async_copy(mem0_hbm, mem0_ref, sems.at[5])
    cp_wob = pltpu.make_async_copy(wob_hbm, stage_ref.at[3], sems.at[6])
    cp_phi.start()
    cp_x(0).start()
    cp_wqkv(1).start()
    cp_wqkv(2).start()
    cp_x(1).start()
    cp_x(2).start()
    cp_x(3).start()
    cp_wqkv(0).start()
    cp_woa.start()
    cp_mem.start()
    for i in range(NCH):
        for m in range(3):
            cp_w(m, i).start()
    cp_wob.start()

    def phi_blocks():
        wphi = wphi_ref[...].astype(f32)
        cat = jnp.concatenate([wphi[d] for d in range(FA)], axis=1)
        cat = jnp.concatenate([cat, jnp.zeros((32 - FA, D), f32)], axis=0).astype(bf16)
        p_row, p_col = _iota((D, D), 0), _iota((D, D), 1)
        spread = (FA * (p_row & 31) + (p_row >> 5) == p_col).astype(f32).astype(bf16)
        u = _dot(cat, spread).astype(bf16)
        dup = ((_iota((48, 32), 0) >> 1) == _iota((48, 32), 1)).astype(f32).astype(bf16)
        u2 = _dot(dup, u)[:GR]
        lane, par = _iota((GR, 128), 1), _iota((GR, 128), 0) & 1
        lhs = []
        for c in range(5):
            blocks = []
            for g in range(3 * c, 3 * c + 4):
                lo = GR * g - 128 * c + FA * par
                blocks.append(jnp.where((lane >= lo) & (lane < lo + FA), u2[:, 128 * c:128 * c + 128], 0.0))
            lhs.append(jnp.concatenate(blocks, axis=0).astype(bf16))
        return lhs

    def fold_phi(lhs, m, dst):
        parts = [_dot_nt(lhs[c], wqkv_ref[m, :, 128 * c:128 * c + 128]) for c in range(5)]
        rows = []
        for c in range(5):
            first = parts[c][:GR] if c == 0 else parts[c][:GR] + parts[c - 1][3 * GR:]
            rows += [first, parts[c][GR:3 * GR]]
        rows.append(parts[4][3 * GR:])
        dst[...] = _pack(jnp.concatenate(rows, axis=0))

    def fold(x, op):
        r = op(op(op(x[:, 0], x[:, 1]), op(x[:, 2], x[:, 3])), x[:, 4])
        r = op(r, pltpu.roll(r, 2, 1))
        return op(r, pltpu.roll(r, 4, 1))

    def feature_map(pt):
        p = pt.reshape(-1, 5, 8, TB)
        ep = jnp.exp(p - fold(p, jnp.maximum)[:, None])
        en = jnp.exp(fold(p, jnp.minimum)[:, None] - p)
        ep = ep * _recip(fold(ep, jnp.add))[:, None]
        en = en * _recip(fold(en, jnp.add))[:, None]
        return jnp.concatenate([ep, en], axis=1)

    def rows_of(b):
        if isinstance(b, int):
            return pl.ds(b * TB, TB), pl.ds(b * TB // 2, TB // 2)
        return pl.ds(pl.multiple_of(b * TB, TB), TB), pl.ds(pl.multiple_of(b * (TB // 2), TB // 2), TB // 2)

    CG = 4
    NC = NG // CG
    CR = CG * GR

    def k_blocks(blocks, load_x=None, ahead=None, init=False, mid=None):
        xn, v, phi = {}, {}, {}

        def LN(j):
            rows, prows = rows_of(blocks[j] if j < len(blocks) else ahead)
            if load_x is not None and j > 0:
                xn[j] = _layernorm(load_x(rows)).astype(bf16)
                xna_ref[prows, :] = pltpu.bitcast(xn[j], u32)
            else:
                xn[j] = _unpack(xna_ref[prows, :])

        def P(j, c):
            pk = _dot_nt(_unpack(wpkt_ref[c * CR // 2:(c + 1) * CR // 2, :]), xn[j])
            f = feature_map(pk).reshape(2 * CR, TB)
            for g in range(CG):
                phi[j, CG * c + g] = f[2 * GR * g:2 * GR * (g + 1)].astype(bf16)

        def V(j, c):
            vt = _dot_nt(_unpack(wvt_ref[c * CR // 2:(c + 1) * CR // 2, :]), xn[j])
            for g in range(CG):
                v[j, CG * c + g] = jnp.concatenate([vt[GR * g:GR * (g + 1)], jnp.ones((8, TB), f32)], axis=0).astype(bf16)

        def KV(j):
            for g in range(NG):
                r = _dot_nt(v[j, g], phi[j, g])
                if init and j == 0:
                    acc_ref[g] = r
                else:
                    acc_ref[g] += r

        LN(0)
        for j in range(len(blocks)):
            if j + 1 < len(blocks) or ahead is not None:
                LN(j + 1)
            for c in range(NC):
                P(j, c)
            if mid is not None:
                mid()
            for c in range(NC):
                V(j, c)
            KV(j)

    def finish_kv():
        r48, odd = _iota((48, 2 * GR), 0), (_iota((48, 2 * GR), 1) & 1) == 1
        same = (((r48 >= FA) & (r48 < GR)) | (r48 >= GR + 4)) == odd
        for g in range(NG):
            kvt_ref[g] = _pack(jnp.where(same, acc_ref[g], 0.0))

    def q_blocks(blocks, load_x, hooks, between=None):
        top = _iota((8, TB), 0) < 4
        phi, ot, o, y = {}, {}, {}, {}
        n = len(blocks)

        def P(j):
            xn = _unpack(xna_ref[rows_of(blocks[j])[1], :])
            for c in range(NC):
                f = feature_map(_dot_nt(_unpack(wpqt_ref[c * CR // 2:(c + 1) * CR // 2, :]), xn)).reshape(2 * CR, TB)
                for g in range(CG):
                    phi[j, CG * c + g] = f[2 * GR * g:2 * GR * (g + 1)].astype(bf16)

        def N(j):
            outs = []
            for g in range(NG):
                num = _dot(_unpack(kvt_ref[g]), phi[j, g])
                rm = 1.0 / (num[GR:] + 1e-6)
                rs = pltpu.roll(rm, 4, 0)
                r0, r1 = jnp.where(top, rm, rs), jnp.where(top, rs, rm)
                outs.append(num[:GR] * jnp.concatenate([r0, r0, rm, r1, r1], axis=0))
            ot[j] = jnp.concatenate(outs, axis=0)

        def W(j, t):
            if t == 0:
                o_ref[j] = pltpu.bitcast(ot[j].astype(bf16).T, u32)
                o[j] = _unpack(o_ref[j])
            y[j, t] = _dot(o[j], woa_ref[:, 128 * t:128 * t + 128])
            if t == 4:
                rows = rows_of(blocks[j])[0]
                xres_ref[rows, :] = load_x(rows) + jnp.concatenate([y[j, t] for t in range(5)], axis=1)

        def WW(j):
            for t in range(5):
                W(j, t)
                if (j, t) in hooks:
                    hooks[j, t]()

        P(0), P(1)
        if between is not None:
            between()
        N(0), P(2), N(1), WW(0), N(2)
        for j in range(3, n):
            P(j), WW(j - 2), N(j)
        WW(n - 2), WW(n - 1)

    VPERM = [(h * DHB + 64 * c) for c in range(3) for h in range(2)]

    def relayout_weights(j):
        r0 = pl.multiple_of(j * PW, PW)
        for m in range(2):
            wb_ref[j, :, m * PW:(m + 1) * PW] = pltpu.bitcast(stage_ref[m, pl.ds(r0, PW), :].T, u32)
        for c in range(3):
            w = jnp.concatenate([stage_ref[2, pl.ds(pl.multiple_of(r0 + o, 64), 64), :] for o in VPERM[2 * c:2 * c + 2]], axis=0)
            wb_ref[j, :, 2 * PW + 128 * c:2 * PW + 128 * (c + 1)] = pltpu.bitcast(w.T, u32)

    scale = DHB ** -0.5
    NQ = 32
    row, col = _iota((2 * NQ, 2 * L), 0), _iota((2 * NQ, 2 * L), 1)
    same = (row < NQ) == (col < L)
    rr = jnp.where(row < NQ, row, row - NQ)
    kk = jnp.where(col < L, col, col - L)
    keep = same & ((rr < MEM) | (rr >= kk) | (kk >= NQ))
    fill = jnp.where(same, -1e9 / scale, -jnp.inf).astype(f32)
    lo = lambda n, w=128: (_iota((n, w), 1) & 64) == 0
    sub8 = _iota((8, 128), 0)

    def halves(x):
        m = lo(*x.shape)
        return jnp.concatenate([jnp.where(m, x, 0.0), jnp.where(m, 0.0, x)], axis=0).astype(bf16)

    def outer(x):
        return jnp.concatenate([x[:, 0:128], x[:, 256:384]], axis=0).astype(bf16)

    def scores(q, k):
        s1 = _dot_nt(outer(q), outer(k))
        s2 = _dot_nt(q[:, 128:256].astype(bf16), halves(k[:, 128:256]))
        s = s1 + jnp.concatenate([s2, s2], axis=0)
        s = jnp.where(keep, s, fill)
        e = jnp.exp2((s - jnp.max(s, axis=1, keepdims=True)) * (scale * LOG2E))
        return e, jnp.sum(e, axis=1, keepdims=True)

    def values(e, l, v):
        rab = _recip(jnp.where(lo(NQ), l[:NQ], l[NQ:]))
        return _dot((e[:NQ] + e[NQ:]).astype(bf16), halves(v)) * jnp.concatenate([rab] * 3, axis=1)

    def head_attention(q, kv):
        rot = lambda x, r: pltpu.roll(x, r % 8, 0) if r % 8 else x
        tile = lambda x, c: x[:, 128 * c:128 * c + 128]
        q = q * (scale * LOG2E)
        ks = []
        for b in range(2):
            kb = kv[8 * b:8 * b + 8]
            ks.append((tile(kb, 0), jnp.where(lo(8), tile(kb, 1), 0.0), jnp.where(lo(8), 0.0, tile(kb, 1)), tile(kb, 2)))
        ss, m = {}, None
        for r in range(7, -1, -1):
            qr = [rot(tile(q, c), 8 - r) for c in range(3)]
            for b in range(2):
                k0, kl, kh, k2 = ks[b]
                sa = jnp.sum(qr[0] * k0 + qr[1] * kl, axis=1, keepdims=True)
                sb = jnp.sum(qr[2] * k2 + qr[1] * kh, axis=1, keepdims=True)
                x = jnp.where(lo(8), sa, sb)
                if b == 1 and r > 0:
                    x = jnp.where(sub8 <= 7 - r, x, -1e9 * LOG2E)
                ss[b, r] = x
            mx = jnp.maximum(ss[0, r], ss[1, r])
            m = mx if m is None else jnp.maximum(rot(m, 1), mx)
        acc = None
        for r in range(7, -1, -1):
            mr = rot(m, 8 - r)
            e0, e1 = jnp.exp2(ss[0, r] - mr), jnp.exp2(ss[1, r] - mr)
            t = [e0 + e1] + [e0 * tile(kv[0:8], 3 + c) + e1 * tile(kv[8:16], 3 + c) for c in range(3)]
            acc = t if acc is None else [rot(u, 1) + w for u, w in zip(acc, t)]
        r = _recip(acc[0])
        return jnp.concatenate([acc[1] * r, acc[2] * r, acc[3] * r], axis=1)

    def bstep(h, first, never, early, chained_in, pre=None):
        qkv, ps, os_, ov = {}, {}, {}, {}
        acc = [None]
        nxt = [0]

        split = pre is not None and first

        def is_long(first, t, m):
            flipped = m in FLIPM and t in FLIP
            return (flipped and not first) if pre is not None else first != flipped

        def PR(t, ms):
            hs = {m: h if is_long(first, t, m) else h[:NQ] for m in ms}
            if t == 0 and chained_in:
                rs = {}
                for k in range(5):
                    for m in ms:
                        c = _dot(hs[m][:, 128 * k:128 * k + 128].astype(bf16),
                                 _unpack(wb_ref[t, 64 * k:64 * k + 64, m * PW:(m + 1) * PW]))
                        rs[m] = c if k == 0 else rs[m] + c
            else:
                rs = {m: _dot(hs[m].astype(bf16), _unpack(wb_ref[t, :, m * PW:(m + 1) * PW])) for m in ms}
            for m in ms:
                if is_long(first, t, m):
                    svq_ref[t, :, m * PW:(m + 1) * PW] = rs[m][L:]
                    qkv[t, m] = rs[m][:L]
                else:
                    cols = slice(m * PW, (m + 1) * PW)
                    saved = svq_ref[t, :, cols] if pre is None else pre_ref[t, pl.ds(pl.multiple_of(pre * 8, 8), 8), cols]
                    qkv[t, m] = jnp.concatenate([rs[m], saved], axis=0)
            if not (split and t >= NP - 2):
                HA_(t)

        def HA_(t):
            kv = jnp.concatenate([qkv[t, 1], qkv[t, 2]], axis=1)
            ov[t] = head_attention(qkv[t, 0][NQ:], jnp.concatenate([kv[:MEM], kv[NQ:]], axis=0))

        def SS(j):
            ps[j] = scores(qkv[j, 0][:NQ], qkv[j, 1])

        def PV(j):
            e, l = ps[j]
            if j >= 1:
                e = jnp.concatenate([jnp.where(never, ov[j - 1][:, 128 * c:128 * c + 2 * L], e[8 * c:8 * c + 8])
                                     for c in range(3)] + [e[24:]], axis=0)
            if j in early:
                e = jnp.concatenate([e[:24], jnp.where(never, early[j][:, :2 * L], e[24:32]), e[32:]], axis=0)
            o = values(e, l, qkv[j, 2])
            if first:
                svo_ref[j] = o[24:32]
                o = jnp.concatenate([o[:24], ov[j]], axis=0)
            else:
                o = jnp.concatenate([o, ov[j], svo_ref[j]], axis=0)
            os_[j] = o

        def OO(merge=1):
            js = range(nxt[0], nxt[0] + merge)
            ws = []
            for j in js:
                if pre is not None:
                    ws.append(jnp.concatenate(
                        [pltpu.bitcast(stage_ref[3, j * PW + o:j * PW + o + 64, :], u32) for o in VPERM], axis=0))
                    if not first:
                        wob_ref[j] = ws[-1]
                else:
                    ws.append(wob_ref[j])
            c = _dot(jnp.concatenate([os_[j] for j in js], axis=1).astype(bf16), _unpack(jnp.concatenate(ws, axis=0)))
            acc[0] = c if acc[0] is None else acc[0] + c
            nxt[0] += merge

        order, tail = (ORD_A, TAIL_W if split else TAIL_A) if first else (ORD_B, TAIL_B)
        nl = 3 if first else 1
        nd = tail.count("O") + nl
        for t in range(NP):
            for op in order:
                if op == "Q":
                    PR(t, PORD_A if first else PORD_B)
                    if split and t == NP - 1:
                        pl.when(pre == 0)(lambda: cp_wob.wait())
                        HA_(NP - 2), HA_(NP - 1)
                if op == "S" and t >= 1:
                    SS(t - 1)
                if op == "P" and t >= 2:
                    PV(t - 2)
                if op == "O" and OLAG <= t < NP - 1 and nxt[0] < NP - nd:
                    OO()
        p = NP - 2
        for op in tail:
            if op == "O":
                OO()
            if op == "S":
                SS(NP - 1)
            if op == "P":
                PV(p)
                p += 1
        OO(nl)
        assert nxt[0] == NP and p == NP
        return acc[0]

    def bpass(last, lo_it, hi_it, warm=False):
        def body(i, c):
            never = flag_ref[:, :2 * L] > 0
            probe = lambda x, g: x[8 * g:8 * g + 8, 0:128]
            mem = mem_ref[...]
            if warm:
                slots = [pl.ds(pl.multiple_of(i * 64, 64), 64)]
                heads = [xnb_ref[pl.ds(pl.multiple_of((1 - i) * 64, 64), 8), :]]
            else:
                slots = [pl.ds(0, 64), pl.ds(64, 64)]
            xs = [xnb_ref[sl, :] for sl in slots]
            n = len(slots)
            for u in range(n):
                r0 = pl.multiple_of((i * n + u) * 64, 64)
                xa = xs[u]
                rn = pl.multiple_of(jnp.minimum(r0 + 128, S - 64), 64)
                xn = _layernorm(xres_ref[pl.ds(rn, 64), :])
                xnb_ref[slots[u], :] = xn
                if not warm and u == 0:
                    heads = [xs[1][0:8], xn[0:8]]
                early = {LN_AT + g: probe(xn, g) for g in range(8)}
                if not last:
                    rp = pl.multiple_of(jnp.maximum(r0 - 64, 0), 64)
                    xn = _layernorm(xres_ref[pl.ds(rp, 64), :])
                    xna_ref[pl.ds(pl.multiple_of(rp // 2, 32), 32), :] = _pack(xn)
                    for g in range(8):
                        j = LN_AT2 + g
                        early[j] = jnp.maximum(early[j], probe(xn, g)) if j in early else probe(xn, g)
                ya = bstep(jnp.concatenate([mem, xa[8:32], xa[0:8], xa[32:40]], axis=0), True, never, early,
                           u > 0, 2 * i if warm else None)
                yb = bstep(jnp.concatenate([ya[:MEM], xa[40:64], xa[32:40], heads[u]], axis=0), False, never, {},
                           True, 2 * i + 1 if warm else None)
                mem = yb[:MEM]
                y = xres_ref[pl.ds(r0, 64), :] + jnp.concatenate([ya[24:32], ya[MEM:24], yb[40:48], yb[32:40], yb[MEM:32]], axis=0)
                if last:
                    out_ref[pl.ds(r0, 64), :] = y.astype(bf16)
                else:
                    xres_ref[pl.ds(r0, 64), :] = y
            mem_ref[...] = mem
            if last:
                rows = pl.ds(pl.multiple_of(i * 128, 128), 128)
                pltpu.make_async_copy(out_ref.at[rows, :], out_hbm.at[rows, :], sems.at[7]).start()
            return c
        lax.fori_loop(lo_it, hi_it, body, 0)

    load_in = lambda rows: x_ref[rows, :].astype(f32)
    load_res = lambda rows: xres_ref[rows, :]
    NB = S // (TB * NCH)

    def k1_body(i, c):
        pl.when(i == 1)(lambda: cp_x(3).wait())
        k_blocks([1 + i * KB + j for j in range(KB)], load_in, jnp.minimum(1 + i * KB + KB, S // TB - 1))
        return c

    def q1_body(i, c):
        for m in range(3):
            cp_w(m, i).wait()
        pairs = [i * (NP // NCH) + j for j in range(NP // NCH)]
        for j in pairs:
            relayout_weights(j)
        head = []

        def norm_first():
            x0 = _layernorm(xres_ref[0:128, :])
            xnb_ref[...] = x0
            head.append(jnp.concatenate([x0[32 * sg:32 * sg + 8] for sg in range(4)], axis=0).astype(bf16))

        def project(js):
            for j in js:
                pre_ref[j] = _dot(head[0], _unpack(wb_ref[j]))

        q_blocks([i * NB + j for j in range(NB)], load_in,
                 {(0, 4): norm_first, (1, 4): lambda: project(pairs[:1]), (2, 4): lambda: project(pairs[1:3]),
                  (3, 4): lambda: project(pairs[3:])})
        return c

    with _scope("pro"):
        flag_ref[...] = jnp.zeros(flag_ref.shape, jnp.int32)
        cnt_ref[0] = 0
        cp_phi.wait()
        cp_x(0).wait()
        phi_lhs = phi_blocks()
        xna_ref[0:TB // 2, :] = _pack(_layernorm(load_in(pl.ds(0, TB))))
        cp_wqkv(1).wait()
        fold_phi(phi_lhs, 1, wpkt_ref)

        def values_ready():
            cp_wqkv(2).wait()
            cp_x(1).wait()
            wvt_ref[...] = pltpu.bitcast(wqkv_ref[2].T, u32)
            xna_ref[TB // 2:TB, :] = _pack(_layernorm(load_in(pl.ds(TB, TB))))

        k_blocks([0], init=True, mid=values_ready)
        cp_x(2).wait()
    with _scope("k1"):
        lax.fori_loop(0, (S // TB - 1) // KB, k1_body, 0)
    with _scope("f1"):
        cp_wqkv(0).wait()
        cp_woa.wait()
        cp_mem.wait()
        fold_phi(phi_lhs, 0, wpqt_ref)
        finish_kv()
        mem_ref[...] = mem0_ref[...].astype(f32)
    with _scope("q1"):
        lax.fori_loop(0, NCH, q1_body, 0)
    with _scope("b1w"):
        bpass(False, 0, 2, warm=True)
    with _scope("b1"):
        bpass(False, 1, S // 128)
    with _scope("a2"):
        lax.fori_loop(0, cnt_ref[0] + 1, lambda i, c: (k_blocks(list(range(KSPLIT)), init=True), c)[1], 0)
        xna_ref[(S - 64) // 2:, :] = _pack(_layernorm(xres_ref[S - 64:, :]))
        k_blocks(list(range(KSPLIT, S // TB)))
        head = []

        def norm_first():
            x0 = _layernorm(xres_ref[0:128, :])
            xnb_ref[...] = x0
            head.append(x0[0:16].astype(bf16))

        def save_rows(t, c):
            svq_ref[t, :, c:c + 128] = _dot(head[0], _unpack(wb_ref[t, :, c:c + 128]))[:8]

        hooks = {(0, 4): norm_first}
        pieces = [(t, m * PW + 128 * c) for t in FLIP for m in FLIPM for c in range(3)]
        for n, piece in enumerate(pieces):
            hooks[2 + n // 2, 1 + 2 * (n % 2)] = functools.partial(save_rows, *piece)
        q_blocks(list(range(S // TB)), load_res, hooks, between=finish_kv)
        mem_ref[...] = mem0_ref[...].astype(f32)
    with _scope("b2"):
        bpass(True, 0, S // 128)
    pltpu.make_async_copy(out_ref, out_hbm, sems.at[7]).wait()


@functools.partial(jax.jit, static_argnames=("B_seg_len",))
def pallas_interleave_layers__linear_kernel_hedgehog__memory_aug_recurrent_mem_tr__prompt_kernel(
    A_x: jax.Array,
    A_wqkv: jax.Array,
    A_w_phi: jax.Array,
    A_wo: jax.Array,
    B_x: jax.Array,
    B_mem0: jax.Array,
    B_Wq: jax.Array,
    B_Wk: jax.Array,
    B_Wv: jax.Array,
    B_Wo: jax.Array,
    B_seg_len: int,
):
    del B_x
    assert B_seg_len == SEG
    assert A_x.shape == (1, S, D) and B_mem0.shape == (1, MEM, D)
    assert B_Wq.shape == (D, HB, DHB) and A_w_phi.shape == (HA, FA, FA)
    tr = lambda w: jnp.transpose(w, (1, 2, 0)).reshape(HB * DHB, D)
    hbm = pl.BlockSpec(memory_space=pl.ANY)
    out = pl.pallas_call(
        _kernel,
        out_shape=jax.ShapeDtypeStruct((S, D), bf16),
        in_specs=[hbm] * 9,
        out_specs=hbm,
        scratch_shapes=[
            pltpu.VMEM((S, D), bf16),
            pltpu.VMEM((3, D, D), bf16),
            pltpu.VMEM((FA, FA, HA), bf16),
            pltpu.VMEM((D, D), bf16),
            pltpu.VMEM((MEM, D), bf16),
            pltpu.VMEM((S, D), bf16),
            pltpu.VMEM((4, HB * DHB, D), bf16),
            pltpu.VMEM((NP, D // 2, 3 * PW), u32),
            pltpu.VMEM((NP, PW // 2, D), u32),
            pltpu.VMEM((S, D), f32),
            pltpu.VMEM((S // 2, D), u32),
            pltpu.VMEM((128, D), f32),
            pltpu.VMEM((D // 2, D), u32),
            pltpu.VMEM((D // 2, D), u32),
            pltpu.VMEM((D // 2, D), u32),
            pltpu.VMEM((NG, 48, 2 * GR), f32),
            pltpu.VMEM((NG, 24, 2 * GR), u32),
            pltpu.VMEM((S // TB, TB // 2, D), u32),
            pltpu.VMEM((MEM, D), f32),
            pltpu.VMEM((NP, 8, 3 * PW), f32),
            pltpu.VMEM((NP, 32, 3 * PW), f32),
            pltpu.VMEM((NP, 8, PW), f32),
            pltpu.VMEM((8, 128), jnp.int32),
            pltpu.SMEM((1,), jnp.int32),
            pltpu.SemaphoreType.DMA((12 + 3 * NCH,)),
        ],
        compiler_params=pltpu.CompilerParams(vmem_limit_bytes=120 * 1024 * 1024),
        name="hedgehog_rmt",
    )(A_x.reshape(S, D), A_wqkv, jnp.transpose(A_w_phi, (1, 2, 0)), A_wo, B_mem0.reshape(MEM, D),
      tr(B_Wq), tr(B_Wk), tr(B_Wv), B_Wo.reshape(HB * DHB, D))
    return out.reshape(1, S, D)
```

```python
import contextlib
import functools

import jax
import jax.numpy as jnp
from jax import lax
import jax.experimental.pallas as pl
import jax.experimental.pallas.tpu as pltpu

f32, bf16, u32 = jnp.float32, jnp.bfloat16, jnp.uint32

S, D = 2048, 640
HA, FA = 32, 20
HB, DHB = 32, 192
MEM, SEG = 8, 32
L = MEM + SEG
NP = HB // 2
PW = 2 * DHB
TB = 128
NG = 16
GR = 2 * FA
NCH = 4
NT = (((1,), (1,)), ((), ()))
LOG2E = 1.4426950408889634

FLIP = {t: 2 for t in (0, 1, 2, 3, 4, 13, 14, 15)}
ORD_A, ORD_B = "QSOP", "QOPS"
TAIL_A, TAIL_B, TAIL_C, TAIL_W = "OOOSPOOOPOO", "OOSPOOPO", "OOSPOOPO", "SOOOOPOOOPOOOOOO"
PORD_A, PORD_B = (1, 2, 0), (0, 1, 2)
OLAG_A, OLAG_B = 4, 4
MERGE_A = 2
ANCHOR_A, ANCHOR_B = 1, 1
LN_AT, LN_AT2 = 2, 3
KB = 3
KSPLIT = 7


_scope = lambda name: contextlib.nullcontext()


def _dot(a, b):
    return jnp.dot(a, b, preferred_element_type=f32)


def _dot_nt(a, b):
    return lax.dot_general(a, b, NT, preferred_element_type=f32)


def _pack(x):
    return pltpu.bitcast(x.astype(bf16), u32)


def _unpack(x):
    return pltpu.bitcast(x, bf16)


def _recip(x):
    r = pl.reciprocal(x, approx=True)
    return r * (2.0 - x * r)


def _layernorm(x):
    m = jnp.mean(x, axis=-1, keepdims=True)
    xc = x - m
    v = jnp.mean(xc * xc, axis=-1, keepdims=True)
    return xc * lax.rsqrt(v + 1e-5)


def _iota(shape, dim):
    return lax.broadcasted_iota(jnp.int32, shape, dim)


def _kernel(x_hbm, wqkv_hbm, wphi_hbm, woa_hbm, mem0_hbm, wqt_hbm, wkt_hbm, wvt_hbm, wob_hbm,
            out_hbm,
            x_ref, wqkv_ref, wphi_ref, woa_ref, mem0_ref, out_ref,
            stage_ref, wb_ref, wob_ref, xres_ref, xna_ref, xnb_ref,
            wpqt_ref, wpkt_ref, wvt_ref, acc_ref, kvt_ref, o_ref,
            mem_ref, svq_ref, pre_ref, svo_ref, flag_ref, cnt_ref, sems):
    WC = HB * DHB // NCH
    X_CUTS = (0, TB, 2 * TB, (2 + KB) * TB, S)

    def cp_wqkv(m):
        return pltpu.make_async_copy(wqkv_hbm.at[:, pl.ds(m * D, D)], wqkv_ref.at[m], sems.at[m])

    def cp_x(n):
        rows = pl.ds(X_CUTS[n], X_CUTS[n + 1] - X_CUTS[n])
        return pltpu.make_async_copy(x_hbm.at[rows, :], x_ref.at[rows, :], sems.at[8 + n])

    def cp_w(m, i):
        rows = pl.ds(pl.multiple_of(i * WC, WC), WC)
        return pltpu.make_async_copy((wqt_hbm, wkt_hbm, wvt_hbm)[m].at[rows, :], stage_ref.at[m, rows, :],
                                     sems.at[12 + NCH * m + i])

    cp_phi = pltpu.make_async_copy(wphi_hbm, wphi_ref, sems.at[3])
    cp_woa = pltpu.make_async_copy(woa_hbm, woa_ref, sems.at[4])
    cp_mem = pltpu.make_async_copy(mem0_hbm, mem0_ref, sems.at[5])
    cp_wob = pltpu.make_async_copy(wob_hbm, stage_ref.at[3], sems.at[6])
    cp_phi.start()
    cp_x(0).start()
    cp_wqkv(1).start()
    cp_wqkv(2).start()
    cp_x(1).start()
    cp_x(2).start()
    cp_x(3).start()
    cp_wqkv(0).start()
    cp_woa.start()
    cp_mem.start()
    for i in range(NCH):
        for m in range(3):
            cp_w(m, i).start()
    cp_wob.start()

    def phi_blocks():
        wphi = wphi_ref[...].astype(f32)
        cat = jnp.concatenate([wphi[d] for d in range(FA)], axis=1)
        cat = jnp.concatenate([cat, jnp.zeros((32 - FA, D), f32)], axis=0).astype(bf16)
        p_row, p_col = _iota((D, D), 0), _iota((D, D), 1)
        spread = (FA * (p_row & 31) + (p_row >> 5) == p_col).astype(f32).astype(bf16)
        u = _dot(cat, spread).astype(bf16)
        dup = ((_iota((48, 32), 0) >> 1) == _iota((48, 32), 1)).astype(f32).astype(bf16)
        u2 = _dot(dup, u)[:GR]
        lane, par = _iota((GR, 128), 1), _iota((GR, 128), 0) & 1
        lhs = []
        for c in range(5):
            blocks = []
            for g in range(3 * c, 3 * c + 4):
                lo = GR * g - 128 * c + FA * par
                blocks.append(jnp.where((lane >= lo) & (lane < lo + FA), u2[:, 128 * c:128 * c + 128], 0.0))
            lhs.append(jnp.concatenate(blocks, axis=0).astype(bf16))
        return lhs

    def fold_phi(lhs, m, dst):
        parts = [_dot_nt(lhs[c], wqkv_ref[m, :, 128 * c:128 * c + 128]) for c in range(5)]
        rows = []
        for c in range(5):
            first = parts[c][:GR] if c == 0 else parts[c][:GR] + parts[c - 1][3 * GR:]
            rows += [first, parts[c][GR:3 * GR]]
        rows.append(parts[4][3 * GR:])
        dst[...] = _pack(jnp.concatenate(rows, axis=0))

    def fold(x, op):
        r = op(op(op(x[:, 0], x[:, 1]), op(x[:, 2], x[:, 3])), x[:, 4])
        r = op(r, pltpu.roll(r, 2, 1))
        return op(r, pltpu.roll(r, 4, 1))

    def feature_map(pt):
        p = pt.reshape(-1, 5, 8, TB)
        ep = jnp.exp(p - fold(p, jnp.maximum)[:, None])
        en = jnp.exp(fold(p, jnp.minimum)[:, None] - p)
        ep = ep * _recip(fold(ep, jnp.add))[:, None]
        en = en * _recip(fold(en, jnp.add))[:, None]
        return jnp.concatenate([ep, en], axis=1)

    def rows_of(b):
        if isinstance(b, int):
            return pl.ds(b * TB, TB), pl.ds(b * TB // 2, TB // 2)
        return pl.ds(pl.multiple_of(b * TB, TB), TB), pl.ds(pl.multiple_of(b * (TB // 2), TB // 2), TB // 2)

    CG = 4
    NC = NG // CG
    CR = CG * GR

    def k_blocks(blocks, load_x=None, ahead=None, init=False, mid=None):
        xn, v, phi = {}, {}, {}

        def LN(j):
            rows, prows = rows_of(blocks[j] if j < len(blocks) else ahead)
            if load_x is not None and j > 0:
                xn[j] = _layernorm(load_x(rows)).astype(bf16)
                xna_ref[prows, :] = pltpu.bitcast(xn[j], u32)
            else:
                xn[j] = _unpack(xna_ref[prows, :])

        def P(j, c):
            pk = _dot_nt(_unpack(wpkt_ref[c * CR // 2:(c + 1) * CR // 2, :]), xn[j])
            f = feature_map(pk).reshape(2 * CR, TB)
            for g in range(CG):
                phi[j, CG * c + g] = f[2 * GR * g:2 * GR * (g + 1)].astype(bf16)

        def V(j, c):
            vt = _dot_nt(_unpack(wvt_ref[c * CR // 2:(c + 1) * CR // 2, :]), xn[j])
            for g in range(CG):
                v[j, CG * c + g] = jnp.concatenate([vt[GR * g:GR * (g + 1)], jnp.ones((8, TB), f32)], axis=0).astype(bf16)

        def KV(j):
            for g in range(NG):
                r = _dot_nt(v[j, g], phi[j, g])
                if init and j == 0:
                    acc_ref[g] = r
                else:
                    acc_ref[g] += r

        LN(0)
        for j in range(len(blocks)):
            if j + 1 < len(blocks) or ahead is not None:
                LN(j + 1)
            for c in range(NC):
                P(j, c)
            if mid is not None:
                mid()
            for c in range(NC):
                V(j, c)
            KV(j)

    def finish_kv():
        r48, odd = _iota((48, 2 * GR), 0), (_iota((48, 2 * GR), 1) & 1) == 1
        same = (((r48 >= FA) & (r48 < GR)) | (r48 >= GR + 4)) == odd
        for g in range(NG):
            kvt_ref[g] = _pack(jnp.where(same, acc_ref[g], 0.0))

    def q_blocks(blocks, load_x, hooks, between=None):
        top = _iota((8, TB), 0) < 4
        phi, ot, o, y = {}, {}, {}, {}
        n = len(blocks)

        def P(j):
            xn = _unpack(xna_ref[rows_of(blocks[j])[1], :])
            for c in range(NC):
                f = feature_map(_dot_nt(_unpack(wpqt_ref[c * CR // 2:(c + 1) * CR // 2, :]), xn)).reshape(2 * CR, TB)
                for g in range(CG):
                    phi[j, CG * c + g] = f[2 * GR * g:2 * GR * (g + 1)].astype(bf16)

        def N(j):
            outs = []
            for g in range(NG):
                num = _dot(_unpack(kvt_ref[g]), phi[j, g])
                rm = 1.0 / (num[GR:] + 1e-6)
                rs = pltpu.roll(rm, 4, 0)
                r0, r1 = jnp.where(top, rm, rs), jnp.where(top, rs, rm)
                outs.append(num[:GR] * jnp.concatenate([r0, r0, rm, r1, r1], axis=0))
            ot[j] = jnp.concatenate(outs, axis=0)

        def W(j, t):
            if t == 0:
                o_ref[j] = pltpu.bitcast(ot[j].astype(bf16).T, u32)
                o[j] = _unpack(o_ref[j])
            y[j, t] = _dot(o[j], woa_ref[:, 128 * t:128 * t + 128])
            if t == 4:
                rows = rows_of(blocks[j])[0]
                xres_ref[rows, :] = load_x(rows) + jnp.concatenate([y[j, t] for t in range(5)], axis=1)

        def WW(j):
            for t in range(5):
                W(j, t)
                if (j, t) in hooks:
                    hooks[j, t]()

        P(0), P(1)
        if between is not None:
            between()
        N(0), P(2), N(1), WW(0), N(2)
        for j in range(3, n):
            P(j), WW(j - 2), N(j)
        WW(n - 2), WW(n - 1)

    VPERM = [(h * DHB + 64 * c) for c in range(3) for h in range(2)]

    def relayout_weights(j):
        r0 = pl.multiple_of(j * PW, PW)
        for m in range(2):
            wb_ref[j, :, m * PW:(m + 1) * PW] = pltpu.bitcast(stage_ref[m, pl.ds(r0, PW), :].T, u32)
        for c in range(3):
            w = jnp.concatenate([stage_ref[2, pl.ds(pl.multiple_of(r0 + o, 64), 64), :] for o in VPERM[2 * c:2 * c + 2]], axis=0)
            wb_ref[j, :, 2 * PW + 128 * c:2 * PW + 128 * (c + 1)] = pltpu.bitcast(w.T, u32)

    scale = DHB ** -0.5
    NQ = 32
    row, col = _iota((2 * NQ, 2 * L), 0), _iota((2 * NQ, 2 * L), 1)
    same = (row < NQ) == (col < L)
    rr = jnp.where(row < NQ, row, row - NQ)
    kk = jnp.where(col < L, col, col - L)
    keep = same & ((rr < MEM) | (rr >= kk) | (kk >= NQ))
    fill = jnp.where(same, -1e9 / scale, -jnp.inf).astype(f32)
    lo = lambda n, w=128: (_iota((n, w), 1) & 64) == 0
    sub8 = _iota((8, 128), 0)

    def halves(x):
        m = lo(*x.shape)
        return jnp.concatenate([jnp.where(m, x, 0.0), jnp.where(m, 0.0, x)], axis=0).astype(bf16)

    def outer(x):
        return jnp.concatenate([x[:, 0:128], x[:, 256:384]], axis=0).astype(bf16)

    def scores(q, k):
        s1 = _dot_nt(outer(q), outer(k))
        s2 = _dot_nt(q[:, 128:256].astype(bf16), halves(k[:, 128:256]))
        s = s1 + jnp.concatenate([s2, s2], axis=0)
        s = jnp.where(keep, s, fill)
        e = jnp.exp2((s - jnp.max(s, axis=1, keepdims=True)) * (scale * LOG2E))
        return e, jnp.sum(e, axis=1, keepdims=True)

    def values(e, l, v):
        rab = _recip(jnp.where(lo(NQ), l[:NQ], l[NQ:]))
        return _dot((e[:NQ] + e[NQ:]).astype(bf16), halves(v)) * jnp.concatenate([rab] * 3, axis=1)

    def head_attention(q, kv):
        rot = lambda x, r: pltpu.roll(x, r % 8, 0) if r % 8 else x
        tile = lambda x, c: x[:, 128 * c:128 * c + 128]
        q = q * (scale * LOG2E)
        ks = []
        for b in range(2):
            kb = kv[8 * b:8 * b + 8]
            ks.append((tile(kb, 0), jnp.where(lo(8), tile(kb, 1), 0.0), jnp.where(lo(8), 0.0, tile(kb, 1)), tile(kb, 2)))
        ss, m = {}, None
        for r in range(7, -1, -1):
            qr = [rot(tile(q, c), 8 - r) for c in range(3)]
            for b in range(2):
                k0, kl, kh, k2 = ks[b]
                sa = jnp.sum(qr[0] * k0 + qr[1] * kl, axis=1, keepdims=True)
                sb = jnp.sum(qr[2] * k2 + qr[1] * kh, axis=1, keepdims=True)
                x = jnp.where(lo(8), sa, sb)
                if b == 1 and r > 0:
                    x = jnp.where(sub8 <= 7 - r, x, -1e9 * LOG2E)
                ss[b, r] = x
            mx = jnp.maximum(ss[0, r], ss[1, r])
            m = mx if m is None else jnp.maximum(rot(m, 1), mx)
        acc = None
        for r in range(7, -1, -1):
            mr = rot(m, 8 - r)
            e0, e1 = jnp.exp2(ss[0, r] - mr), jnp.exp2(ss[1, r] - mr)
            t = [e0 + e1] + [e0 * tile(kv[0:8], 3 + c) + e1 * tile(kv[8:16], 3 + c) for c in range(3)]
            acc = t if acc is None else [rot(u, 1) + w for u, w in zip(acc, t)]
        r = _recip(acc[0])
        return jnp.concatenate([acc[1] * r, acc[2] * r, acc[3] * r], axis=1)

    def bstep(h, first, never, early, chained_in, chained_out, pre=None):
        qkv, ps, os_, ov = {}, {}, {}, {}
        acc = [None]
        nxt = [0]

        split = pre is not None and first

        def is_long(first, t, m):
            flipped = FLIP.get(t) == m
            return (flipped and not first) if pre is not None else first != flipped

        def PR(t, ms):
            hs = {m: h if is_long(first, t, m) else h[:NQ] for m in ms}
            if t == 0 and chained_in:
                rs = {}
                for k in range(5):
                    for m in ms:
                        c = _dot(hs[m][:, 128 * k:128 * k + 128].astype(bf16),
                                 _unpack(wb_ref[t, 64 * k:64 * k + 64, m * PW:(m + 1) * PW]))
                        rs[m] = c if k == 0 else rs[m] + c
            else:
                rs = {m: _dot(hs[m].astype(bf16), _unpack(wb_ref[t, :, m * PW:(m + 1) * PW])) for m in ms}
            for m in ms:
                if is_long(first, t, m):
                    svq_ref[t, :, m * PW:(m + 1) * PW] = rs[m][L:]
                    qkv[t, m] = rs[m][:L]
                else:
                    cols = slice(m * PW, (m + 1) * PW)
                    saved = svq_ref[t, :, cols] if pre is None else pre_ref[t, pl.ds(pl.multiple_of(pre * 8, 8), 8), cols]
                    qkv[t, m] = jnp.concatenate([rs[m], saved], axis=0)
            if not (split and t >= NP - 2):
                HA_(t)

        def HA_(t):
            kv = jnp.concatenate([qkv[t, 1], qkv[t, 2]], axis=1)
            ov[t] = head_attention(qkv[t, 0][NQ:], jnp.concatenate([kv[:MEM], kv[NQ:]], axis=0))

        def SS(j):
            ps[j] = scores(qkv[j, 0][:NQ], qkv[j, 1])

        def PV(j):
            e, l = ps[j]
            ja = j - (1 if split else ANCHOR_A if first else ANCHOR_B)
            if ja >= 0:
                e = jnp.concatenate([jnp.where(never, ov[ja][:, 128 * c:128 * c + 2 * L], e[8 * c:8 * c + 8])
                                     for c in range(3)] + [e[24:]], axis=0)
            if j in early:
                e = jnp.concatenate([e[:24], jnp.where(never, early[j][:, :2 * L], e[24:32]), e[32:]], axis=0)
            o = values(e, l, qkv[j, 2])
            if first:
                svo_ref[j] = o[24:32]
                o = jnp.concatenate([o[:24], ov[j]], axis=0)
            else:
                o = jnp.concatenate([o, ov[j], svo_ref[j]], axis=0)
            os_[j] = o

        def OO(merge=1):
            js = range(nxt[0], nxt[0] + merge)
            ws = []
            for j in js:
                if pre is not None:
                    ws.append(jnp.concatenate(
                        [pltpu.bitcast(stage_ref[3, j * PW + o:j * PW + o + 64, :], u32) for o in VPERM], axis=0))
                    if not first:
                        wob_ref[j] = ws[-1]
                else:
                    ws.append(wob_ref[j])
            c = _dot(jnp.concatenate([os_[j] for j in js], axis=1).astype(bf16), _unpack(jnp.concatenate(ws, axis=0)))
            acc[0] = c if acc[0] is None else acc[0] + c
            nxt[0] += merge

        order, tail = (ORD_A, TAIL_W if split else TAIL_A) if first else (ORD_B, TAIL_C if chained_out else TAIL_B)
        olag = OLAG_A if first else OLAG_B
        nl = (3 if split else MERGE_A) if first else 1
        nd = tail.count("O") + nl
        for t in range(NP):
            for op in order:
                if op == "Q":
                    PR(t, PORD_A if first else PORD_B)
                    if split and t == NP - 1:
                        pl.when(pre == 0)(lambda: cp_wob.wait())
                        HA_(NP - 2), HA_(NP - 1)
                if op == "S" and t >= 1:
                    SS(t - 1)
                if op == "P" and t >= 2:
                    PV(t - 2)
                if op == "O" and olag <= t < NP - 1 and nxt[0] < NP - nd:
                    OO()
        p = NP - 2
        for op in tail:
            if op == "O":
                OO()
            if op == "S":
                SS(NP - 1)
            if op == "P":
                PV(p)
                p += 1
        OO(nl)
        assert nxt[0] == NP and p == NP
        return acc[0]

    def bpass(last, lo_it, hi_it, warm=False):
        def body(i, c):
            never = flag_ref[:, :2 * L] > 0
            probe = lambda x, g: x[8 * g:8 * g + 8, 0:128]
            mem = mem_ref[...]
            if warm:
                slots = [pl.ds(pl.multiple_of(i * 64, 64), 64)]
                heads = [xnb_ref[pl.ds(pl.multiple_of((1 - i) * 64, 64), 8), :]]
            else:
                slots = [pl.ds(0, 64), pl.ds(64, 64)]
            xs = [xnb_ref[sl, :] for sl in slots]
            n = len(slots)
            for u in range(n):
                r0 = pl.multiple_of((i * n + u) * 64, 64)
                xa = xs[u]
                rn = pl.multiple_of(jnp.minimum(r0 + 128, S - 64), 64)
                xn = _layernorm(xres_ref[pl.ds(rn, 64), :])
                xnb_ref[slots[u], :] = xn
                if not warm and u == 0:
                    heads = [xs[1][0:8], xn[0:8]]
                early = {LN_AT + g: probe(xn, g) for g in range(8)}
                if not last:
                    rp = pl.multiple_of(jnp.maximum(r0 - 64, 0), 64)
                    xn = _layernorm(xres_ref[pl.ds(rp, 64), :])
                    xna_ref[pl.ds(pl.multiple_of(rp // 2, 32), 32), :] = _pack(xn)
                    for g in range(8):
                        j = LN_AT2 + g
                        early[j] = jnp.maximum(early[j], probe(xn, g)) if j in early else probe(xn, g)
                ya = bstep(jnp.concatenate([mem, xa[8:32], xa[0:8], xa[32:40]], axis=0), True, never, early,
                           u > 0, True, 2 * i if warm else None)
                yb = bstep(jnp.concatenate([ya[:MEM], xa[40:64], xa[32:40], heads[u]], axis=0), False, never, {},
                           True, u < n - 1, 2 * i + 1 if warm else None)
                mem = yb[:MEM]
                y = xres_ref[pl.ds(r0, 64), :] + jnp.concatenate([ya[24:32], ya[MEM:24], yb[40:48], yb[32:40], yb[MEM:32]], axis=0)
                if last:
                    out_ref[pl.ds(r0, 64), :] = y.astype(bf16)
                else:
                    xres_ref[pl.ds(r0, 64), :] = y
            mem_ref[...] = mem
            if last:
                rows = pl.ds(pl.multiple_of(i * 128, 128), 128)
                pltpu.make_async_copy(out_ref.at[rows, :], out_hbm.at[rows, :], sems.at[7]).start()
            return c
        lax.fori_loop(lo_it, hi_it, body, 0)

    load_in = lambda rows: x_ref[rows, :].astype(f32)
    load_res = lambda rows: xres_ref[rows, :]
    NB = S // (TB * NCH)

    def k1_body(i, c):
        pl.when(i == 1)(lambda: cp_x(3).wait())
        k_blocks([1 + i * KB + j for j in range(KB)], load_in, jnp.minimum(1 + i * KB + KB, S // TB - 1))
        return c

    def q1_body(i, c):
        for m in range(3):
            cp_w(m, i).wait()
        pairs = [i * (NP // NCH) + j for j in range(NP // NCH)]
        for j in pairs:
            relayout_weights(j)
        head = []

        def norm_first():
            x0 = _layernorm(xres_ref[0:128, :])
            xnb_ref[...] = x0
            head.append(jnp.concatenate([x0[32 * sg:32 * sg + 8] for sg in range(4)], axis=0).astype(bf16))

        def project(js):
            for j in js:
                pre_ref[j] = _dot(head[0], _unpack(wb_ref[j]))

        q_blocks([i * NB + j for j in range(NB)], load_in,
                 {(0, 4): norm_first, (1, 4): lambda: project(pairs[:1]), (2, 4): lambda: project(pairs[1:3]),
                  (3, 4): lambda: project(pairs[3:])})
        return c

    with _scope("pro"):
        flag_ref[...] = jnp.zeros(flag_ref.shape, jnp.int32)
        cnt_ref[0] = 0
        cp_phi.wait()
        cp_x(0).wait()
        phi_lhs = phi_blocks()
        xna_ref[0:TB // 2, :] = _pack(_layernorm(load_in(pl.ds(0, TB))))
        cp_wqkv(1).wait()
        fold_phi(phi_lhs, 1, wpkt_ref)

        def values_ready():
            cp_wqkv(2).wait()
            cp_x(1).wait()
            wvt_ref[...] = pltpu.bitcast(wqkv_ref[2].T, u32)
            xna_ref[TB // 2:TB, :] = _pack(_layernorm(load_in(pl.ds(TB, TB))))

        k_blocks([0], init=True, mid=values_ready)
        cp_x(2).wait()
    with _scope("k1"):
        lax.fori_loop(0, (S // TB - 1) // KB, k1_body, 0)
    with _scope("f1"):
        cp_wqkv(0).wait()
        cp_woa.wait()
        cp_mem.wait()
        fold_phi(phi_lhs, 0, wpqt_ref)
        finish_kv()
        mem_ref[...] = mem0_ref[...].astype(f32)
    with _scope("q1"):
        lax.fori_loop(0, NCH, q1_body, 0)
    with _scope("b1w"):
        bpass(False, 0, 2, warm=True)
    with _scope("b1"):
        bpass(False, 1, S // 128)
    with _scope("a2"):
        lax.fori_loop(0, cnt_ref[0] + 1, lambda i, c: (k_blocks(list(range(KSPLIT)), init=True), c)[1], 0)
        xna_ref[(S - 64) // 2:, :] = _pack(_layernorm(xres_ref[S - 64:, :]))
        k_blocks(list(range(KSPLIT, S // TB)))
        head = []

        def norm_first():
            x0 = _layernorm(xres_ref[0:128, :])
            xnb_ref[...] = x0
            head.append(x0[0:16].astype(bf16))

        def save_rows(t, c):
            svq_ref[t, :, c:c + 128] = _dot(head[0], _unpack(wb_ref[t, :, c:c + 128]))[:8]

        hooks = {(0, 4): norm_first}
        pieces = [(t, m * PW + 128 * c) for t, m in FLIP.items() for c in range(3)]
        for n, piece in enumerate(pieces):
            hooks[2 + n // 2, 1 + 2 * (n % 2)] = functools.partial(save_rows, *piece)
        q_blocks(list(range(S // TB)), load_res, hooks, between=finish_kv)
        mem_ref[...] = mem0_ref[...].astype(f32)
    with _scope("b2"):
        bpass(True, 0, S // 128)
    pltpu.make_async_copy(out_ref, out_hbm, sems.at[7]).wait()


@functools.partial(jax.jit, static_argnames=("B_seg_len",))
def pallas_interleave_layers__linear_kernel_hedgehog__memory_aug_recurrent_mem_tr__prompt_kernel(
    A_x: jax.Array,
    A_wqkv: jax.Array,
    A_w_phi: jax.Array,
    A_wo: jax.Array,
    B_x: jax.Array,
    B_mem0: jax.Array,
    B_Wq: jax.Array,
    B_Wk: jax.Array,
    B_Wv: jax.Array,
    B_Wo: jax.Array,
    B_seg_len: int,
):
    del B_x
    assert B_seg_len == SEG
    assert A_x.shape == (1, S, D) and B_mem0.shape == (1, MEM, D)
    assert B_Wq.shape == (D, HB, DHB) and A_w_phi.shape == (HA, FA, FA)
    tr = lambda w: jnp.transpose(w, (1, 2, 0)).reshape(HB * DHB, D)
    hbm = pl.BlockSpec(memory_space=pl.ANY)
    out = pl.pallas_call(
        _kernel,
        out_shape=jax.ShapeDtypeStruct((S, D), bf16),
        in_specs=[hbm] * 9,
        out_specs=hbm,
        scratch_shapes=[
            pltpu.VMEM((S, D), bf16),
            pltpu.VMEM((3, D, D), bf16),
            pltpu.VMEM((FA, FA, HA), bf16),
            pltpu.VMEM((D, D), bf16),
            pltpu.VMEM((MEM, D), bf16),
            pltpu.VMEM((S, D), bf16),
            pltpu.VMEM((4, HB * DHB, D), bf16),
            pltpu.VMEM((NP, D // 2, 3 * PW), u32),
            pltpu.VMEM((NP, PW // 2, D), u32),
            pltpu.VMEM((S, D), f32),
            pltpu.VMEM((S // 2, D), u32),
            pltpu.VMEM((128, D), f32),
            pltpu.VMEM((D // 2, D), u32),
            pltpu.VMEM((D // 2, D), u32),
            pltpu.VMEM((D // 2, D), u32),
            pltpu.VMEM((NG, 48, 2 * GR), f32),
            pltpu.VMEM((NG, 24, 2 * GR), u32),
            pltpu.VMEM((S // TB, TB // 2, D), u32),
            pltpu.VMEM((MEM, D), f32),
            pltpu.VMEM((NP, 8, 3 * PW), f32),
            pltpu.VMEM((NP, 32, 3 * PW), f32),
            pltpu.VMEM((NP, 8, PW), f32),
            pltpu.VMEM((8, 128), jnp.int32),
            pltpu.SMEM((1,), jnp.int32),
            pltpu.SemaphoreType.DMA((12 + 3 * NCH,)),
        ],
        compiler_params=pltpu.CompilerParams(vmem_limit_bytes=120 * 1024 * 1024),
        name="hedgehog_rmt",
    )(A_x.reshape(S, D), A_wqkv, jnp.transpose(A_w_phi, (1, 2, 0)), A_wo, B_mem0.reshape(MEM, D),
      tr(B_Wq), tr(B_Wk), tr(B_Wv), B_Wo.reshape(HB * DHB, D))
    return out.reshape(1, S, D)
```

```python
import contextlib
import functools

import jax
import jax.numpy as jnp
from jax import lax
import jax.experimental.pallas as pl
import jax.experimental.pallas.tpu as pltpu

f32, bf16, u32 = jnp.float32, jnp.bfloat16, jnp.uint32

S, D = 2048, 640
HA, FA = 32, 20
HB, DHB = 32, 192
MEM, SEG = 8, 32
L = MEM + SEG
NP = HB // 2
PW = 2 * DHB
TB = 128
NG = 16
GR = 2 * FA
NCH = 4
NT = (((1,), (1,)), ((), ()))
LOG2E = 1.4426950408889634

FLIP = {0: 2, 2: 2, 3: 2, 6: 1, 8: 1, 13: 2, 14: 2, 15: 2}
ORD_A, ORD_B = "QSPO", "QOPS"
TAIL_A, TAIL_B, TAIL_C, TAIL_W = "OOOSPOOOPOO", "OOSPOOPO", "OOSPOOPO", "SOOOOPOOOPOOOOOO"
PORD_A, PORD_B = (1, 2, 0), (0, 1, 2)
OLAG_A, OLAG_B = 4, 4
MERGE_A = 2
LATE, LATE_AT = 2, 3
ANCHOR_A, ANCHOR_B = 0, 1
LN_AT, LN_AT2 = 0, 3
KB = 3
KSPLIT = 7


_scope = lambda name: contextlib.nullcontext()


def _dot(a, b):
    return jnp.dot(a, b, preferred_element_type=f32)


def _dot_nt(a, b):
    return lax.dot_general(a, b, NT, preferred_element_type=f32)


def _pack(x):
    return pltpu.bitcast(x.astype(bf16), u32)


def _unpack(x):
    return pltpu.bitcast(x, bf16)


def _recip(x):
    r = pl.reciprocal(x, approx=True)
    return r * (2.0 - x * r)


def _layernorm(x):
    m = jnp.mean(x, axis=-1, keepdims=True)
    xc = x - m
    v = jnp.mean(xc * xc, axis=-1, keepdims=True)
    return xc * lax.rsqrt(v + 1e-5)


def _iota(shape, dim):
    return lax.broadcasted_iota(jnp.int32, shape, dim)


def _kernel(x_hbm, wqkv_hbm, wphi_hbm, woa_hbm, mem0_hbm, wqt_hbm, wkt_hbm, wvt_hbm, wob_hbm,
            out_hbm,
            x_ref, wqkv_ref, wphi_ref, woa_ref, mem0_ref, out_ref,
            stage_ref, wb_ref, wob_ref, xres_ref, xna_ref, xnb_ref,
            wpqt_ref, wpkt_ref, wvt_ref, acc_ref, kvt_ref, o_ref,
            mem_ref, svq_ref, pre_ref, svo_ref, flag_ref, cnt_ref, sems):
    WC = HB * DHB // NCH
    X_CUTS = (0, TB, 2 * TB, (2 + KB) * TB, S)

    def cp_wqkv(m):
        return pltpu.make_async_copy(wqkv_hbm.at[:, pl.ds(m * D, D)], wqkv_ref.at[m], sems.at[m])

    def cp_x(n):
        rows = pl.ds(X_CUTS[n], X_CUTS[n + 1] - X_CUTS[n])
        return pltpu.make_async_copy(x_hbm.at[rows, :], x_ref.at[rows, :], sems.at[8 + n])

    def cp_w(m, i):
        rows = pl.ds(pl.multiple_of(i * WC, WC), WC)
        return pltpu.make_async_copy((wqt_hbm, wkt_hbm, wvt_hbm)[m].at[rows, :], stage_ref.at[m, rows, :],
                                     sems.at[12 + NCH * m + i])

    cp_phi = pltpu.make_async_copy(wphi_hbm, wphi_ref, sems.at[3])
    cp_woa = pltpu.make_async_copy(woa_hbm, woa_ref, sems.at[4])
    cp_mem = pltpu.make_async_copy(mem0_hbm, mem0_ref, sems.at[5])
    cp_wob = pltpu.make_async_copy(wob_hbm, stage_ref.at[3], sems.at[6])
    cp_phi.start()
    cp_x(0).start()
    cp_wqkv(1).start()
    cp_wqkv(2).start()
    cp_x(1).start()
    cp_x(2).start()
    cp_x(3).start()
    cp_wqkv(0).start()
    cp_woa.start()
    cp_mem.start()
    for i in range(NCH):
        for m in range(3):
            cp_w(m, i).start()
    cp_wob.start()

    def phi_blocks():
        wphi = wphi_ref[...].astype(f32)
        cat = jnp.concatenate([wphi[d] for d in range(FA)], axis=1)
        cat = jnp.concatenate([cat, jnp.zeros((32 - FA, D), f32)], axis=0).astype(bf16)
        p_row, p_col = _iota((D, D), 0), _iota((D, D), 1)
        spread = (FA * (p_row & 31) + (p_row >> 5) == p_col).astype(f32).astype(bf16)
        u = _dot(cat, spread).astype(bf16)
        dup = ((_iota((48, 32), 0) >> 1) == _iota((48, 32), 1)).astype(f32).astype(bf16)
        u2 = _dot(dup, u)[:GR]
        lane, par = _iota((GR, 128), 1), _iota((GR, 128), 0) & 1
        lhs = []
        for c in range(5):
            blocks = []
            for g in range(3 * c, 3 * c + 4):
                lo = GR * g - 128 * c + FA * par
                blocks.append(jnp.where((lane >= lo) & (lane < lo + FA), u2[:, 128 * c:128 * c + 128], 0.0))
            lhs.append(jnp.concatenate(blocks, axis=0).astype(bf16))
        return lhs

    def fold_phi(lhs, m, dst):
        parts = [_dot_nt(lhs[c], wqkv_ref[m, :, 128 * c:128 * c + 128]) for c in range(5)]
        rows = []
        for c in range(5):
            first = parts[c][:GR] if c == 0 else parts[c][:GR] + parts[c - 1][3 * GR:]
            rows += [first, parts[c][GR:3 * GR]]
        rows.append(parts[4][3 * GR:])
        dst[...] = _pack(jnp.concatenate(rows, axis=0))

    def fold(x, red, op):
        r = red(x, axis=1)
        r = op(r, pltpu.roll(r, 2, 1))
        return op(r, pltpu.roll(r, 4, 1))

    def feature_map(pt):
        p = pt.reshape(-1, 5, 8, TB)
        ep = jnp.exp(p - fold(p, jnp.max, jnp.maximum)[:, None])
        en = jnp.exp(fold(p, jnp.min, jnp.minimum)[:, None] - p)
        ep = ep * _recip(fold(ep, jnp.sum, jnp.add))[:, None]
        en = en * _recip(fold(en, jnp.sum, jnp.add))[:, None]
        return jnp.concatenate([ep, en], axis=1)

    def rows_of(b):
        if isinstance(b, int):
            return pl.ds(b * TB, TB), pl.ds(b * TB // 2, TB // 2)
        return pl.ds(pl.multiple_of(b * TB, TB), TB), pl.ds(pl.multiple_of(b * (TB // 2), TB // 2), TB // 2)

    CG = 4
    NC = NG // CG
    CR = CG * GR

    def k_blocks(blocks, load_x=None, ahead=None, init=False, mid=None):
        xn, v, phi = {}, {}, {}
        ones8 = jnp.ones((8, TB), f32)

        def LN(j):
            rows, prows = rows_of(blocks[j] if j < len(blocks) else ahead)
            if load_x is not None and j > 0:
                xn[j] = _layernorm(load_x(rows)).astype(bf16)
                xna_ref[prows, :] = pltpu.bitcast(xn[j], u32)
            else:
                xn[j] = _unpack(xna_ref[prows, :])

        def P(j, c):
            pk = _dot_nt(_unpack(wpkt_ref[c * CR // 2:(c + 1) * CR // 2, :]), xn[j])
            f = feature_map(pk).reshape(2 * CR, TB)
            for g in range(CG):
                phi[j, CG * c + g] = f[2 * GR * g:2 * GR * (g + 1)].astype(bf16)

        def V(j, c):
            vt = _dot_nt(_unpack(wvt_ref[c * CR // 2:(c + 1) * CR // 2, :]), xn[j])
            for g in range(CG):
                v[j, CG * c + g] = jnp.concatenate([vt[GR * g:GR * (g + 1)], ones8], axis=0).astype(bf16)

        def KV(j):
            for g in range(NG):
                r = _dot_nt(v[j, g], phi[j, g])
                if init and j == 0:
                    acc_ref[g] = r
                else:
                    acc_ref[g] += r

        LN(0)
        for j in range(len(blocks)):
            if j + 1 < len(blocks) or ahead is not None:
                LN(j + 1)
            for c in range(NC):
                P(j, c)
            if mid is not None:
                mid()
            for c in range(NC):
                V(j, c)
            KV(j)

    def finish_kv():
        r48, odd = _iota((48, 2 * GR), 0), (_iota((48, 2 * GR), 1) & 1) == 1
        same = (((r48 >= FA) & (r48 < GR)) | (r48 >= GR + 4)) == odd
        for g in range(NG):
            kvt_ref[g] = _pack(jnp.where(same, acc_ref[g], 0.0))

    def q_blocks(blocks, load_x, hooks, between=None):
        top = _iota((NG, 8, TB), 1) < 4
        phi, ot, o, y = {}, {}, {}, {}
        n = len(blocks)

        def P(j):
            xn = _unpack(xna_ref[rows_of(blocks[j])[1], :])
            for c in range(NC):
                f = feature_map(_dot_nt(_unpack(wpqt_ref[c * CR // 2:(c + 1) * CR // 2, :]), xn)).reshape(2 * CR, TB)
                for g in range(CG):
                    phi[j, CG * c + g] = f[2 * GR * g:2 * GR * (g + 1)].astype(bf16)

        def N(j):
            num = jnp.concatenate([_dot(_unpack(kvt_ref[g]), phi[j, g]) for g in range(NG)], axis=0).reshape(NG, 48, TB)
            rm = 1.0 / (num[:, GR:] + 1e-6)
            rs = pltpu.roll(rm, 4, 1)
            r0, r1 = jnp.where(top, rm, rs), jnp.where(top, rs, rm)
            ot[j] = (num[:, :GR] * jnp.concatenate([r0, r0, rm, r1, r1], axis=1)).reshape(D, TB)

        def W(j, t):
            if t == 0:
                o_ref[j] = pltpu.bitcast(ot[j].astype(bf16).T, u32)
                o[j] = _unpack(o_ref[j])
            y[j, t] = _dot(o[j], woa_ref[:, 128 * t:128 * t + 128])
            if t == 4:
                rows = rows_of(blocks[j])[0]
                xres_ref[rows, :] = load_x(rows) + jnp.concatenate([y[j, t] for t in range(5)], axis=1)

        def WW(j):
            for t in range(5):
                W(j, t)
                if (j, t) in hooks:
                    hooks[j, t]()

        P(0), P(1)
        if between is not None:
            between()
        N(0), P(2), N(1), WW(0), N(2)
        for j in range(3, n):
            P(j), WW(j - 2), N(j)
        WW(n - 2), WW(n - 1)

    VPERM = [(h * DHB + 64 * c) for c in range(3) for h in range(2)]

    def relayout_weights(j):
        r0 = pl.multiple_of(j * PW, PW)
        for m in range(2):
            wb_ref[j, :, m * PW:(m + 1) * PW] = pltpu.bitcast(stage_ref[m, pl.ds(r0, PW), :].T, u32)
        for c in range(3):
            w = jnp.concatenate([stage_ref[2, pl.ds(pl.multiple_of(r0 + o, 64), 64), :] for o in VPERM[2 * c:2 * c + 2]], axis=0)
            wb_ref[j, :, 2 * PW + 128 * c:2 * PW + 128 * (c + 1)] = pltpu.bitcast(w.T, u32)

    scale = DHB ** -0.5
    NQ = 32
    row, col = _iota((2 * NQ, 2 * L), 0), _iota((2 * NQ, 2 * L), 1)
    same = (row < NQ) == (col < L)
    rr = jnp.where(row < NQ, row, row - NQ)
    kk = jnp.where(col < L, col, col - L)
    keep = same & ((rr < MEM) | (rr >= kk) | (kk >= NQ))
    fill = jnp.where(same, -1e9 / scale, -jnp.inf).astype(f32)
    lo = {sh: (_iota(sh, len(sh) - 1) & 64) == 0 for sh in ((L, 128), (L, PW), (NQ, 128), (16, 128), (8, 8, 128))}
    causal = _iota((8, 8, 128), 1) <= _iota((8, 8, 128), 0)

    def halves(x):
        m = lo[x.shape]
        return jnp.concatenate([jnp.where(m, x, 0.0), jnp.where(m, 0.0, x)], axis=0).astype(bf16)

    def outer(x):
        return jnp.concatenate([x[:, 0:128], x[:, 256:384]], axis=0).astype(bf16)

    def scores(q, k):
        s1 = _dot_nt(outer(q), outer(k))
        s2 = _dot_nt(q[:, 128:256].astype(bf16), halves(k[:, 128:256]))
        s = s1 + jnp.concatenate([s2, s2], axis=0)
        s = jnp.where(keep, s, fill)
        e = jnp.exp2((s - jnp.max(s, axis=1, keepdims=True)) * (scale * LOG2E))
        return e, jnp.sum(e, axis=1, keepdims=True)

    def values(e, l, v):
        rab = _recip(jnp.where(lo[NQ, 128], l[:NQ], l[NQ:]))
        return _dot((e[:NQ] + e[NQ:]).astype(bf16), halves(v)) * jnp.concatenate([rab] * 3, axis=1)

    def head_attention(q, k, v):
        steps = lambda x: jnp.stack([pltpu.roll(x, i + 1, 0) for i in range(7)] + [x])
        qr = steps(q * (scale * LOG2E))
        mid = k[:, 128:256]
        ka = jnp.concatenate([k[:, 0:128], jnp.where(lo[16, 128], mid, 0.0)], axis=1)
        kb = jnp.concatenate([jnp.where(lo[16, 128], 0.0, mid), k[:, 256:384]], axis=1)
        qa, qb = qr[:, :, 0:256], qr[:, :, 128:384]
        ss = []
        for b in range(2):
            sa = jnp.sum(qa * ka[8 * b:8 * b + 8][None], axis=2, keepdims=True)
            sb = jnp.sum(qb * kb[8 * b:8 * b + 8][None], axis=2, keepdims=True)
            ss.append(jnp.where(lo[8, 8, 128], sa, sb))
        ss[1] = jnp.where(causal, ss[1], -1e9 * LOG2E)

        def unrotate(x, op):
            r = x[0]
            for i in range(1, 8):
                r = op(pltpu.roll(r, 1, 0), x[i])
            return r

        m = steps(unrotate(jnp.maximum(ss[0], ss[1]), jnp.maximum))
        e0, e1 = jnp.exp2(ss[0] - m), jnp.exp2(ss[1] - m)
        t = jnp.concatenate([e0] * 3, axis=2) * v[0:8][None] + jnp.concatenate([e1] * 3, axis=2) * v[8:16][None]
        acc = unrotate(jnp.concatenate([t, e0 + e1], axis=2), jnp.add)
        return acc[:, :PW] * jnp.concatenate([_recip(acc[:, PW:])] * 3, axis=1)

    def bstep(h, first, never, early, chained_in, chained_out, pre=None):
        qkv, ps, os_, ov = {}, {}, {}, {}
        acc = {}
        nxt = [0]
        late = NP - (3 if pre is not None else LATE)

        split = pre is not None and first

        def is_long(first, t, m):
            flipped = FLIP.get(t) == m
            return (flipped and not first) if pre is not None else first != flipped

        hb = {True: h.astype(bf16), False: h[:NQ].astype(bf16)}

        def PR(t, ms):
            hs = {m: h if is_long(first, t, m) else h[:NQ] for m in ms}
            if t == 0 and chained_in:
                rs = {}
                for k in range(5):
                    for m in ms:
                        c = _dot(hs[m][:, 128 * k:128 * k + 128].astype(bf16),
                                 _unpack(wb_ref[t, 64 * k:64 * k + 64, m * PW:(m + 1) * PW]))
                        rs[m] = c if k == 0 else rs[m] + c
            else:
                rs = {m: _dot(hb[is_long(first, t, m)], _unpack(wb_ref[t, :, m * PW:(m + 1) * PW])) for m in ms}
            for m in ms:
                if is_long(first, t, m):
                    svq_ref[t, :, m * PW:(m + 1) * PW] = rs[m][L:]
                    qkv[t, m] = rs[m][:L]
                else:
                    cols = slice(m * PW, (m + 1) * PW)
                    saved = svq_ref[t, :, cols] if pre is None else pre_ref[t, pl.ds(pl.multiple_of(pre * 8, 8), 8), cols]
                    qkv[t, m] = jnp.concatenate([rs[m], saved], axis=0)
            if not (split and t >= NP - 2):
                HA_(t)

        def HA_(t):
            k, v = [jnp.concatenate([qkv[t, m][:MEM], qkv[t, m][NQ:]], axis=0) for m in (1, 2)]
            ov[t] = head_attention(qkv[t, 0][NQ:], k, v)

        def SS(j):
            ps[j] = scores(qkv[j, 0][:NQ], qkv[j, 1])

        def PV(j):
            e, l = ps[j]
            ja = j - (1 if split else ANCHOR_A if first else ANCHOR_B)
            if ja >= 0 and not (first and ja >= late):
                e = jnp.concatenate([jnp.where(never, ov[ja][:, 128 * c:128 * c + 2 * L], e[8 * c:8 * c + 8])
                                     for c in range(3)] + [e[24:]], axis=0)
            if j in early:
                e = jnp.concatenate([e[:24], jnp.where(never, early[j][:, :2 * L], e[24:32]), e[32:]], axis=0)
            o = values(e, l, qkv[j, 2])
            if first and j >= late:
                svo_ref[j] = ov[j]
            elif first:
                svo_ref[j] = o[24:32]
                o = jnp.concatenate([o[:24], ov[j]], axis=0)
            else:
                o = jnp.concatenate([o, ov[j], svo_ref[j]], axis=0)
            os_[j] = o

        def OO(merge=1):
            js = range(nxt[0], nxt[0] + merge)
            ws = []
            for j in js:
                if pre is not None:
                    ws.append(jnp.concatenate(
                        [pltpu.bitcast(stage_ref[3, j * PW + o:j * PW + o + 64, :], u32) for o in VPERM], axis=0))
                    if not first:
                        wob_ref[j] = ws[-1]
                else:
                    ws.append(wob_ref[j])
            c = _dot(jnp.concatenate([os_[j] for j in js], axis=1).astype(bf16), _unpack(jnp.concatenate(ws, axis=0)))
            for key, part in ((0, c[:-8]), (1 + (js[0] >= late), c[-8:])):
                acc[key] = acc[key] + part if key in acc else part
            nxt[0] += merge

        order, tail = (ORD_A, TAIL_W if split else TAIL_A) if first else (ORD_B, TAIL_C if chained_out else TAIL_B)
        olag = OLAG_A if first else OLAG_B
        nl = (3 if split else MERGE_A) if first else 1
        nd = tail.count("O") + nl
        for t in range(NP):
            for op in order:
                if op == "Q":
                    PR(t, PORD_A if first else PORD_B)
                    if split and t == NP - 1:
                        pl.when(pre == 0)(lambda: cp_wob.wait())
                        HA_(NP - 2), HA_(NP - 1)
                if op == "S" and t >= 1:
                    SS(t - 1)
                if op == "P" and t >= 2:
                    PV(t - 2)
                if op == "O" and olag <= t < NP - 1 and nxt[0] < NP - nd:
                    OO()
        p = NP - 2
        for op in tail:
            if op == "O":
                OO()
            if op == "S":
                SS(NP - 1)
            if op == "P":
                PV(p)
                p += 1
        OO(nl)
        assert nxt[0] == NP and p == NP
        hand = {LATE_AT + n: jnp.maximum(jnp.maximum(ov[j][:, 0:128], ov[j][:, 128:256]), ov[j][:, 256:384])
                for n, j in enumerate(range(late, NP))} if first else None
        return acc[0], acc[1], acc[2], hand

    def bpass(last, lo_it, hi_it, warm=False):
        def body(i, c):
            never = flag_ref[:, :2 * L] > 0
            probe = lambda x, g: x[8 * g:8 * g + 8, 0:128]
            mem = mem_ref[...]
            if warm:
                slots = [pl.ds(pl.multiple_of(i * 64, 64), 64)]
                heads = [xnb_ref[pl.ds(pl.multiple_of((1 - i) * 64, 64), 8), :]]
            else:
                slots = [pl.ds(0, 64), pl.ds(64, 64)]
            xs = [xnb_ref[sl, :] for sl in slots]
            n = len(slots)
            for u in range(n):
                r0 = pl.multiple_of((i * n + u) * 64, 64)
                xa = xs[u]
                rn = pl.multiple_of(jnp.minimum(r0 + 128, S - 64), 64)
                xn = _layernorm(xres_ref[pl.ds(rn, 64), :])
                xnb_ref[slots[u], :] = xn
                if not warm and u == 0:
                    heads = [xs[1][0:8], xn[0:8]]
                early = {LN_AT + g: probe(xn, g) for g in range(8)}
                if not last:
                    rp = pl.multiple_of(jnp.maximum(r0 - 64, 0), 64)
                    xn = _layernorm(xres_ref[pl.ds(rp, 64), :])
                    xna_ref[pl.ds(pl.multiple_of(rp // 2, 32), 32), :] = _pack(xn)
                    for g in range(8):
                        j = LN_AT2 + g
                        early[j] = jnp.maximum(early[j], probe(xn, g)) if j in early else probe(xn, g)
                ya, a0, a24, hand = bstep(jnp.concatenate([mem, xa[8:32], xa[0:8], xa[32:40]], axis=0), True, never, early,
                           u > 0, True, 2 * i if warm else None)
                yb, b24, b0, _ = bstep(jnp.concatenate([ya[:MEM], xa[40:64], xa[32:40], heads[u]], axis=0), False, never, hand,
                           True, u < n - 1, 2 * i + 1 if warm else None)
                mem = yb[:MEM]
                y = xres_ref[pl.ds(r0, 64), :] + jnp.concatenate([a0 + b0, ya[MEM:24], a24 + b24, yb[32:40], yb[MEM:32]], axis=0)
                if last:
                    out_ref[pl.ds(r0, 64), :] = y.astype(bf16)
                else:
                    xres_ref[pl.ds(r0, 64), :] = y
            mem_ref[...] = mem
            if last:
                rows = pl.ds(pl.multiple_of(i * 128, 128), 128)
                pltpu.make_async_copy(out_ref.at[rows, :], out_hbm.at[rows, :], sems.at[7]).start()
            return c
        lax.fori_loop(lo_it, hi_it, body, 0)

    load_in = lambda rows: x_ref[rows, :].astype(f32)
    load_res = lambda rows: xres_ref[rows, :]
    NB = S // (TB * NCH)

    def k1_body(i, c):
        pl.when(i == 1)(lambda: cp_x(3).wait())
        k_blocks([1 + i * KB + j for j in range(KB)], load_in, jnp.minimum(1 + i * KB + KB, S // TB - 1))
        return c

    def q1_body(i, c):
        for m in range(3):
            cp_w(m, i).wait()
        pairs = [i * (NP // NCH) + j for j in range(NP // NCH)]
        for j in pairs:
            relayout_weights(j)
        head = []

        def norm_first():
            x0 = _layernorm(xres_ref[0:128, :])
            xnb_ref[...] = x0
            head.append(jnp.concatenate([x0[32 * sg:32 * sg + 8] for sg in range(4)], axis=0).astype(bf16))

        def project(js):
            for j in js:
                pre_ref[j] = _dot(head[0], _unpack(wb_ref[j]))

        q_blocks([i * NB + j for j in range(NB)], load_in,
                 {(0, 4): norm_first, (1, 4): lambda: project(pairs[:1]), (2, 4): lambda: project(pairs[1:3]),
                  (3, 4): lambda: project(pairs[3:])})
        return c

    with _scope("pro"):
        flag_ref[...] = jnp.zeros(flag_ref.shape, jnp.int32)
        cnt_ref[0] = 0
        cp_phi.wait()
        cp_x(0).wait()
        phi_lhs = phi_blocks()
        xna_ref[0:TB // 2, :] = _pack(_layernorm(load_in(pl.ds(0, TB))))
        cp_wqkv(1).wait()
        fold_phi(phi_lhs, 1, wpkt_ref)

        def values_ready():
            cp_wqkv(2).wait()
            cp_x(1).wait()
            wvt_ref[...] = pltpu.bitcast(wqkv_ref[2].T, u32)
            xna_ref[TB // 2:TB, :] = _pack(_layernorm(load_in(pl.ds(TB, TB))))

        k_blocks([0], init=True, mid=values_ready)
        cp_x(2).wait()
    with _scope("k1"):
        lax.fori_loop(0, (S // TB - 1) // KB, k1_body, 0)
    with _scope("f1"):
        cp_wqkv(0).wait()
        cp_woa.wait()
        cp_mem.wait()
        fold_phi(phi_lhs, 0, wpqt_ref)
        finish_kv()
        mem_ref[...] = mem0_ref[...].astype(f32)
    with _scope("q1"):
        lax.fori_loop(0, NCH, q1_body, 0)
    with _scope("b1w"):
        bpass(False, 0, 2, warm=True)
    with _scope("b1"):
        bpass(False, 1, S // 128)
    with _scope("a2"):
        lax.fori_loop(0, cnt_ref[0] + 1, lambda i, c: (k_blocks(list(range(KSPLIT)), init=True), c)[1], 0)
        xna_ref[(S - 64) // 2:, :] = _pack(_layernorm(xres_ref[S - 64:, :]))
        k_blocks(list(range(KSPLIT, S // TB)))
        head = []

        def norm_first():
            x0 = _layernorm(xres_ref[0:128, :])
            xnb_ref[...] = x0
            head.append(x0[0:16].astype(bf16))

        def save_rows(t, c):
            svq_ref[t, :, c:c + 128] = _dot(head[0], _unpack(wb_ref[t, :, c:c + 128]))[:8]

        hooks = {(0, 4): norm_first}
        pieces = [(t, m * PW + 128 * c) for t, m in FLIP.items() for c in range(3)]
        for n, piece in enumerate(pieces):
            hooks[2 + n // 2, 1 + 2 * (n % 2)] = functools.partial(save_rows, *piece)
        q_blocks(list(range(S // TB)), load_res, hooks, between=finish_kv)
        mem_ref[...] = mem0_ref[...].astype(f32)
    with _scope("b2"):
        bpass(True, 0, S // 128)
    pltpu.make_async_copy(out_ref, out_hbm, sems.at[7]).wait()


@functools.partial(jax.jit, static_argnames=("B_seg_len",))
def pallas_interleave_layers__linear_kernel_hedgehog__memory_aug_recurrent_mem_tr__prompt_kernel(
    A_x: jax.Array,
    A_wqkv: jax.Array,
    A_w_phi: jax.Array,
    A_wo: jax.Array,
    B_x: jax.Array,
    B_mem0: jax.Array,
    B_Wq: jax.Array,
    B_Wk: jax.Array,
    B_Wv: jax.Array,
    B_Wo: jax.Array,
    B_seg_len: int,
):
    del B_x
    assert B_seg_len == SEG
    assert A_x.shape == (1, S, D) and B_mem0.shape == (1, MEM, D)
    assert B_Wq.shape == (D, HB, DHB) and A_w_phi.shape == (HA, FA, FA)
    tr = lambda w: jnp.transpose(w, (1, 2, 0)).reshape(HB * DHB, D)
    hbm = pl.BlockSpec(memory_space=pl.ANY)
    out = pl.pallas_call(
        _kernel,
        out_shape=jax.ShapeDtypeStruct((S, D), bf16),
        in_specs=[hbm] * 9,
        out_specs=hbm,
        scratch_shapes=[
            pltpu.VMEM((S, D), bf16),
            pltpu.VMEM((3, D, D), bf16),
            pltpu.VMEM((FA, FA, HA), bf16),
            pltpu.VMEM((D, D), bf16),
            pltpu.VMEM((MEM, D), bf16),
            pltpu.VMEM((S, D), bf16),
            pltpu.VMEM((4, HB * DHB, D), bf16),
            pltpu.VMEM((NP, D // 2, 3 * PW), u32),
            pltpu.VMEM((NP, PW // 2, D), u32),
            pltpu.VMEM((S, D), f32),
            pltpu.VMEM((S // 2, D), u32),
            pltpu.VMEM((128, D), f32),
            pltpu.VMEM((D // 2, D), u32),
            pltpu.VMEM((D // 2, D), u32),
            pltpu.VMEM((D // 2, D), u32),
            pltpu.VMEM((NG, 48, 2 * GR), f32),
            pltpu.VMEM((NG, 24, 2 * GR), u32),
            pltpu.VMEM((S // TB, TB // 2, D), u32),
            pltpu.VMEM((MEM, D), f32),
            pltpu.VMEM((NP, 8, 3 * PW), f32),
            pltpu.VMEM((NP, 32, 3 * PW), f32),
            pltpu.VMEM((NP, 8, PW), f32),
            pltpu.VMEM((8, 128), jnp.int32),
            pltpu.SMEM((1,), jnp.int32),
            pltpu.SemaphoreType.DMA((12 + 3 * NCH,)),
        ],
        compiler_params=pltpu.CompilerParams(vmem_limit_bytes=120 * 1024 * 1024),
        name="hedgehog_rmt",
    )(A_x.reshape(S, D), A_wqkv, jnp.transpose(A_w_phi, (1, 2, 0)), A_wo, B_mem0.reshape(MEM, D),
      tr(B_Wq), tr(B_Wk), tr(B_Wv), B_Wo.reshape(HB * DHB, D))
    return out.reshape(1, S, D)
```

```python
import contextlib
import functools

import jax
import jax.numpy as jnp
from jax import lax
import jax.experimental.pallas as pl
import jax.experimental.pallas.tpu as pltpu

f32, bf16, u32 = jnp.float32, jnp.bfloat16, jnp.uint32

S, D = 2048, 640
HA, FA = 32, 20
HB, DHB = 32, 192
MEM, SEG = 8, 32
L = MEM + SEG
NP = HB // 2
PW = 2 * DHB
TB = 128
NG = 16
GR = 2 * FA
PR_ROWS = NG * (GR - 2)
NCH = 4
NT = (((1,), (1,)), ((), ()))
LOG2E = 1.4426950408889634

FLIP = {0: 2, 2: 2, 3: 2, 6: 1, 8: 1, 13: 2, 14: 2, 15: 2}
ORD_A, ORD_B = "QSPO", "QOPS"
TAIL_A, TAIL_B, TAIL_C, TAIL_W = "OOOSPOOOPOO", "OOSPOOPO", "OOSPOOPO", "SOOOOPOOOPOOOOOO"
PORD_A, PORD_B = (1, 2, 0), (0, 1, 2)
OLAG_A, OLAG_B = 4, 4
MERGE_A = 2
LATE, LATE_AT = 2, 3
ANCHOR_A, ANCHOR_B = 0, 1
LN_AT, LN_AT2 = 0, 3
KB = 3
KSPLIT = 7


_scope = lambda name: contextlib.nullcontext()


def _dot(a, b):
    return jnp.dot(a, b, preferred_element_type=f32)


def _dot_nt(a, b):
    return lax.dot_general(a, b, NT, preferred_element_type=f32)


def _pack(x):
    return pltpu.bitcast(x.astype(bf16), u32)


def _unpack(x):
    return pltpu.bitcast(x, bf16)


def _recip(x):
    r = pl.reciprocal(x, approx=True)
    return r * (2.0 - x * r)


def _layernorm(x):
    m = jnp.mean(x, axis=-1, keepdims=True)
    xc = x - m
    v = jnp.mean(xc * xc, axis=-1, keepdims=True)
    return xc * lax.rsqrt(v + 1e-5)


def _iota(shape, dim):
    return lax.broadcasted_iota(jnp.int32, shape, dim)


def _kernel(x_hbm, wqkv_hbm, wphi_hbm, woa_hbm, mem0_hbm, wqt_hbm, wkt_hbm, wvt_hbm, wob_hbm,
            out_hbm,
            x_ref, wqkv_ref, wphi_ref, woa_ref, mem0_ref, out_ref,
            stage_ref, wb_ref, wob_ref, xres_ref, xna_ref, xnb_ref,
            wpqt_ref, wpkt_ref, wvt_ref, acc_ref, kvt_ref, o_ref,
            mem_ref, svq_ref, pre_ref, svo_ref, flag_ref, cnt_ref, sems):
    WC = HB * DHB // NCH
    X_CUTS = (0, TB, 2 * TB, (2 + KB) * TB, S)

    def cp_wqkv(m):
        return pltpu.make_async_copy(wqkv_hbm.at[:, pl.ds(m * D, D)], wqkv_ref.at[m], sems.at[m])

    def cp_x(n):
        rows = pl.ds(X_CUTS[n], X_CUTS[n + 1] - X_CUTS[n])
        return pltpu.make_async_copy(x_hbm.at[rows, :], x_ref.at[rows, :], sems.at[8 + n])

    def cp_w(m, i):
        rows = pl.ds(pl.multiple_of(i * WC, WC), WC)
        return pltpu.make_async_copy((wqt_hbm, wkt_hbm, wvt_hbm)[m].at[rows, :], stage_ref.at[m, rows, :],
                                     sems.at[12 + NCH * m + i])

    cp_phi = pltpu.make_async_copy(wphi_hbm, wphi_ref, sems.at[3])
    cp_woa = pltpu.make_async_copy(woa_hbm, woa_ref, sems.at[4])
    cp_mem = pltpu.make_async_copy(mem0_hbm, mem0_ref, sems.at[5])
    cp_wob = pltpu.make_async_copy(wob_hbm, stage_ref.at[3], sems.at[6])
    cp_phi.start()
    cp_x(0).start()
    cp_wqkv(1).start()
    cp_wqkv(2).start()
    cp_x(1).start()
    cp_x(2).start()
    cp_x(3).start()
    cp_wqkv(0).start()
    cp_woa.start()
    cp_mem.start()
    for i in range(NCH):
        for m in range(3):
            cp_w(m, i).start()
    cp_wob.start()

    def phi_blocks():
        wphi = wphi_ref[...].astype(f32)
        cat = jnp.concatenate([wphi[d] for d in range(FA)], axis=1)
        cat = jnp.concatenate([cat, jnp.zeros((32 - FA, D), f32)], axis=0).astype(bf16)
        p_row, p_col = _iota((D, D), 0), _iota((D, D), 1)
        spread = (FA * (p_row & 31) + (p_row >> 5) == p_col).astype(f32).astype(bf16)
        u = _dot(cat, spread).astype(bf16)
        dup = ((_iota((48, 32), 0) >> 1) == _iota((48, 32), 1)).astype(f32).astype(bf16)
        u2 = _dot(dup, u)[:GR]
        lane, par = _iota((GR, 128), 1), _iota((GR, 128), 0) & 1
        lhs = []
        for c in range(5):
            blocks = []
            for g in range(3 * c, 3 * c + 4):
                lo = GR * g - 128 * c + FA * par
                blocks.append(jnp.where((lane >= lo) & (lane < lo + FA), u2[:, 128 * c:128 * c + 128], 0.0))
            lhs.append(jnp.concatenate(blocks, axis=0).astype(bf16))
        return lhs

    def fold_phi(lhs, m, dst):
        parts = [_dot_nt(lhs[c], wqkv_ref[m, :, 128 * c:128 * c + 128]) for c in range(5)]
        rows = []
        for c in range(5):
            first = parts[c][:GR] if c == 0 else parts[c][:GR] + parts[c - 1][3 * GR:]
            rows += [first, parts[c][GR:3 * GR]]
        rows.append(parts[4][3 * GR:])
        w = jnp.concatenate(rows, axis=0).reshape(NG, 5, 8, D)
        sub = _iota((NG, 8, D), 1)
        ref = jnp.where(sub >= 6, w[:, 4], 0.0)
        ref = ref + pltpu.roll(ref, 2, 1)
        w = (w - (ref + pltpu.roll(ref, 4, 1))[:, None]).reshape(4, 20, 8, D)
        sub = _iota((4, 8, D), 1)
        tails = [jnp.where(sub < 6, w[:, 5 * n + 4], pltpu.roll(w[:, 19], 6 - 2 * n, 1))[:, None] for n in range(3)]
        w = jnp.concatenate([w[:, 0:4], tails[0], w[:, 5:9], tails[1], w[:, 10:14], tails[2], w[:, 15:19]], axis=1)
        dst[...] = _pack(w.reshape(PR_ROWS, D))

    def fold(x, red, op):
        r = red(x, axis=1)
        r = op(r, pltpu.roll(r, 2, 1))
        return op(r, pltpu.roll(r, 4, 1))

    def project_features(w_ref, xn):
        cuts = (0, 160, 304, 464, PR_ROWS)
        part = {}

        def chunk(c):
            part[c] = _dot_nt(_unpack(w_ref[cuts[c] // 2:cuts[c + 1] // 2, :]), xn)
            pt = part[c][:152] if c % 2 == 0 else jnp.concatenate([part[c - 1][152:], part[c]], axis=0)
            sub = _iota((8, TB), 0)
            t = [pt[40 * n + 32:40 * n + 40] for n in range(3)]
            last = jnp.where(sub < 2, pltpu.roll(t[0], 2, 0), jnp.where(sub < 4, pltpu.roll(t[1], 4, 0), pltpu.roll(t[2], 6, 0)))
            t = [jnp.where(sub < 6, x, 0.0) for x in t + [last]]
            pt = jnp.concatenate([x for n in range(4) for x in (pt[40 * n:40 * n + 32], t[n])], axis=0)
            f = feature_map(pt).reshape(8 * GR, TB)
            return [f[2 * GR * g:2 * GR * (g + 1)].astype(bf16) for g in range(4)]
        return chunk

    def feature_map(pt):
        p = pt.reshape(-1, 5, 8, TB)
        ep = jnp.exp(p - fold(p, jnp.max, jnp.maximum)[:, None])
        en = jnp.exp(fold(p, jnp.min, jnp.minimum)[:, None] - p)
        ep = ep * _recip(fold(ep, jnp.sum, jnp.add))[:, None]
        en = en * _recip(fold(en, jnp.sum, jnp.add))[:, None]
        return jnp.concatenate([ep, en], axis=1)

    def rows_of(b):
        if isinstance(b, int):
            return pl.ds(b * TB, TB), pl.ds(b * TB // 2, TB // 2)
        return pl.ds(pl.multiple_of(b * TB, TB), TB), pl.ds(pl.multiple_of(b * (TB // 2), TB // 2), TB // 2)

    CG = 4
    NC = NG // CG
    CR = CG * GR

    def k_blocks(blocks, load_x=None, ahead=None, init=False, mid=None):
        xn, v, phi = {}, {}, {}
        ones8 = jnp.ones((8, TB), f32)

        def LN(j):
            rows, prows = rows_of(blocks[j] if j < len(blocks) else ahead)
            if load_x is not None and j > 0:
                xn[j] = _layernorm(load_x(rows)).astype(bf16)
                xna_ref[prows, :] = pltpu.bitcast(xn[j], u32)
            else:
                xn[j] = _unpack(xna_ref[prows, :])

        def P(j):
            chunk = project_features(wpkt_ref, xn[j])
            phi[j] = [f for c in range(NC) for f in chunk(c)]

        def V(j, c):
            vt = _dot_nt(_unpack(wvt_ref[c * CR // 2:(c + 1) * CR // 2, :]), xn[j])
            for g in range(CG):
                v[j, CG * c + g] = jnp.concatenate([vt[GR * g:GR * (g + 1)], ones8], axis=0).astype(bf16)

        def KV(j):
            for g in range(NG):
                r = _dot_nt(v[j, g], phi[j][g])
                if init and j == 0:
                    acc_ref[g] = r
                else:
                    acc_ref[g] += r

        LN(0)
        for j in range(len(blocks)):
            if j + 1 < len(blocks) or ahead is not None:
                LN(j + 1)
            P(j)
            if mid is not None:
                mid()
            for c in range(NC):
                V(j, c)
            KV(j)

    def finish_kv():
        r48, odd = _iota((48, 2 * GR), 0), (_iota((48, 2 * GR), 1) & 1) == 1
        same = (((r48 >= FA) & (r48 < GR)) | (r48 >= GR + 4)) == odd
        for g in range(NG):
            kvt_ref[g] = _pack(jnp.where(same, acc_ref[g], 0.0))

    def q_blocks(blocks, load_x, hooks, between=None):
        top = _iota((NG, 8, TB), 1) < 4
        phi, ot, o, y = {}, {}, {}, {}
        n = len(blocks)

        def P(j):
            chunk = project_features(wpqt_ref, _unpack(xna_ref[rows_of(blocks[j])[1], :]))
            phi[j] = [f for c in range(NC) for f in chunk(c)]

        def N(j):
            num = jnp.concatenate([_dot(_unpack(kvt_ref[g]), phi[j][g]) for g in range(NG)], axis=0).reshape(NG, 48, TB)
            rm = 1.0 / (num[:, GR:] + 1e-6)
            rs = pltpu.roll(rm, 4, 1)
            r0, r1 = jnp.where(top, rm, rs), jnp.where(top, rs, rm)
            ot[j] = (num[:, :GR] * jnp.concatenate([r0, r0, rm, r1, r1], axis=1)).reshape(D, TB)

        def W(j, t):
            if t == 0:
                o_ref[j] = pltpu.bitcast(ot[j].astype(bf16).T, u32)
                o[j] = _unpack(o_ref[j])
            y[j, t] = _dot(o[j], woa_ref[:, 128 * t:128 * t + 128])
            if t == 4:
                rows = rows_of(blocks[j])[0]
                xres_ref[rows, :] = load_x(rows) + jnp.concatenate([y[j, t] for t in range(5)], axis=1)

        def WW(j):
            for t in range(5):
                W(j, t)
                if (j, t) in hooks:
                    hooks[j, t]()

        P(0), P(1)
        if between is not None:
            between()
        N(0), P(2), N(1), WW(0), N(2)
        for j in range(3, n):
            P(j), WW(j - 2), N(j)
        WW(n - 2), WW(n - 1)

    VPERM = [(h * DHB + 64 * c) for c in range(3) for h in range(2)]

    def relayout_weights(j):
        r0 = pl.multiple_of(j * PW, PW)
        for m in range(2):
            wb_ref[j, :, m * PW:(m + 1) * PW] = pltpu.bitcast(stage_ref[m, pl.ds(r0, PW), :].T, u32)
        for c in range(3):
            w = jnp.concatenate([stage_ref[2, pl.ds(pl.multiple_of(r0 + o, 64), 64), :] for o in VPERM[2 * c:2 * c + 2]], axis=0)
            wb_ref[j, :, 2 * PW + 128 * c:2 * PW + 128 * (c + 1)] = pltpu.bitcast(w.T, u32)

    scale = DHB ** -0.5
    NQ = 32
    row, col = _iota((2 * NQ, 2 * L), 0), _iota((2 * NQ, 2 * L), 1)
    same = (row < NQ) == (col < L)
    rr = jnp.where(row < NQ, row, row - NQ)
    kk = jnp.where(col < L, col, col - L)
    keep = same & ((rr < MEM) | (rr >= kk) | (kk >= NQ))
    fill = jnp.where(same, -1e9 / scale, -jnp.inf).astype(f32)
    lo = {sh: (_iota(sh, len(sh) - 1) & 64) == 0 for sh in ((L, 128), (L, PW), (NQ, 128), (16, 128), (8, 8, 128))}
    causal = _iota((8, 8, 128), 1) <= _iota((8, 8, 128), 0)

    def halves(x):
        m = lo[x.shape]
        return jnp.concatenate([jnp.where(m, x, 0.0), jnp.where(m, 0.0, x)], axis=0).astype(bf16)

    def outer(x):
        return jnp.concatenate([x[:, 0:128], x[:, 256:384]], axis=0).astype(bf16)

    def scores(q, k):
        s1 = _dot_nt(outer(q), outer(k))
        s2 = _dot_nt(q[:, 128:256].astype(bf16), halves(k[:, 128:256]))
        s = s1 + jnp.concatenate([s2, s2], axis=0)
        s = jnp.where(keep, s, fill)
        e = jnp.exp2((s - jnp.max(s, axis=1, keepdims=True)) * (scale * LOG2E))
        return e, jnp.sum(e, axis=1, keepdims=True)

    def values(e, l, v):
        rab = _recip(jnp.where(lo[NQ, 128], l[:NQ], l[NQ:]))
        return _dot((e[:NQ] + e[NQ:]).astype(bf16), halves(v)) * jnp.concatenate([rab] * 3, axis=1)

    def head_attention(q, k, v):
        steps = lambda x: jnp.stack([pltpu.roll(x, i + 1, 0) for i in range(7)] + [x])
        qr = steps(q * (scale * LOG2E))
        mid = k[:, 128:256]
        ka = jnp.concatenate([k[:, 0:128], jnp.where(lo[16, 128], mid, 0.0)], axis=1)
        kb = jnp.concatenate([jnp.where(lo[16, 128], 0.0, mid), k[:, 256:384]], axis=1)
        qa, qb = qr[:, :, 0:256], qr[:, :, 128:384]
        ss = []
        for b in range(2):
            sa = jnp.sum(qa * ka[8 * b:8 * b + 8][None], axis=2, keepdims=True)
            sb = jnp.sum(qb * kb[8 * b:8 * b + 8][None], axis=2, keepdims=True)
            ss.append(jnp.where(lo[8, 8, 128], sa, sb))
        ss[1] = jnp.where(causal, ss[1], -1e9 * LOG2E)

        def unrotate(x, op):
            r = x[0]
            for i in range(1, 8):
                r = op(pltpu.roll(r, 1, 0), x[i])
            return r

        m = steps(unrotate(jnp.maximum(ss[0], ss[1]), jnp.maximum))
        e0, e1 = jnp.exp2(ss[0] - m), jnp.exp2(ss[1] - m)
        t = jnp.concatenate([e0] * 3, axis=2) * v[0:8][None] + jnp.concatenate([e1] * 3, axis=2) * v[8:16][None]
        acc = unrotate(jnp.concatenate([t, e0 + e1], axis=2), jnp.add)
        return acc[:, :PW] * jnp.concatenate([_recip(acc[:, PW:])] * 3, axis=1)

    def bstep(h, first, never, early, chained_in, chained_out, pre=None):
        qkv, ps, os_, ov = {}, {}, {}, {}
        acc = {}
        nxt = [0]
        late = NP - (3 if pre is not None else LATE)

        split = pre is not None and first

        def is_long(first, t, m):
            flipped = FLIP.get(t) == m
            return (flipped and not first) if pre is not None else first != flipped

        hb = {True: h.astype(bf16), False: h[:NQ].astype(bf16)}

        def PR(t, ms):
            hs = {m: h if is_long(first, t, m) else h[:NQ] for m in ms}
            if t == 0 and chained_in:
                rs = {}
                for k in range(5):
                    for m in ms:
                        c = _dot(hs[m][:, 128 * k:128 * k + 128].astype(bf16),
                                 _unpack(wb_ref[t, 64 * k:64 * k + 64, m * PW:(m + 1) * PW]))
                        rs[m] = c if k == 0 else rs[m] + c
            else:
                rs = {m: _dot(hb[is_long(first, t, m)], _unpack(wb_ref[t, :, m * PW:(m + 1) * PW])) for m in ms}
            for m in ms:
                if is_long(first, t, m):
                    svq_ref[t, :, m * PW:(m + 1) * PW] = rs[m][L:]
                    qkv[t, m] = rs[m][:L]
                else:
                    cols = slice(m * PW, (m + 1) * PW)
                    saved = svq_ref[t, :, cols] if pre is None else pre_ref[t, pl.ds(pl.multiple_of(pre * 8, 8), 8), cols]
                    qkv[t, m] = jnp.concatenate([rs[m], saved], axis=0)
            if not (split and t >= NP - 2):
                HA_(t)

        def HA_(t):
            k, v = [jnp.concatenate([qkv[t, m][:MEM], qkv[t, m][NQ:]], axis=0) for m in (1, 2)]
            ov[t] = head_attention(qkv[t, 0][NQ:], k, v)

        def SS(j):
            ps[j] = scores(qkv[j, 0][:NQ], qkv[j, 1])

        def PV(j):
            e, l = ps[j]
            ja = j - (1 if split else ANCHOR_A if first else ANCHOR_B)
            if ja >= 0 and not (first and ja >= late):
                e = jnp.concatenate([jnp.where(never, ov[ja][:, 128 * c:128 * c + 2 * L], e[8 * c:8 * c + 8])
                                     for c in range(3)] + [e[24:]], axis=0)
            if j in early:
                e = jnp.concatenate([e[:24], jnp.where(never, early[j][:, :2 * L], e[24:32]), e[32:]], axis=0)
            o = values(e, l, qkv[j, 2])
            if first and j >= late:
                svo_ref[j] = ov[j]
            elif first:
                svo_ref[j] = o[24:32]
                o = jnp.concatenate([o[:24], ov[j]], axis=0)
            else:
                o = jnp.concatenate([o, ov[j], svo_ref[j]], axis=0)
            os_[j] = o

        def OO(merge=1):
            js = range(nxt[0], nxt[0] + merge)
            ws = []
            for j in js:
                if pre is not None:
                    ws.append(jnp.concatenate(
                        [pltpu.bitcast(stage_ref[3, j * PW + o:j * PW + o + 64, :], u32) for o in VPERM], axis=0))
                    if not first:
                        wob_ref[j] = ws[-1]
                else:
                    ws.append(wob_ref[j])
            c = _dot(jnp.concatenate([os_[j] for j in js], axis=1).astype(bf16), _unpack(jnp.concatenate(ws, axis=0)))
            for key, part in ((0, c[:-8]), (1 + (js[0] >= late), c[-8:])):
                acc[key] = acc[key] + part if key in acc else part
            nxt[0] += merge

        order, tail = (ORD_A, TAIL_W if split else TAIL_A) if first else (ORD_B, TAIL_C if chained_out else TAIL_B)
        olag = OLAG_A if first else OLAG_B
        nl = (3 if split else MERGE_A) if first else 1
        nd = tail.count("O") + nl
        for t in range(NP):
            for op in order:
                if op == "Q":
                    PR(t, PORD_A if first else PORD_B)
                    if split and t == NP - 1:
                        pl.when(pre == 0)(lambda: cp_wob.wait())
                        HA_(NP - 2), HA_(NP - 1)
                if op == "S" and t >= 1:
                    SS(t - 1)
                if op == "P" and t >= 2:
                    PV(t - 2)
                if op == "O" and olag <= t < NP - 1 and nxt[0] < NP - nd:
                    OO()
        p = NP - 2
        for op in tail:
            if op == "O":
                OO()
            if op == "S":
                SS(NP - 1)
            if op == "P":
                PV(p)
                p += 1
        OO(nl)
        assert nxt[0] == NP and p == NP
        hand = {LATE_AT + n: jnp.maximum(jnp.maximum(ov[j][:, 0:128], ov[j][:, 128:256]), ov[j][:, 256:384])
                for n, j in enumerate(range(late, NP))} if first else None
        return acc[0], acc[1], acc[2], hand

    def bpass(last, lo_it, hi_it, warm=False):
        def body(i, c):
            never = flag_ref[:, :2 * L] > 0
            probe = lambda x, g: x[8 * g:8 * g + 8, 0:128]
            mem = mem_ref[...]
            if warm:
                slots = [pl.ds(pl.multiple_of(i * 64, 64), 64)]
                heads = [xnb_ref[pl.ds(pl.multiple_of((1 - i) * 64, 64), 8), :]]
            else:
                slots = [pl.ds(0, 64), pl.ds(64, 64)]
            xs = [xnb_ref[sl, :] for sl in slots]
            n = len(slots)
            for u in range(n):
                r0 = pl.multiple_of((i * n + u) * 64, 64)
                xa = xs[u]
                rn = pl.multiple_of(jnp.minimum(r0 + 128, S - 64), 64)
                xn = _layernorm(xres_ref[pl.ds(rn, 64), :])
                xnb_ref[slots[u], :] = xn
                if not warm and u == 0:
                    heads = [xs[1][0:8], xn[0:8]]
                early = {LN_AT + g: probe(xn, g) for g in range(8)}
                if not last:
                    rp = pl.multiple_of(jnp.maximum(r0 - 64, 0), 64)
                    xn = _layernorm(xres_ref[pl.ds(rp, 64), :])
                    xna_ref[pl.ds(pl.multiple_of(rp // 2, 32), 32), :] = _pack(xn)
                    for g in range(8):
                        j = LN_AT2 + g
                        early[j] = jnp.maximum(early[j], probe(xn, g)) if j in early else probe(xn, g)
                ya, a0, a24, hand = bstep(jnp.concatenate([mem, xa[8:32], xa[0:8], xa[32:40]], axis=0), True, never, early,
                           u > 0, True, 2 * i if warm else None)
                yb, b24, b0, _ = bstep(jnp.concatenate([ya[:MEM], xa[40:64], xa[32:40], heads[u]], axis=0), False, never, hand,
                           True, u < n - 1, 2 * i + 1 if warm else None)
                mem = yb[:MEM]
                y = xres_ref[pl.ds(r0, 64), :] + jnp.concatenate([a0 + b0, ya[MEM:24], a24 + b24, yb[32:40], yb[MEM:32]], axis=0)
                if last:
                    out_ref[pl.ds(r0, 64), :] = y.astype(bf16)
                else:
                    xres_ref[pl.ds(r0, 64), :] = y
            mem_ref[...] = mem
            if last:
                rows = pl.ds(pl.multiple_of(i * 128, 128), 128)
                pltpu.make_async_copy(out_ref.at[rows, :], out_hbm.at[rows, :], sems.at[7]).start()
            return c
        lax.fori_loop(lo_it, hi_it, body, 0)

    load_in = lambda rows: x_ref[rows, :].astype(f32)
    load_res = lambda rows: xres_ref[rows, :]
    NB = S // (TB * NCH)

    def k1_body(i, c):
        pl.when(i == 1)(lambda: cp_x(3).wait())
        k_blocks([1 + i * KB + j for j in range(KB)], load_in, jnp.minimum(1 + i * KB + KB, S // TB - 1))
        return c

    def q1_body(i, c):
        for m in range(3):
            cp_w(m, i).wait()
        pairs = [i * (NP // NCH) + j for j in range(NP // NCH)]
        for j in pairs:
            relayout_weights(j)
        head = []

        def norm_first():
            x0 = _layernorm(xres_ref[0:128, :])
            xnb_ref[...] = x0
            head.append(jnp.concatenate([x0[32 * sg:32 * sg + 8] for sg in range(4)], axis=0).astype(bf16))

        def project(js):
            for j in js:
                pre_ref[j] = _dot(head[0], _unpack(wb_ref[j]))

        q_blocks([i * NB + j for j in range(NB)], load_in,
                 {(0, 4): norm_first, (1, 4): lambda: project(pairs[:1]), (2, 4): lambda: project(pairs[1:3]),
                  (3, 4): lambda: project(pairs[3:])})
        return c

    with _scope("pro"):
        flag_ref[...] = jnp.zeros(flag_ref.shape, jnp.int32)
        cnt_ref[0] = 0
        cp_phi.wait()
        cp_x(0).wait()
        phi_lhs = phi_blocks()
        xna_ref[0:TB // 2, :] = _pack(_layernorm(load_in(pl.ds(0, TB))))
        cp_wqkv(1).wait()
        fold_phi(phi_lhs, 1, wpkt_ref)

        def values_ready():
            cp_wqkv(2).wait()
            cp_x(1).wait()
            wvt_ref[...] = pltpu.bitcast(wqkv_ref[2].T, u32)
            xna_ref[TB // 2:TB, :] = _pack(_layernorm(load_in(pl.ds(TB, TB))))

        k_blocks([0], init=True, mid=values_ready)
        cp_x(2).wait()
    with _scope("k1"):
        lax.fori_loop(0, (S // TB - 1) // KB, k1_body, 0)
    with _scope("f1"):
        cp_wqkv(0).wait()
        cp_woa.wait()
        cp_mem.wait()
        fold_phi(phi_lhs, 0, wpqt_ref)
        finish_kv()
        mem_ref[...] = mem0_ref[...].astype(f32)
    with _scope("q1"):
        lax.fori_loop(0, NCH, q1_body, 0)
    with _scope("b1w"):
        bpass(False, 0, 2, warm=True)
    with _scope("b1"):
        bpass(False, 1, S // 128)
    with _scope("a2"):
        lax.fori_loop(0, cnt_ref[0] + 1, lambda i, c: (k_blocks(list(range(KSPLIT)), init=True), c)[1], 0)
        xna_ref[(S - 64) // 2:, :] = _pack(_layernorm(xres_ref[S - 64:, :]))
        k_blocks(list(range(KSPLIT, S // TB)))
        head = []

        def norm_first():
            x0 = _layernorm(xres_ref[0:128, :])
            xnb_ref[...] = x0
            head.append(x0[0:16].astype(bf16))

        def save_rows(t, c):
            svq_ref[t, :, c:c + 128] = _dot(head[0], _unpack(wb_ref[t, :, c:c + 128]))[:8]

        hooks = {(0, 4): norm_first}
        pieces = [(t, m * PW + 128 * c) for t, m in FLIP.items() for c in range(3)]
        for n, piece in enumerate(pieces):
            hooks[2 + n // 2, 1 + 2 * (n % 2)] = functools.partial(save_rows, *piece)
        q_blocks(list(range(S // TB)), load_res, hooks, between=finish_kv)
        mem_ref[...] = mem0_ref[...].astype(f32)
    with _scope("b2"):
        bpass(True, 0, S // 128)
    pltpu.make_async_copy(out_ref, out_hbm, sems.at[7]).wait()


@functools.partial(jax.jit, static_argnames=("B_seg_len",))
def pallas_interleave_layers__linear_kernel_hedgehog__memory_aug_recurrent_mem_tr__prompt_kernel(
    A_x: jax.Array,
    A_wqkv: jax.Array,
    A_w_phi: jax.Array,
    A_wo: jax.Array,
    B_x: jax.Array,
    B_mem0: jax.Array,
    B_Wq: jax.Array,
    B_Wk: jax.Array,
    B_Wv: jax.Array,
    B_Wo: jax.Array,
    B_seg_len: int,
):
    del B_x
    assert B_seg_len == SEG
    assert A_x.shape == (1, S, D) and B_mem0.shape == (1, MEM, D)
    assert B_Wq.shape == (D, HB, DHB) and A_w_phi.shape == (HA, FA, FA)
    tr = lambda w: jnp.transpose(w, (1, 2, 0)).reshape(HB * DHB, D)
    hbm = pl.BlockSpec(memory_space=pl.ANY)
    out = pl.pallas_call(
        _kernel,
        out_shape=jax.ShapeDtypeStruct((S, D), bf16),
        in_specs=[hbm] * 9,
        out_specs=hbm,
        scratch_shapes=[
            pltpu.VMEM((S, D), bf16),
            pltpu.VMEM((3, D, D), bf16),
            pltpu.VMEM((FA, FA, HA), bf16),
            pltpu.VMEM((D, D), bf16),
            pltpu.VMEM((MEM, D), bf16),
            pltpu.VMEM((S, D), bf16),
            pltpu.VMEM((4, HB * DHB, D), bf16),
            pltpu.VMEM((NP, D // 2, 3 * PW), u32),
            pltpu.VMEM((NP, PW // 2, D), u32),
            pltpu.VMEM((S, D), f32),
            pltpu.VMEM((S // 2, D), u32),
            pltpu.VMEM((128, D), f32),
            pltpu.VMEM((PR_ROWS // 2, D), u32),
            pltpu.VMEM((PR_ROWS // 2, D), u32),
            pltpu.VMEM((D // 2, D), u32),
            pltpu.VMEM((NG, 48, 2 * GR), f32),
            pltpu.VMEM((NG, 24, 2 * GR), u32),
            pltpu.VMEM((S // TB, TB // 2, D), u32),
            pltpu.VMEM((MEM, D), f32),
            pltpu.VMEM((NP, 8, 3 * PW), f32),
            pltpu.VMEM((NP, 32, 3 * PW), f32),
            pltpu.VMEM((NP, 8, PW), f32),
            pltpu.VMEM((8, 128), jnp.int32),
            pltpu.SMEM((1,), jnp.int32),
            pltpu.SemaphoreType.DMA((12 + 3 * NCH,)),
        ],
        compiler_params=pltpu.CompilerParams(vmem_limit_bytes=120 * 1024 * 1024),
        name="hedgehog_rmt",
    )(A_x.reshape(S, D), A_wqkv, jnp.transpose(A_w_phi, (1, 2, 0)), A_wo, B_mem0.reshape(MEM, D),
      tr(B_Wq), tr(B_Wk), tr(B_Wv), B_Wo.reshape(HB * DHB, D))
    return out.reshape(1, S, D)
```

```python
import contextlib
import functools

import jax
import jax.numpy as jnp
from jax import lax
import jax.experimental.pallas as pl
import jax.experimental.pallas.tpu as pltpu

f32, bf16, u32 = jnp.float32, jnp.bfloat16, jnp.uint32

S, D = 2048, 640
HA, FA = 32, 20
HB, DHB = 32, 192
MEM, SEG = 8, 32
L = MEM + SEG
NP = HB // 2
PW = 2 * DHB
TB = 128
NG = 16
GR = 2 * FA
PR_ROWS = NG * (GR - 2)
NCH = 4
NT = (((1,), (1,)), ((), ()))
LOG2E = 1.4426950408889634

FLIP = {0: 2, 2: 2, 3: 2, 6: 1, 8: 1, 13: 2, 14: 2, 15: 2}
ORD_A, ORD_B = "QSPO", "QOPS"
TAIL_A, TAIL_B, TAIL_C, TAIL_W = "OOOSPOOOPOO", "OOSPOOPO", "OOSPOOPO", "OSOOPOOPOOOOOOOO"
PORD_A, PORD_B = (1, 2, 0), (0, 1, 2)
OLAG_A, OLAG_B = 4, 4
MERGE_A = 2
LATE, LATE_AT = 2, 3
ANCHOR_A, ANCHOR_B = 0, 1
LN_AT, LN_AT2 = 0, 3
KB = 3
KSPLIT = 7


_scope = lambda name: contextlib.nullcontext()


def _dot(a, b):
    return jnp.dot(a, b, preferred_element_type=f32)


def _dot_nt(a, b):
    return lax.dot_general(a, b, NT, preferred_element_type=f32)


def _pack(x):
    return pltpu.bitcast(x.astype(bf16), u32)


def _unpack(x):
    return pltpu.bitcast(x, bf16)


def _recip(x):
    r = pl.reciprocal(x, approx=True)
    return r * (2.0 - x * r)


def _layernorm(x):
    m = jnp.mean(x, axis=-1, keepdims=True)
    xc = x - m
    v = jnp.mean(xc * xc, axis=-1, keepdims=True)
    return xc * lax.rsqrt(v + 1e-5)


def _iota(shape, dim):
    return lax.broadcasted_iota(jnp.int32, shape, dim)


def _kernel(x_hbm, wqkv_hbm, wphi_hbm, woa_hbm, mem0_hbm, wqt_hbm, wkt_hbm, wvt_hbm, wob_hbm,
            out_hbm,
            x_ref, wqkv_ref, wphi_ref, woa_ref, mem0_ref, out_ref,
            stage_ref, wb_ref, wob_ref, xres_ref, xna_ref, xnb_ref,
            wpqt_ref, wpkt_ref, wvt_ref, acc_ref, kvt_ref, o_ref,
            mem_ref, svq_ref, pre_ref, svo_ref, flag_ref, cnt_ref, sems):
    WC = HB * DHB // NCH // 2
    X_CUTS = (0, TB, 2 * TB, (2 + KB) * TB, S)

    def cp_wqkv(m):
        return pltpu.make_async_copy(wqkv_hbm.bitcast(u32).at[:, pl.ds(m * D, D)], wqkv_ref.at[m], sems.at[m])

    def cp_x(n):
        rows = pl.ds(X_CUTS[n], X_CUTS[n + 1] - X_CUTS[n])
        return pltpu.make_async_copy(x_hbm.at[rows, :], x_ref.at[rows, :], sems.at[8 + n])

    def cp_w(m, i):
        rows = pl.ds(pl.multiple_of(i * WC, WC), WC)
        return pltpu.make_async_copy((wqt_hbm, wkt_hbm, wvt_hbm)[m].bitcast(u32).at[rows, :], stage_ref.at[m, rows, :],
                                     sems.at[12 + NCH * m + i])

    cp_phi = pltpu.make_async_copy(wphi_hbm, wphi_ref, sems.at[3])
    cp_woa = pltpu.make_async_copy(woa_hbm.bitcast(u32), woa_ref, sems.at[4])
    cp_mem = pltpu.make_async_copy(mem0_hbm, mem0_ref, sems.at[5])
    cp_wob = pltpu.make_async_copy(wob_hbm.bitcast(u32), wob_ref, sems.at[6])
    cp_phi.start()
    cp_x(0).start()
    cp_wqkv(1).start()
    cp_wqkv(2).start()
    cp_x(1).start()
    cp_x(2).start()
    cp_x(3).start()
    cp_wqkv(0).start()
    cp_woa.start()
    cp_mem.start()
    for i in range(NCH):
        for m in range(3):
            cp_w(m, i).start()
    cp_wob.start()

    def phi_blocks():
        wphi = wphi_ref[...].astype(f32)
        cat = jnp.concatenate([wphi[d] for d in range(FA)], axis=1)
        cat = jnp.concatenate([cat, jnp.zeros((32 - FA, D), f32)], axis=0).astype(bf16)
        p_row, p_col = _iota((D, D), 0), _iota((D, D), 1)
        spread = (FA * (p_row & 31) + (p_row >> 5) == p_col).astype(f32).astype(bf16)
        u = _dot(cat, spread).astype(bf16)
        dup = ((_iota((48, 32), 0) >> 1) == _iota((48, 32), 1)).astype(f32).astype(bf16)
        u2 = _dot(dup, u)[:GR]
        lane, par = _iota((GR, 128), 1), _iota((GR, 128), 0) & 1
        lhs = []
        for c in range(5):
            blocks = []
            for g in range(3 * c, 3 * c + 4):
                lo = GR * g - 128 * c + FA * par
                blocks.append(jnp.where((lane >= lo) & (lane < lo + FA), u2[:, 128 * c:128 * c + 128], 0.0))
            lhs.append(jnp.concatenate(blocks, axis=0).astype(bf16))
        return lhs

    def fold_phi(lhs, m, dst):
        parts = [_dot_nt(lhs[c], _unpack(wqkv_ref[m, :, 128 * c:128 * c + 128])) for c in range(5)]
        rows = []
        for c in range(5):
            first = parts[c][:GR] if c == 0 else parts[c][:GR] + parts[c - 1][3 * GR:]
            rows += [first, parts[c][GR:3 * GR]]
        rows.append(parts[4][3 * GR:])
        w = jnp.concatenate(rows, axis=0).reshape(NG, 5, 8, D)
        sub = _iota((NG, 8, D), 1)
        ref = jnp.where(sub >= 6, w[:, 4], 0.0)
        ref = ref + pltpu.roll(ref, 2, 1)
        w = (w - (ref + pltpu.roll(ref, 4, 1))[:, None]).reshape(4, 20, 8, D)
        sub = _iota((4, 8, D), 1)
        tails = [jnp.where(sub < 6, w[:, 5 * n + 4], pltpu.roll(w[:, 19], 6 - 2 * n, 1))[:, None] for n in range(3)]
        w = jnp.concatenate([w[:, 0:4], tails[0], w[:, 5:9], tails[1], w[:, 10:14], tails[2], w[:, 15:19]], axis=1)
        dst[...] = _pack(w.reshape(PR_ROWS, D))

    def fold(x, red, op):
        r = red(x, axis=1)
        r = op(r, pltpu.roll(r, 2, 1))
        return op(r, pltpu.roll(r, 4, 1))

    def project_features(w_ref, xn):
        cuts = (0, 160, 304, 464, PR_ROWS)
        part = {}

        def chunk(c):
            part[c] = _dot_nt(_unpack(w_ref[cuts[c] // 2:cuts[c + 1] // 2, :]), xn)
            pt = part[c][:152] if c % 2 == 0 else jnp.concatenate([part[c - 1][152:], part[c]], axis=0)
            sub = _iota((8, TB), 0)
            t = [pt[40 * n + 32:40 * n + 40] for n in range(3)]
            last = jnp.where(sub < 2, pltpu.roll(t[0], 2, 0), jnp.where(sub < 4, pltpu.roll(t[1], 4, 0), pltpu.roll(t[2], 6, 0)))
            t = [jnp.where(sub < 6, x, 0.0) for x in t + [last]]
            pt = jnp.concatenate([x for n in range(4) for x in (pt[40 * n:40 * n + 32], t[n])], axis=0)
            f = feature_map(pt).reshape(8 * GR, TB)
            return [f[2 * GR * g:2 * GR * (g + 1)].astype(bf16) for g in range(4)]
        return chunk

    def feature_map(pt):
        p = pt.reshape(-1, 5, 8, TB)
        ep = jnp.exp(p - fold(p, jnp.max, jnp.maximum)[:, None])
        en = jnp.exp(fold(p, jnp.min, jnp.minimum)[:, None] - p)
        ep = ep * _recip(fold(ep, jnp.sum, jnp.add))[:, None]
        en = en * _recip(fold(en, jnp.sum, jnp.add))[:, None]
        return jnp.concatenate([ep, en], axis=1)

    def rows_of(b):
        if isinstance(b, int):
            return pl.ds(b * TB, TB), pl.ds(b * TB // 2, TB // 2)
        return pl.ds(pl.multiple_of(b * TB, TB), TB), pl.ds(pl.multiple_of(b * (TB // 2), TB // 2), TB // 2)

    CG = 4
    NC = NG // CG
    CR = CG * GR

    def k_blocks(blocks, load_x=None, ahead=None, init=False, mid=None):
        xn, v, phi = {}, {}, {}
        ones8 = jnp.ones((8, TB), f32)

        def LN(j):
            rows, prows = rows_of(blocks[j] if j < len(blocks) else ahead)
            if load_x is not None and j > 0:
                xn[j] = _layernorm(load_x(rows)).astype(bf16)
                xna_ref[prows, :] = pltpu.bitcast(xn[j], u32)
            else:
                xn[j] = _unpack(xna_ref[prows, :])

        def P(j):
            chunk = project_features(wpkt_ref, xn[j])
            phi[j] = [f for c in range(NC) for f in chunk(c)]

        def V(j, c):
            vt = _dot_nt(_unpack(wvt_ref[c * CR // 2:(c + 1) * CR // 2, :]), xn[j])
            for g in range(CG):
                v[j, CG * c + g] = jnp.concatenate([vt[GR * g:GR * (g + 1)], ones8], axis=0).astype(bf16)

        def KV(j):
            for g in range(NG):
                r = _dot_nt(v[j, g], phi[j][g])
                if init and j == 0:
                    acc_ref[g] = r
                else:
                    acc_ref[g] += r

        LN(0)
        for j in range(len(blocks)):
            if j + 1 < len(blocks) or ahead is not None:
                LN(j + 1)
            P(j)
            if mid is not None:
                mid()
            for c in range(NC):
                V(j, c)
            KV(j)

    def finish_kv():
        r48, odd = _iota((48, 2 * GR), 0), (_iota((48, 2 * GR), 1) & 1) == 1
        same = (((r48 >= FA) & (r48 < GR)) | (r48 >= GR + 4)) == odd
        for g in range(NG):
            kvt_ref[g] = _pack(jnp.where(same, acc_ref[g], 0.0))

    def q_blocks(blocks, load_x, hooks, between=None):
        top = _iota((NG, 8, TB), 1) < 4
        phi, ot, o, y = {}, {}, {}, {}
        n = len(blocks)

        def P(j):
            chunk = project_features(wpqt_ref, _unpack(xna_ref[rows_of(blocks[j])[1], :]))
            phi[j] = [f for c in range(NC) for f in chunk(c)]

        def N(j):
            num = jnp.concatenate([_dot(_unpack(kvt_ref[g]), phi[j][g]) for g in range(NG)], axis=0).reshape(NG, 48, TB)
            rm = 1.0 / (num[:, GR:] + 1e-6)
            rs = pltpu.roll(rm, 4, 1)
            r0, r1 = jnp.where(top, rm, rs), jnp.where(top, rs, rm)
            ot[j] = (num[:, :GR] * jnp.concatenate([r0, r0, rm, r1, r1], axis=1)).reshape(D, TB)

        def W(j, t):
            if t == 0:
                o_ref[j] = pltpu.bitcast(ot[j].astype(bf16).T, u32)
                o[j] = _unpack(o_ref[j])
            y[j, t] = _dot(o[j], _unpack(woa_ref[:, 128 * t:128 * t + 128]))
            if t == 4:
                rows = rows_of(blocks[j])[0]
                xres_ref[rows, :] = load_x(rows) + jnp.concatenate([y[j, t] for t in range(5)], axis=1)

        def WW(j):
            for t in range(5):
                W(j, t)
                if (j, t) in hooks:
                    hooks[j, t]()

        P(0), P(1)
        if between is not None:
            between()
        N(0), P(2), N(1), WW(0), N(2)
        for j in range(3, n):
            P(j), WW(j - 2), N(j)
        WW(n - 2), WW(n - 1)

    VPERM = [(h * DHB + 64 * c) // 2 for c in range(3) for h in range(2)]

    def relayout_weights(j):
        r0 = pl.multiple_of(j * DHB, DHB)
        for m in range(2):
            wb_ref[j, :, m * PW:(m + 1) * PW] = pltpu.bitcast(_unpack(stage_ref[m, pl.ds(r0, DHB), :]).T, u32)
        for c in range(3):
            w = jnp.concatenate([stage_ref[2, pl.ds(pl.multiple_of(r0 + o, 32), 32), :] for o in VPERM[2 * c:2 * c + 2]], axis=0)
            wb_ref[j, :, 2 * PW + 128 * c:2 * PW + 128 * (c + 1)] = pltpu.bitcast(_unpack(w).T, u32)

    scale = DHB ** -0.5
    NQ = 32
    row, col = _iota((2 * NQ, 2 * L), 0), _iota((2 * NQ, 2 * L), 1)
    same = (row < NQ) == (col < L)
    rr = jnp.where(row < NQ, row, row - NQ)
    kk = jnp.where(col < L, col, col - L)
    keep = same & ((rr < MEM) | (rr >= kk) | (kk >= NQ))
    fill = jnp.where(same, -1e9 / scale, -jnp.inf).astype(f32)
    lo = {sh: (_iota(sh, len(sh) - 1) & 64) == 0 for sh in ((L, 128), (L, PW), (NQ, 128), (16, 128), (8, 8, 128))}
    causal = _iota((8, 8, 128), 1) <= _iota((8, 8, 128), 0)

    def halves(x):
        m = lo[x.shape]
        return jnp.concatenate([jnp.where(m, x, 0.0), jnp.where(m, 0.0, x)], axis=0).astype(bf16)

    def outer(x):
        return jnp.concatenate([x[:, 0:128], x[:, 256:384]], axis=0).astype(bf16)

    def scores(q, k):
        s1 = _dot_nt(outer(q), outer(k))
        s2 = _dot_nt(q[:, 128:256].astype(bf16), halves(k[:, 128:256]))
        s = s1 + jnp.concatenate([s2, s2], axis=0)
        s = jnp.where(keep, s, fill)
        e = jnp.exp2((s - jnp.max(s, axis=1, keepdims=True)) * (scale * LOG2E))
        return e, jnp.sum(e, axis=1, keepdims=True)

    def values(e, l, v):
        rab = _recip(jnp.where(lo[NQ, 128], l[:NQ], l[NQ:]))
        return _dot((e[:NQ] + e[NQ:]).astype(bf16), halves(v)) * jnp.concatenate([rab] * 3, axis=1)

    def head_attention(q, k, v):
        steps = lambda x: jnp.stack([pltpu.roll(x, i + 1, 0) for i in range(7)] + [x])
        qr = steps(q * (scale * LOG2E))
        mid = k[:, 128:256]
        ka = jnp.concatenate([k[:, 0:128], jnp.where(lo[16, 128], mid, 0.0)], axis=1)
        kb = jnp.concatenate([jnp.where(lo[16, 128], 0.0, mid), k[:, 256:384]], axis=1)
        qa, qb = qr[:, :, 0:256], qr[:, :, 128:384]
        ss = []
        for b in range(2):
            sa = jnp.sum(qa * ka[8 * b:8 * b + 8][None], axis=2, keepdims=True)
            sb = jnp.sum(qb * kb[8 * b:8 * b + 8][None], axis=2, keepdims=True)
            ss.append(jnp.where(lo[8, 8, 128], sa, sb))
        ss[1] = jnp.where(causal, ss[1], -1e9 * LOG2E)

        def unrotate(x, op):
            r = x[0]
            for i in range(1, 8):
                r = op(pltpu.roll(r, 1, 0), x[i])
            return r

        m = steps(unrotate(jnp.maximum(ss[0], ss[1]), jnp.maximum))
        e0, e1 = jnp.exp2(ss[0] - m), jnp.exp2(ss[1] - m)
        t = jnp.concatenate([e0] * 3, axis=2) * v[0:8][None] + jnp.concatenate([e1] * 3, axis=2) * v[8:16][None]
        acc = unrotate(jnp.concatenate([t, e0 + e1], axis=2), jnp.add)
        return acc[:, :PW] * jnp.concatenate([_recip(acc[:, PW:])] * 3, axis=1)

    def bstep(h, first, never, early, chained_in, chained_out, pre=None):
        qkv, ps, os_, ov = {}, {}, {}, {}
        acc = {}
        nxt = [0]
        late = NP - (3 if pre is not None else LATE)

        split = pre is not None and first

        def is_long(first, t, m):
            flipped = FLIP.get(t) == m
            return (flipped and not first) if pre is not None else first != flipped

        hb = {True: h.astype(bf16), False: h[:NQ].astype(bf16)}

        def PR(t, ms):
            hs = {m: h if is_long(first, t, m) else h[:NQ] for m in ms}
            if t == 0 and chained_in:
                rs = {}
                for k in range(5):
                    for m in ms:
                        c = _dot(hs[m][:, 128 * k:128 * k + 128].astype(bf16),
                                 _unpack(wb_ref[t, 64 * k:64 * k + 64, m * PW:(m + 1) * PW]))
                        rs[m] = c if k == 0 else rs[m] + c
            else:
                rs = {m: _dot(hb[is_long(first, t, m)], _unpack(wb_ref[t, :, m * PW:(m + 1) * PW])) for m in ms}
            for m in ms:
                if is_long(first, t, m):
                    svq_ref[t, :, m * PW:(m + 1) * PW] = rs[m][L:]
                    qkv[t, m] = rs[m][:L]
                else:
                    cols = slice(m * PW, (m + 1) * PW)
                    saved = svq_ref[t, :, cols] if pre is None else pre_ref[t, pl.ds(pl.multiple_of(pre * 8, 8), 8), cols]
                    qkv[t, m] = jnp.concatenate([rs[m], saved], axis=0)
            if not (split and t >= NP - 2):
                HA_(t)

        def HA_(t):
            k, v = [jnp.concatenate([qkv[t, m][:MEM], qkv[t, m][NQ:]], axis=0) for m in (1, 2)]
            ov[t] = head_attention(qkv[t, 0][NQ:], k, v)

        def SS(j):
            ps[j] = scores(qkv[j, 0][:NQ], qkv[j, 1])

        def PV(j):
            e, l = ps[j]
            ja = j - (ANCHOR_A if first else ANCHOR_B)
            if ja >= 0 and not (first and ja >= late):
                e = jnp.concatenate([jnp.where(never, ov[ja][:, 128 * c:128 * c + 2 * L], e[8 * c:8 * c + 8])
                                     for c in range(3)] + [e[24:]], axis=0)
            if j in early:
                e = jnp.concatenate([e[:24], jnp.where(never, early[j][:, :2 * L], e[24:32]), e[32:]], axis=0)
            o = values(e, l, qkv[j, 2])
            if first and j >= late:
                svo_ref[j] = ov[j]
            elif first:
                svo_ref[j] = o[24:32]
                o = jnp.concatenate([o[:24], ov[j]], axis=0)
            else:
                o = jnp.concatenate([o, ov[j], svo_ref[j]], axis=0)
            os_[j] = o

        def OO(merge=1):
            js = range(nxt[0], nxt[0] + merge)
            w = wob_ref[js[0] * DHB:(js[-1] + 1) * DHB, :]
            ws = [w[n * DHB + o:n * DHB + o + 32] for n in range(merge) for o in VPERM]
            c = _dot(jnp.concatenate([os_[j] for j in js], axis=1).astype(bf16), _unpack(jnp.concatenate(ws, axis=0)))
            for key, part in ((0, c[:-8]), (1 + (js[0] >= late), c[-8:])):
                acc[key] = acc[key] + part if key in acc else part
            nxt[0] += merge

        order, tail = (ORD_A, TAIL_W if split else TAIL_A) if first else (ORD_B, TAIL_C if chained_out else TAIL_B)
        olag = OLAG_A if first else OLAG_B
        nl = (3 if split else MERGE_A) if first else 1
        nd = tail.count("O") + nl
        for t in range(NP):
            for op in order:
                if op == "Q":
                    PR(t, PORD_A if first else PORD_B)
                    if split and t == NP - 1:
                        pl.when(pre == 0)(lambda: cp_wob.wait())
                        HA_(NP - 2), HA_(NP - 1)
                if op == "S" and t >= 1:
                    SS(t - 1)
                if op == "P" and t >= 2:
                    PV(t - 2)
                if op == "O" and olag <= t < NP - 1 and nxt[0] < NP - nd:
                    OO()
        p = NP - 2
        for op in tail:
            if op == "O":
                OO()
            if op == "S":
                SS(NP - 1)
            if op == "P":
                PV(p)
                p += 1
        OO(nl)
        assert nxt[0] == NP and p == NP
        hand = {LATE_AT + n: jnp.maximum(jnp.maximum(ov[j][:, 0:128], ov[j][:, 128:256]), ov[j][:, 256:384])
                for n, j in enumerate(range(late, NP))} if first else None
        return acc[0], acc[1], acc[2], hand

    def bpass(last, lo_it, hi_it, warm=False):
        def body(i, c):
            never = flag_ref[:, :2 * L] > 0
            probe = lambda x, g: x[8 * g:8 * g + 8, 0:128]
            mem = mem_ref[...]
            if warm:
                slots = [pl.ds(pl.multiple_of(i * 64, 64), 64)]
                heads = [xnb_ref[pl.ds(pl.multiple_of((1 - i) * 64, 64), 8), :]]
            else:
                slots = [pl.ds(0, 64), pl.ds(64, 64)]
            xs = [xnb_ref[sl, :] for sl in slots]
            n = len(slots)
            for u in range(n):
                r0 = pl.multiple_of((i * n + u) * 64, 64)
                xa = xs[u]
                rn = pl.multiple_of(jnp.minimum(r0 + 128, S - 64), 64)
                xn = _layernorm(xres_ref[pl.ds(rn, 64), :])
                xnb_ref[slots[u], :] = xn
                if not warm and u == 0:
                    heads = [xs[1][0:8], xn[0:8]]
                early = {LN_AT + g: probe(xn, g) for g in range(8)}
                if not last:
                    rp = pl.multiple_of(jnp.maximum(r0 - 64, 0), 64)
                    xn = _layernorm(xres_ref[pl.ds(rp, 64), :])
                    xna_ref[pl.ds(pl.multiple_of(rp // 2, 32), 32), :] = _pack(xn)
                    for g in range(8):
                        j = LN_AT2 + g
                        early[j] = jnp.maximum(early[j], probe(xn, g)) if j in early else probe(xn, g)
                ya, a0, a24, hand = bstep(jnp.concatenate([mem, xa[8:32], xa[0:8], xa[32:40]], axis=0), True, never, early,
                           u > 0, True, 2 * i if warm else None)
                yb, b24, b0, _ = bstep(jnp.concatenate([ya[:MEM], xa[40:64], xa[32:40], heads[u]], axis=0), False, never, hand,
                           True, u < n - 1, 2 * i + 1 if warm else None)
                mem = yb[:MEM]
                y = xres_ref[pl.ds(r0, 64), :] + jnp.concatenate([a0 + b0, ya[MEM:24], a24 + b24, yb[32:40], yb[MEM:32]], axis=0)
                if last:
                    out_ref[pl.ds(r0, 64), :] = y.astype(bf16)
                else:
                    xres_ref[pl.ds(r0, 64), :] = y
            mem_ref[...] = mem
            if last:
                rows = pl.ds(pl.multiple_of(i * 128, 128), 128)
                pltpu.make_async_copy(out_ref.at[rows, :], out_hbm.at[rows, :], sems.at[7]).start()
            return c
        lax.fori_loop(lo_it, hi_it, body, 0)

    load_in = lambda rows: x_ref[rows, :].astype(f32)
    load_res = lambda rows: xres_ref[rows, :]
    NB = S // (TB * NCH)

    def k1_body(i, c):
        pl.when(i == 1)(lambda: cp_x(3).wait())
        k_blocks([1 + i * KB + j for j in range(KB)], load_in, jnp.minimum(1 + i * KB + KB, S // TB - 1))
        return c

    def q1_body(i, c):
        for m in range(3):
            cp_w(m, i).wait()
        pairs = [i * (NP // NCH) + j for j in range(NP // NCH)]
        for j in pairs:
            relayout_weights(j)
        head = []

        def norm_first():
            x0 = _layernorm(xres_ref[0:128, :])
            xnb_ref[...] = x0
            head.append(jnp.concatenate([x0[32 * sg:32 * sg + 8] for sg in range(4)], axis=0).astype(bf16))

        def project(js):
            for j in js:
                pre_ref[j] = _dot(head[0], _unpack(wb_ref[j]))

        q_blocks([i * NB + j for j in range(NB)], load_in,
                 {(0, 4): norm_first, (1, 4): lambda: project(pairs[:1]), (2, 4): lambda: project(pairs[1:3]),
                  (3, 4): lambda: project(pairs[3:])})
        return c

    with _scope("pro"):
        flag_ref[...] = jnp.zeros(flag_ref.shape, jnp.int32)
        cnt_ref[0] = 0
        cp_phi.wait()
        cp_x(0).wait()
        phi_lhs = phi_blocks()
        xna_ref[0:TB // 2, :] = _pack(_layernorm(load_in(pl.ds(0, TB))))
        cp_wqkv(1).wait()
        fold_phi(phi_lhs, 1, wpkt_ref)

        def values_ready():
            cp_wqkv(2).wait()
            cp_x(1).wait()
            wvt_ref[...] = pltpu.bitcast(_unpack(wqkv_ref[2]).T, u32)
            xna_ref[TB // 2:TB, :] = _pack(_layernorm(load_in(pl.ds(TB, TB))))

        k_blocks([0], init=True, mid=values_ready)
        cp_x(2).wait()
    with _scope("k1"):
        lax.fori_loop(0, (S // TB - 1) // KB, k1_body, 0)
    with _scope("f1"):
        cp_wqkv(0).wait()
        cp_woa.wait()
        cp_mem.wait()
        fold_phi(phi_lhs, 0, wpqt_ref)
        finish_kv()
        mem_ref[...] = mem0_ref[...].astype(f32)
    with _scope("q1"):
        lax.fori_loop(0, NCH, q1_body, 0)
    with _scope("b1w"):
        bpass(False, 0, 2, warm=True)
    with _scope("b1"):
        bpass(False, 1, S // 128)
    with _scope("a2"):
        lax.fori_loop(0, cnt_ref[0] + 1, lambda i, c: (k_blocks(list(range(KSPLIT)), init=True), c)[1], 0)
        xna_ref[(S - 64) // 2:, :] = _pack(_layernorm(xres_ref[S - 64:, :]))
        k_blocks(list(range(KSPLIT, S // TB)))
        head = []

        def norm_first():
            x0 = _layernorm(xres_ref[0:128, :])
            xnb_ref[...] = x0
            head.append(x0[0:16].astype(bf16))

        def save_rows(t, c):
            svq_ref[t, :, c:c + 128] = _dot(head[0], _unpack(wb_ref[t, :, c:c + 128]))[:8]

        hooks = {(0, 4): norm_first}
        pieces = [(t, m * PW + 128 * c) for t, m in FLIP.items() for c in range(3)]
        for n, piece in enumerate(pieces):
            hooks[2 + n // 2, 1 + 2 * (n % 2)] = functools.partial(save_rows, *piece)
        q_blocks(list(range(S // TB)), load_res, hooks, between=finish_kv)
        mem_ref[...] = mem0_ref[...].astype(f32)
    with _scope("b2"):
        bpass(True, 0, S // 128)
    pltpu.make_async_copy(out_ref, out_hbm, sems.at[7]).wait()


@jax.jit
def pallas_interleave_layers__linear_kernel_hedgehog__memory_aug_recurrent_mem_tr__prompt_kernel(
    A_x: jax.Array,
    A_wqkv: jax.Array,
    A_w_phi: jax.Array,
    A_wo: jax.Array,
    B_x: jax.Array,
    B_mem0: jax.Array,
    B_Wq: jax.Array,
    B_Wk: jax.Array,
    B_Wv: jax.Array,
    B_Wo: jax.Array,
    B_seg_len: jax.Array,
):
    del B_x
    del B_seg_len
    assert A_x.shape == (1, S, D) and B_mem0.shape == (1, MEM, D)
    assert B_Wq.shape == (D, HB, DHB) and A_w_phi.shape == (HA, FA, FA)
    tr = lambda w: jnp.transpose(w, (1, 2, 0)).reshape(HB * DHB, D)
    hbm = pl.BlockSpec(memory_space=pl.ANY)
    out = pl.pallas_call(
        _kernel,
        out_shape=jax.ShapeDtypeStruct((S, D), bf16),
        in_specs=[hbm] * 9,
        out_specs=hbm,
        scratch_shapes=[
            pltpu.VMEM((S, D), bf16),
            pltpu.VMEM((3, D // 2, D), u32),
            pltpu.VMEM((FA, FA, HA), bf16),
            pltpu.VMEM((D // 2, D), u32),
            pltpu.VMEM((MEM, D), bf16),
            pltpu.VMEM((S, D), bf16),
            pltpu.VMEM((3, HB * DHB // 2, D), u32),
            pltpu.VMEM((NP, D // 2, 3 * PW), u32),
            pltpu.VMEM((HB * DHB // 2, D), u32),
            pltpu.VMEM((S, D), f32),
            pltpu.VMEM((S // 2, D), u32),
            pltpu.VMEM((128, D), f32),
            pltpu.VMEM((PR_ROWS // 2, D), u32),
            pltpu.VMEM((PR_ROWS // 2, D), u32),
            pltpu.VMEM((D // 2, D), u32),
            pltpu.VMEM((NG, 48, 2 * GR), f32),
            pltpu.VMEM((NG, 24, 2 * GR), u32),
            pltpu.VMEM((S // TB, TB // 2, D), u32),
            pltpu.VMEM((MEM, D), f32),
            pltpu.VMEM((NP, 8, 3 * PW), f32),
            pltpu.VMEM((NP, 32, 3 * PW), f32),
            pltpu.VMEM((NP, 8, PW), f32),
            pltpu.VMEM((8, 128), jnp.int32),
            pltpu.SMEM((1,), jnp.int32),
            pltpu.SemaphoreType.DMA((12 + 3 * NCH,)),
        ],
        compiler_params=pltpu.CompilerParams(vmem_limit_bytes=120 * 1024 * 1024, disable_bounds_checks=True,
                                             disable_semaphore_checks=True),
        name="hedgehog_rmt",
    )(A_x.reshape(S, D), A_wqkv, jnp.transpose(A_w_phi, (1, 2, 0)), A_wo, B_mem0.reshape(MEM, D),
      tr(B_Wq), tr(B_Wk), tr(B_Wv), B_Wo.reshape(HB * DHB, D))
    return out.reshape(1, S, D)
```
